```python
import jax
import jax.numpy as jnp

def _softmax(x, axis=-1):
    return jax.nn.softmax(x, axis=axis)

def _gelu(x):
    return jax.nn.gelu(x, approximate=True)

def _silu(x):
    return jax.nn.silu(x)

def _sigmoid(x):
    return jax.nn.sigmoid(x)

def _layernorm(x, axis=-1, eps=1e-05):
    m = jnp.mean(x, axis=axis, keepdims=True)
    v = jnp.var(x, axis=axis, keepdims=True)
    return (x - m) / jnp.sqrt(v + eps)

def _scatter_add(tgt, idx, src, axis=0):
    return tgt.at[idx].add(src)

def _segment_sum(src, seg, n):
    return jax.ops.segment_sum(src, seg, n)

class _Rng:

    def __init__(self, key):
        self._k = key

    def _next(self):
        self._k, sub = jax.random.split(self._k)
        return sub

    def normal(self, shape):
        return jax.random.normal(self._next(), shape, dtype=jnp.bfloat16)

    def randint(self, lo, hi, shape):
        return jax.random.randint(self._next(), shape, lo, hi, dtype=jnp.int32)

    def uniform(self, shape, lo=0.0, hi=1.0):
        return jax.random.uniform(self._next(), shape, jnp.bfloat16, lo, hi)

    def permutation(self, n):
        return jax.random.permutation(self._next(), n)
kernel_name = 'interleave_layers__memory_aug_recurrent_mem_tr__mixer_s_mlp__prompt'

def setup_inputs():
    _rng = _Rng(jax.random.key(int.from_bytes(__import__("os").urandom(4), "little")))
    _w = lambda a: (lambda t: t.astype(jnp.bfloat16) if jnp.issubdtype(t.dtype, jnp.floating) else t)(jnp.asarray(a))

    def _A_setup():
        B, S, Dm = (1, 2048, 640)
        H, Dh = (32, 192)
        M, seg = (8, 32)
        seg = min(seg, S)
        S = S // seg * seg
        return {'x': _w((lambda *s: _rng.normal(s) * 0.05)(B, S, Dm)), 'mem0': _w((lambda *s: _rng.normal(s) * 0.05)(B, M, Dm)), 'Wq': _w((lambda *s: _rng.normal(s) * 0.05)(Dm, H, Dh) * Dm ** (-0.5)), 'Wk': _w((lambda *s: _rng.normal(s) * 0.05)(Dm, H, Dh) * Dm ** (-0.5)), 'Wv': _w((lambda *s: _rng.normal(s) * 0.05)(Dm, H, Dh) * Dm ** (-0.5)), 'Wo': _w((lambda *s: _rng.normal(s) * 0.05)(H, Dh, Dm) * (H * Dh) ** (-0.5)), 'seg_len': seg}
    _A_in = _A_setup()

    def _B_setup():
        B, S, D, F = (1, 2048, 640, 1536)
        return {'x': _w((lambda *s: _rng.normal(s) * 0.05)(B, S, D)), 'w1': _w((lambda *s: _rng.normal(s) * 0.05)(D, D) * D ** (-0.5)), 'w2': _w((lambda *s: _rng.normal(s) * 0.05)(D, D) * D ** (-0.5)), 'w3': _w((lambda *s: _rng.normal(s) * 0.05)(D, F) * D ** (-0.5)), 'w4': _w((lambda *s: _rng.normal(s) * 0.05)(F, D) * F ** (-0.5))}
    _B_in = _B_setup()
    return {'A_x': _A_in['x'], 'A_mem0': _A_in['mem0'], 'A_Wq': _A_in['Wq'], 'A_Wk': _A_in['Wk'], 'A_Wv': _A_in['Wv'], 'A_Wo': _A_in['Wo'], 'A_seg_len': _A_in['seg_len'], 'B_x': _B_in['x'], 'B_w1': _B_in['w1'], 'B_w2': _B_in['w2'], 'B_w3': _B_in['w3'], 'B_w4': _B_in['w4']}

def reference(A_x, A_mem0, A_Wq, A_Wk, A_Wv, A_Wo, A_seg_len, B_x, B_w1, B_w2, B_w3, B_w4):

    def _A_ref(x, mem0, Wq, Wk, Wv, Wo, seg_len):
        B, S, Dm = x.shape
        H, Dh = (Wq.shape[1], Wq.shape[2])
        M = mem0.shape[1]
        scale = Dh ** (-0.5)
        n_seg = S // seg_len
        L = M + seg_len
        idx = jnp.arange(L)
        mask = (idx[:, None] < M) | (idx[:, None] >= idx[None, :])
        mem = mem0
        outs = []
        for s in range(n_seg):
            xs = x[:, s * seg_len:(s + 1) * seg_len, :].copy()
            h = jnp.concatenate([mem, xs], axis=1)
            q = jnp.einsum('btd,dhe->bhte', h, Wq)
            k = jnp.einsum('btd,dhe->bhte', h, Wk)
            v = jnp.einsum('btd,dhe->bhte', h, Wv)
            scores = jnp.einsum('bhqe,bhke->bhqk', q, k) * scale
            scores = jnp.where(mask[None, None], scores, -1000000000.0)
            p = _softmax(scores, axis=-1)
            o = jnp.einsum('bhqk,bhke->bhqe', p, v)
            o = jnp.einsum('bhte,hed->btd', o, Wo)
            mem = o[:, :M, :].copy()
            outs.append(o[:, M:, :])
        return jnp.concatenate(outs, axis=1)

    def _B_ref(x, w1, w2, w3, w4):
        B, S, D = x.shape
        h = _gelu(_layernorm(x, axis=-1) @ w1)
        c = D // 4
        g0 = jnp.pad(h[:, :, 0 * c:1 * c], ((0, 0), (1, 0), (0, 0)))[:, :S, :]
        g1 = jnp.pad(h[:, :, 1 * c:2 * c], ((0, 0), (0, 1), (0, 0)))[:, 1:, :]
        g2 = jnp.pad(h[:, :, 2 * c:3 * c], ((0, 0), (2, 0), (0, 0)))[:, :S, :]
        g3 = jnp.pad(h[:, :, 3 * c:], ((0, 0), (0, 2), (0, 0)))[:, 2:, :]
        hs = jnp.concatenate([g0, g1, g2, g3], axis=-1) @ w2
        x1 = x + hs
        h2 = _gelu(_layernorm(x1, axis=-1) @ w3) @ w4
        return x1 + h2
    x = A_x
    x = x + _A_ref(_layernorm(x, axis=-1), A_mem0, A_Wq, A_Wk, A_Wv, A_Wo, A_seg_len)
    x = x + _B_ref(_layernorm(x, axis=-1), B_w1, B_w2, B_w3, B_w4)
    x = x + _A_ref(_layernorm(x, axis=-1), A_mem0, A_Wq, A_Wk, A_Wv, A_Wo, A_seg_len)
    x = x + _B_ref(_layernorm(x, axis=-1), B_w1, B_w2, B_w3, B_w4)
    return x
```

```python
import functools
import jax
import jax.numpy as jnp
import numpy as np
import jax.experimental.pallas as pl
import jax.experimental.pallas.tpu as pltpu

F32 = jnp.float32
BF16 = jnp.bfloat16

S_TOT = 2048
DM = 640
NH = 32
DH = 192
HD = NH * DH
MEM = 8
SEG = 32
NSEG = S_TOT // SEG
L = MEM + SEG
NP = NH // 2
PW = 2 * DH
FF = 1536
CH = 256
NCH = S_TOT // CH
NSLOT = 3
LOG2E = 1.4426950408889634


def _ln(x, eps=1e-5):
    m = jnp.mean(x, axis=-1, keepdims=True)
    xc = x - m
    v = jnp.mean(xc * xc, axis=-1, keepdims=True)
    return xc * jax.lax.rsqrt(v + eps)


def _gelu(x):
    return jax.nn.gelu(x, approximate=True)


def _dot(a, b):
    return jnp.dot(a, b, preferred_element_type=F32)


def _dot_nt(a, b):
    return jax.lax.dot_general(a, b, (((1,), (1,)), ((), ())), preferred_element_type=F32)


def _kernel(x_hbm, mem0_hbm, wq_hbm, wk_hbm, wv_hbm, wo_hbm, w1_hbm, w2_hbm, w3_hbm, w4_hbm,
            out_hbm,
            wqkv, wo, w1, w2, w3, w4, stage, xin, mem0, xbuf, ybuf, hbuf, obuf,
            sem_stage, sem_misc, sem_out):
    def stage_copies(p, slot):
        return [pltpu.make_async_copy(w.at[pl.ds(p * PW, PW), :], stage.at[slot, j], sem_stage.at[slot, j])
                for j, w in enumerate((wq_hbm, wk_hbm, wv_hbm))]

    cx = pltpu.make_async_copy(x_hbm, xin, sem_misc.at[0])
    cm = pltpu.make_async_copy(mem0_hbm, mem0, sem_misc.at[1])
    cwo = pltpu.make_async_copy(wo_hbm, wo, sem_misc.at[2])
    cw1 = pltpu.make_async_copy(w1_hbm, w1, sem_misc.at[3])
    cw2 = pltpu.make_async_copy(w2_hbm, w2, sem_misc.at[4])
    cw3 = pltpu.make_async_copy(w3_hbm, w3, sem_misc.at[5])
    cw4 = pltpu.make_async_copy(w4_hbm, w4, sem_misc.at[6])
    cx.start()
    cm.start()
    for p in range(NSLOT):
        for c in stage_copies(p, p):
            c.start()
    cx.wait()
    cm.wait()

    def ln0(c, carry):
        r = pl.multiple_of(c * CH, CH)
        xv = xin[pl.ds(r, CH), :].astype(F32)
        xbuf[pl.ds(r, CH), :] = xv
        ybuf[pl.ds(r, CH), :] = _ln(xv)
        return carry
    jax.lax.fori_loop(0, NCH, ln0, 0)
    hbuf[pl.ds(0, 8), :] = jnp.zeros((8, DM), F32)
    hbuf[pl.ds(8 + S_TOT, 8), :] = jnp.zeros((8, DM), F32)

    for p in range(NP):
        slot = p % NSLOT
        for c in stage_copies(p, slot):
            c.wait()
        for j in range(3):
            wqkv[p, :, j * PW:(j + 1) * PW] = stage[slot, j].T
        if p + NSLOT < NP:
            for c in stage_copies(p + NSLOT, slot):
                c.start()
        if p + NSLOT == NP - 1:
            cwo.start()
    cw1.start()
    cw2.start()
    cw3.start()
    cw4.start()
    cwo.wait()

    row = jax.lax.broadcasted_iota(jnp.int32, (L, 128), 0)
    lane = jax.lax.broadcasted_iota(jnp.int32, (L, 128), 1)
    NEG = np.float32(-1e30)
    MASKED = np.float32(-1e9 * LOG2E)
    realA = lane < L
    realB = (lane >= 64) & (lane < 64 + L)
    validA = realA & ((row < MEM) | (row >= lane))
    validB = realB & ((row < MEM) | (row >= lane - 64))
    fillA = jnp.where(realA, MASKED, NEG)
    fillB = jnp.where(realB, MASKED, NEG)
    isA = lane < 64
    SC = np.float32(DH ** -0.5 * LOG2E)
    lane48 = jax.lax.broadcasted_iota(jnp.int32, (48, 128), 1)
    lo48 = lane48 < 64

    def blk(t):
        tb = jnp.concatenate([t, jnp.zeros((8, PW), F32)], axis=0).astype(BF16)
        t0 = tb[:, 0:128]
        t1 = tb[:, 128:256]
        t2 = tb[:, 256:384]
        z16 = jnp.zeros((16, 128), BF16)
        z64 = jnp.zeros((64, 128), BF16)
        z80 = jnp.zeros((80, 128), BF16)
        zb = jnp.zeros((48, 128), BF16)
        c0 = jnp.concatenate([t0, z80], axis=0)
        c1 = jnp.concatenate([jnp.where(lo48, t1, zb), z16, jnp.where(lo48, zb, t1), z16], axis=0)
        c2 = jnp.concatenate([z64, t2, z16], axis=0)
        return jnp.concatenate([c0, c1, c2], axis=1)

    def a_step(s, mem):
        r = pl.multiple_of(s * SEG, SEG)
        y = ybuf[pl.ds(r, SEG), :]
        h = jnp.concatenate([mem, y], axis=0)
        acc = None
        for p in range(NP):
            qkv = _dot(h, wqkv[p])
            q = qkv[:, 0:PW]
            kb = blk(qkv[:, PW:2 * PW])
            vb = blk(qkv[:, 2 * PW:3 * PW])
            t = _dot_nt(q, kb) * SC
            sA = jnp.where(validA, t, fillA)
            sB = jnp.where(validB, t, fillB)
            mA = jnp.max(sA, axis=-1, keepdims=True)
            mB = jnp.max(sB, axis=-1, keepdims=True)
            e = jnp.exp2(jnp.where(isA, sA - mA, sB - mB))
            lA = jnp.sum(jnp.where(isA, e, 0.0), axis=-1, keepdims=True)
            lB = jnp.sum(jnp.where(isA, 0.0, e), axis=-1, keepdims=True)
            pr = e * jnp.where(isA, 1.0 / lA, 1.0 / lB)
            o = _dot(pr, vb)
            c = _dot(o, wo[pl.ds(p * PW, PW), :])
            acc = c if acc is None else acc + c
        xbuf[pl.ds(r, SEG), :] = xbuf[pl.ds(r, SEG), :] + acc[MEM:, :]
        return acc[0:MEM, :]

    lane_h = jax.lax.broadcasted_iota(jnp.int32, (CH, 128), 1)

    def b1(c, carry):
        r = pl.multiple_of(c * CH, CH)
        x1 = xbuf[pl.ds(r, CH), :]
        y = _ln(x1)
        ybuf[pl.ds(r, CH), :] = y
        yy = _ln(y)
        hbuf[pl.ds(r + 8, CH), :] = _gelu(_dot(yy, w1[...]))
        return carry

    def b2(c, layer):
        r = pl.multiple_of(c * CH, CH)

        def sh(j, d):
            win = hbuf[pl.ds(r, CH + 16), j * 128:(j + 1) * 128]
            return win[8 + d:8 + d + CH, :]
        cols = [
            sh(0, -1),
            jnp.where(lane_h < 32, sh(1, -1), sh(1, 1)),
            jnp.where(lane_h < 64, sh(2, 1), sh(2, -2)),
            jnp.where(lane_h < 96, sh(3, -2), sh(3, 2)),
            sh(4, 2),
        ]
        hs_in = jnp.concatenate(cols, axis=1)
        y1 = ybuf[pl.ds(r, CH), :] + _dot(hs_in, w2[...])
        z = _ln(y1)
        g = _gelu(_dot(z, w3[...]))
        xn = xbuf[pl.ds(r, CH), :] + (y1 + _dot(g, w4[...]))
        xbuf[pl.ds(r, CH), :] = xn
        ybuf[pl.ds(r, CH), :] = _ln(xn)
        obuf[pl.ds(r, CH), :] = xn.astype(BF16)

        @pl.when(layer == 1)
        def _():
            pltpu.make_async_copy(obuf.at[pl.ds(r, CH), :], out_hbm.at[pl.ds(r, CH), :], sem_out.at[c]).start()
        return layer

    def layer_body(layer, carry):
        jax.lax.fori_loop(0, NSEG, a_step, mem0[...].astype(F32))

        @pl.when(layer == 0)
        def _():
            cw1.wait()
            cw2.wait()
            cw3.wait()
            cw4.wait()
        jax.lax.fori_loop(0, NCH, b1, 0)
        jax.lax.fori_loop(0, NCH, b2, layer)
        return carry

    jax.lax.fori_loop(0, 2, layer_body, 0)
    for c in range(NCH):
        pltpu.make_async_copy(obuf.at[pl.ds(c * CH, CH), :], out_hbm.at[pl.ds(c * CH, CH), :], sem_out.at[c]).wait()


@jax.jit
def pallas_interleave_layers__memory_aug_recurrent_mem_tr__mixer_s_mlp__prompt_kernel(A_x, A_mem0, A_Wq, A_Wk, A_Wv, A_Wo, A_seg_len, B_x, B_w1, B_w2, B_w3, B_w4):
    del A_seg_len, B_x
    x2 = A_x.reshape(S_TOT, DM)
    m2 = A_mem0.reshape(MEM, DM)
    wqT = A_Wq.transpose(1, 2, 0).reshape(HD, DM)
    wkT = A_Wk.transpose(1, 2, 0).reshape(HD, DM)
    wvT = A_Wv.transpose(1, 2, 0).reshape(HD, DM)
    wo2 = A_Wo.reshape(HD, DM)
    any_spec = pl.BlockSpec(memory_space=pl.ANY)
    out = pl.pallas_call(
        _kernel,
        out_shape=jax.ShapeDtypeStruct((S_TOT, DM), BF16),
        in_specs=[any_spec] * 10,
        out_specs=any_spec,
        scratch_shapes=[
            pltpu.VMEM((NP, DM, 3 * PW), BF16),
            pltpu.VMEM((HD, DM), BF16),
            pltpu.VMEM((DM, DM), BF16),
            pltpu.VMEM((DM, DM), BF16),
            pltpu.VMEM((DM, FF), BF16),
            pltpu.VMEM((FF, DM), BF16),
            pltpu.VMEM((NSLOT, 3, PW, DM), BF16),
            pltpu.VMEM((S_TOT, DM), BF16),
            pltpu.VMEM((MEM, DM), BF16),
            pltpu.VMEM((S_TOT, DM), F32),
            pltpu.VMEM((S_TOT, DM), F32),
            pltpu.VMEM((S_TOT + 16, DM), F32),
            pltpu.VMEM((S_TOT, DM), BF16),
            pltpu.SemaphoreType.DMA((NSLOT, 3)),
            pltpu.SemaphoreType.DMA((7,)),
            pltpu.SemaphoreType.DMA((NCH,)),
        ],
        compiler_params=pltpu.CompilerParams(vmem_limit_bytes=100 * 1024 * 1024),
    )(x2, m2, wqT, wkT, wvT, wo2, B_w1, B_w2, B_w3, B_w4)
    return out.reshape(1, S_TOT, DM)
```

```python
import functools
import jax
import jax.numpy as jnp
import numpy as np
import jax.experimental.pallas as pl
import jax.experimental.pallas.tpu as pltpu

F32 = jnp.float32
BF16 = jnp.bfloat16

S_TOT = 2048
DM = 640
NH = 32
DH = 192
HD = NH * DH
MEM = 8
SEG = 32
NSEG = S_TOT // SEG
L = MEM + SEG
NP = NH // 2
PW = 2 * DH
FF = 1536
CH = 256
NCH = S_TOT // CH
NSLOT = 3
LOG2E = 1.4426950408889634


def _make_sched(lag_s=1, lag_v=2, lag_o=5):
    ops = []
    i = 0
    done_o = 0
    while done_o < NP:
        if i < NP:
            ops.append(('q', i))
        if 0 <= i - lag_s < NP:
            ops.append(('s', i - lag_s))
        if 0 <= i - lag_o < NP:
            ops.append(('o', i - lag_o))
            done_o += 1
        if 0 <= i - lag_v < NP:
            ops.append(('v', i - lag_v))
        i += 1
    return ops


SCHED = _make_sched()


def _ln(x, eps=1e-5):
    m = jnp.mean(x, axis=-1, keepdims=True)
    xc = x - m
    v = jnp.mean(xc * xc, axis=-1, keepdims=True)
    return xc * jax.lax.rsqrt(v + eps)


def _gelu(x):
    return jax.nn.gelu(x, approximate=True)


def _dot(a, b):
    return jnp.dot(a, b, preferred_element_type=F32)


def _dot_nt(a, b):
    return jax.lax.dot_general(a, b, (((1,), (1,)), ((), ())), preferred_element_type=F32)


def _kernel(x_hbm, mem0_hbm, wq_hbm, wk_hbm, wv_hbm, wo_hbm, w1_hbm, w2_hbm, w3_hbm, w4_hbm,
            out_hbm,
            wqkv, wo, w1, w2, w3, w4, stage, xin, mem0, xbuf, ybuf, hbuf, obuf,
            sem_stage, sem_misc, sem_out, sem_wo):
    def stage_copies(p, slot):
        return [pltpu.make_async_copy(w.at[pl.ds(p * PW, PW), :], stage.at[slot, j], sem_stage.at[slot, j])
                for j, w in enumerate((wq_hbm, wk_hbm, wv_hbm))]

    cx = pltpu.make_async_copy(x_hbm, xin, sem_misc.at[0])
    cm = pltpu.make_async_copy(mem0_hbm, mem0, sem_misc.at[1])
    cwo = [pltpu.make_async_copy(wo_hbm.at[:, pl.ds(j * 128, 128)], wo.at[j], sem_wo.at[j]) for j in range(5)]
    cw1 = pltpu.make_async_copy(w1_hbm, w1, sem_misc.at[3])
    cw2 = pltpu.make_async_copy(w2_hbm, w2, sem_misc.at[4])
    cw3 = pltpu.make_async_copy(w3_hbm, w3, sem_misc.at[5])
    cw4 = pltpu.make_async_copy(w4_hbm, w4, sem_misc.at[6])
    cx.start()
    cm.start()
    for p in range(NSLOT):
        for c in stage_copies(p, p):
            c.start()
    cx.wait()
    cm.wait()

    def ln0(c, carry):
        r = pl.multiple_of(c * CH, CH)
        xv = xin[pl.ds(r, CH), :].astype(F32)
        xbuf[pl.ds(r, CH), :] = xv
        ybuf[pl.ds(r, CH), :] = _ln(xv)
        return carry
    jax.lax.fori_loop(0, NCH, ln0, 0)
    hbuf[pl.ds(0, 8), :] = jnp.zeros((8, DM), F32)
    hbuf[pl.ds(8 + S_TOT, 8), :] = jnp.zeros((8, DM), F32)

    for p in range(NP):
        slot = p % NSLOT
        for c in stage_copies(p, slot):
            c.wait()
        for j in range(3):
            wt = stage[slot, j].T
            for c in range(3):
                wqkv[p, 3 * j + c] = wt[:, c * 128:(c + 1) * 128]
        if p + NSLOT < NP:
            for c in stage_copies(p + NSLOT, slot):
                c.start()
        if p + NSLOT == NP - 1:
            for c in cwo:
                c.start()
    cw1.start()
    cw2.start()
    cw3.start()
    cw4.start()
    for c in cwo:
        c.wait()

    row = jax.lax.broadcasted_iota(jnp.int32, (L, 128), 0)
    lane = jax.lax.broadcasted_iota(jnp.int32, (L, 128), 1)
    NEG = np.float32(-1e30)
    MASKED = np.float32(-1e9 * LOG2E)
    realA = lane < L
    realB = (lane >= 64) & (lane < 64 + L)
    validA = realA & ((row < MEM) | (row >= lane))
    validB = realB & ((row < MEM) | (row >= lane - 64))
    fillA = jnp.where(realA, MASKED, NEG)
    fillB = jnp.where(realB, MASKED, NEG)
    isA = lane < 64
    SC = np.float32(DH ** -0.5 * LOG2E)
    lane48 = jax.lax.broadcasted_iota(jnp.int32, (48, 128), 1)
    lo48 = lane48 < 64

    def blk(t):
        tb = jnp.concatenate([t, jnp.zeros((8, PW), F32)], axis=0).astype(BF16)
        t0 = tb[:, 0:128]
        t1 = tb[:, 128:256]
        t2 = tb[:, 256:384]
        z16 = jnp.zeros((16, 128), BF16)
        z64 = jnp.zeros((64, 128), BF16)
        z80 = jnp.zeros((80, 128), BF16)
        zb = jnp.zeros((48, 128), BF16)
        c0 = jnp.concatenate([t0, z80], axis=0)
        c1 = jnp.concatenate([jnp.where(lo48, t1, zb), z16, jnp.where(lo48, zb, t1), z16], axis=0)
        c2 = jnp.concatenate([z64, t2, z16], axis=0)
        return jnp.concatenate([c0, c1, c2], axis=1)

    def a_step(s, mem):
        r = pl.multiple_of(s * SEG, SEG)
        y = ybuf[pl.ds(r, SEG), :]
        h = jnp.concatenate([mem, y], axis=0)
        st = {}

        def f_qkv(p):
            w = jnp.concatenate([wqkv[p, c] for c in range(9)], axis=1)
            qkv = _dot(h, w)
            st['q', p] = qkv[:, 0:PW]
            st['k', p] = blk(qkv[:, PW:2 * PW])
            st['v', p] = blk(qkv[:, 2 * PW:3 * PW])

        def f_s(p):
            t = _dot_nt(st['q', p], st['k', p]) * SC
            sA = jnp.where(validA, t, fillA)
            sB = jnp.where(validB, t, fillB)
            mA = jnp.max(sA, axis=-1, keepdims=True)
            mB = jnp.max(sB, axis=-1, keepdims=True)
            e = jnp.exp2(jnp.where(isA, sA - mA, sB - mB))
            lA = jnp.sum(jnp.where(isA, e, 0.0), axis=-1, keepdims=True)
            lB = jnp.sum(jnp.where(isA, 0.0, e), axis=-1, keepdims=True)
            st['p', p] = e * jnp.where(isA, 1.0 / lA, 1.0 / lB)

        def f_pv(p):
            st['o', p] = _dot(st['p', p], st['v', p])

        def f_o(p):
            w = jnp.concatenate([wo[j, pl.ds(p * PW, PW), :] for j in range(5)], axis=1)
            c = _dot(st['o', p], w)
            st['acc'] = c if 'acc' not in st else st['acc'] + c

        for op, p in SCHED:
            {'q': f_qkv, 's': f_s, 'v': f_pv, 'o': f_o}[op](p)
        acc = st['acc']
        xbuf[pl.ds(r, SEG), :] = xbuf[pl.ds(r, SEG), :] + acc[MEM:, :]
        return acc[0:MEM, :]

    lane_h = jax.lax.broadcasted_iota(jnp.int32, (CH, 128), 1)

    def b1(c, carry):
        r = pl.multiple_of(c * CH, CH)
        x1 = xbuf[pl.ds(r, CH), :]
        y = _ln(x1)
        ybuf[pl.ds(r, CH), :] = y
        yy = _ln(y)
        hbuf[pl.ds(r + 8, CH), :] = _gelu(_dot(yy, w1[...]))
        return carry

    def b2(c, layer):
        r = pl.multiple_of(c * CH, CH)

        def sh(j, d):
            win = hbuf[pl.ds(r, CH + 16), j * 128:(j + 1) * 128]
            return win[8 + d:8 + d + CH, :]
        cols = [
            sh(0, -1),
            jnp.where(lane_h < 32, sh(1, -1), sh(1, 1)),
            jnp.where(lane_h < 64, sh(2, 1), sh(2, -2)),
            jnp.where(lane_h < 96, sh(3, -2), sh(3, 2)),
            sh(4, 2),
        ]
        hs_in = jnp.concatenate(cols, axis=1)
        y1 = ybuf[pl.ds(r, CH), :] + _dot(hs_in, w2[...])
        z = _ln(y1)
        g = _gelu(_dot(z, w3[...]))
        xn = xbuf[pl.ds(r, CH), :] + (y1 + _dot(g, w4[...]))
        xbuf[pl.ds(r, CH), :] = xn
        ybuf[pl.ds(r, CH), :] = _ln(xn)
        obuf[pl.ds(r, CH), :] = xn.astype(BF16)

        @pl.when(layer == 1)
        def _():
            pltpu.make_async_copy(obuf.at[pl.ds(r, CH), :], out_hbm.at[pl.ds(r, CH), :], sem_out.at[c]).start()
        return layer

    def layer_body(layer, carry):
        jax.lax.fori_loop(0, NSEG, a_step, mem0[...].astype(F32))

        @pl.when(layer == 0)
        def _():
            cw1.wait()
            cw2.wait()
            cw3.wait()
            cw4.wait()
        jax.lax.fori_loop(0, NCH, b1, 0)
        jax.lax.fori_loop(0, NCH, b2, layer)
        return carry

    jax.lax.fori_loop(0, 2, layer_body, 0)
    for c in range(NCH):
        pltpu.make_async_copy(obuf.at[pl.ds(c * CH, CH), :], out_hbm.at[pl.ds(c * CH, CH), :], sem_out.at[c]).wait()


@jax.jit
def pallas_interleave_layers__memory_aug_recurrent_mem_tr__mixer_s_mlp__prompt_kernel(A_x, A_mem0, A_Wq, A_Wk, A_Wv, A_Wo, A_seg_len, B_x, B_w1, B_w2, B_w3, B_w4):
    del A_seg_len, B_x
    x2 = A_x.reshape(S_TOT, DM)
    m2 = A_mem0.reshape(MEM, DM)
    wqT = A_Wq.transpose(1, 2, 0).reshape(HD, DM)
    wkT = A_Wk.transpose(1, 2, 0).reshape(HD, DM)
    wvT = A_Wv.transpose(1, 2, 0).reshape(HD, DM)
    wo2 = A_Wo.reshape(HD, DM)
    any_spec = pl.BlockSpec(memory_space=pl.ANY)
    out = pl.pallas_call(
        _kernel,
        out_shape=jax.ShapeDtypeStruct((S_TOT, DM), BF16),
        in_specs=[any_spec] * 10,
        out_specs=any_spec,
        scratch_shapes=[
            pltpu.VMEM((NP, 9, DM, 128), BF16),
            pltpu.VMEM((5, HD, 128), BF16),
            pltpu.VMEM((DM, DM), BF16),
            pltpu.VMEM((DM, DM), BF16),
            pltpu.VMEM((DM, FF), BF16),
            pltpu.VMEM((FF, DM), BF16),
            pltpu.VMEM((NSLOT, 3, PW, DM), BF16),
            pltpu.VMEM((S_TOT, DM), BF16),
            pltpu.VMEM((MEM, DM), BF16),
            pltpu.VMEM((S_TOT, DM), F32),
            pltpu.VMEM((S_TOT, DM), F32),
            pltpu.VMEM((S_TOT + 16, DM), F32),
            pltpu.VMEM((S_TOT, DM), BF16),
            pltpu.SemaphoreType.DMA((NSLOT, 3)),
            pltpu.SemaphoreType.DMA((7,)),
            pltpu.SemaphoreType.DMA((NCH,)),
            pltpu.SemaphoreType.DMA((5,)),
        ],
        compiler_params=pltpu.CompilerParams(vmem_limit_bytes=100 * 1024 * 1024),
    )(x2, m2, wqT, wkT, wvT, wo2, B_w1, B_w2, B_w3, B_w4)
    return out.reshape(1, S_TOT, DM)
```

```python
import functools
import jax
import jax.numpy as jnp
import numpy as np
import jax.experimental.pallas as pl
import jax.experimental.pallas.tpu as pltpu

F32 = jnp.float32
BF16 = jnp.bfloat16
U32 = jnp.uint32

S_TOT = 2048
DM = 640
NH = 32
DH = 192
HD = NH * DH
MEM = 8
SEG = 32
NSEG = S_TOT // SEG
L = MEM + SEG
NP = NH // 2
PW = 2 * DH
FF = 1536
CH = 256
NCH = S_TOT // CH
NSLOT = 3
LOG2E = 1.4426950408889634
SCOPES = False
KT_XLU = False


def _make_sched(lag_s=1, lag_v=2, lag_o=5):
    ops = []
    i = 0
    done_o = 0
    while done_o < NP:
        if i < NP:
            ops.append(('q', i))
        if 0 <= i - lag_s < NP:
            ops.append(('s', i - lag_s))
        if 0 <= i - lag_o < NP:
            ops.append(('o', i - lag_o))
            done_o += 1
        if 0 <= i - lag_v < NP:
            ops.append(('v', i - lag_v))
        i += 1
    return ops


SCHED = _make_sched()


def _ln(x, eps=1e-5):
    m = jnp.mean(x, axis=-1, keepdims=True)
    xc = x - m
    v = jnp.mean(xc * xc, axis=-1, keepdims=True)
    return xc * jax.lax.rsqrt(v + eps)


def _gelu(x):
    return jax.nn.gelu(x, approximate=True)


def _dot(a, b):
    return jnp.dot(a, b, preferred_element_type=F32)


def _dot_nt(a, b):
    return jax.lax.dot_general(a, b, (((1,), (1,)), ((), ())), preferred_element_type=F32)


def _scope(name):
    import contextlib
    return jax.named_scope(name) if SCOPES else contextlib.nullcontext()


def _kernel(x_hbm, mem0_hbm, wq_hbm, wk_hbm, wv_hbm, wo_hbm, w1_hbm, w2_hbm, w3_hbm, w4_hbm,
            out_hbm,
            wqkv, wo, xbuf, ybuf, hbuf, w1, w2, w3, w4, stage, xin, obuf, mem0,
            sem_stage, sem_misc, sem_out):
    def stage_copies(p, slot):
        return [pltpu.make_async_copy(w.at[pl.ds(p * PW, PW), :], stage.at[slot, j], sem_stage.at[slot, j])
                for j, w in enumerate((wq_hbm, wk_hbm, wv_hbm, wo_hbm))]

    cx = pltpu.make_async_copy(x_hbm, xin, sem_misc.at[0])
    cm = pltpu.make_async_copy(mem0_hbm, mem0, sem_misc.at[1])
    cw1 = pltpu.make_async_copy(w1_hbm, w1, sem_misc.at[3])
    cw2 = pltpu.make_async_copy(w2_hbm, w2, sem_misc.at[4])
    cw3 = pltpu.make_async_copy(w3_hbm, w3, sem_misc.at[5])
    cw4 = pltpu.make_async_copy(w4_hbm, w4, sem_misc.at[6])
    for p in range(NSLOT):
        for c in stage_copies(p, p):
            c.start()
    cx.start()
    cm.start()
    cx.wait()
    cm.wait()

    def ln0(c, carry):
        r = pl.multiple_of(c * CH, CH)
        xv = xin[pl.ds(r, CH), :].astype(F32)
        xbuf[pl.ds(r, CH), :] = xv
        ybuf[pl.ds(r, CH), :] = _ln(xv)
        return carry
    jax.lax.fori_loop(0, NCH, ln0, 0)
    hbuf[pl.ds(0, 8), :] = jnp.zeros((8, DM), F32)
    hbuf[pl.ds(8 + S_TOT, 8), :] = jnp.zeros((8, DM), F32)

    for p in range(NP):
        slot = p % NSLOT
        for c in stage_copies(p, slot):
            c.wait()
        for j in range(3):
            wt = stage[slot, j].T
            for c in range(3):
                wqkv[p, 3 * j + c] = pltpu.bitcast(wt[:, c * 128:(c + 1) * 128], U32)
        for c in range(5):
            wo[c, pl.ds(p * (PW // 2), PW // 2), :] = pltpu.bitcast(stage[slot, 3, :, c * 128:(c + 1) * 128], U32)
        if p + NSLOT < NP:
            for c in stage_copies(p + NSLOT, slot):
                c.start()
        if p + NSLOT == NP:
            cw1.start()
            cw2.start()
            cw3.start()
            cw4.start()

    row = jax.lax.broadcasted_iota(jnp.int32, (L, 128), 0)
    lane = jax.lax.broadcasted_iota(jnp.int32, (L, 128), 1)
    NEG = np.float32(-1e30)
    MASKED = np.float32(-1e9 * LOG2E)
    realA = lane < L
    realB = (lane >= 64) & (lane < 64 + L)
    validA = realA & ((row < MEM) | (row >= lane))
    validB = realB & ((row < MEM) | (row >= lane - 64))
    fillA = jnp.where(realA, MASKED, NEG)
    fillB = jnp.where(realB, MASKED, NEG)
    isA = lane < 64
    SC = np.float32(DH ** -0.5 * LOG2E)
    lane48 = jax.lax.broadcasted_iota(jnp.int32, (48, 128), 1)
    lo48 = lane48 < 64

    def blk(t):
        tb = jnp.concatenate([t, jnp.zeros((8, PW), F32)], axis=0).astype(BF16)
        t0 = tb[:, 0:128]
        t1 = tb[:, 128:256]
        t2 = tb[:, 256:384]
        z16 = jnp.zeros((16, 128), BF16)
        z64 = jnp.zeros((64, 128), BF16)
        z80 = jnp.zeros((80, 128), BF16)
        zb = jnp.zeros((48, 128), BF16)
        c0 = jnp.concatenate([t0, z80], axis=0)
        c1 = jnp.concatenate([jnp.where(lo48, t1, zb), z16, jnp.where(lo48, zb, t1), z16], axis=0)
        c2 = jnp.concatenate([z64, t2, z16], axis=0)
        return jnp.concatenate([c0, c1, c2], axis=1)

    def a_step(s, mem):
        r = pl.multiple_of(s * SEG, SEG)
        y = ybuf[pl.ds(r, SEG), :]
        h = jnp.concatenate([mem, y], axis=0)
        st = {}

        def f_qkv(p):
            w = jnp.concatenate([pltpu.bitcast(wqkv[p, c], BF16) for c in range(9)], axis=1)
            qkv = _dot(h, w)
            st['q', p] = qkv[:, 0:PW]
            kb = blk(qkv[:, PW:2 * PW])
            st['k', p] = pltpu.bitcast(pltpu.bitcast(kb.T, U32), BF16) if KT_XLU else kb
            st['v', p] = blk(qkv[:, 2 * PW:3 * PW])

        def f_s(p):
            if KT_XLU:
                t = _dot(st['q', p], st['k', p]) * SC
            else:
                t = _dot_nt(st['q', p], st['k', p]) * SC
            sA = jnp.where(validA, t, fillA)
            sB = jnp.where(validB, t, fillB)
            mA = jnp.max(sA, axis=-1, keepdims=True)
            mB = jnp.max(sB, axis=-1, keepdims=True)
            e = jnp.exp2(jnp.where(isA, sA - mA, sB - mB))
            lA = jnp.sum(jnp.where(isA, e, 0.0), axis=-1, keepdims=True)
            lB = jnp.sum(jnp.where(isA, 0.0, e), axis=-1, keepdims=True)
            st['p', p] = e * jnp.where(isA, 1.0 / lA, 1.0 / lB)

        def f_pv(p):
            st['o', p] = _dot(st['p', p], st['v', p])

        def f_o(p):
            w = jnp.concatenate([pltpu.bitcast(wo[j, pl.ds(p * (PW // 2), PW // 2), :], BF16) for j in range(5)], axis=1)
            c = _dot(st['o', p], w)
            st['acc'] = c if 'acc' not in st else st['acc'] + c

        for op, p in SCHED:
            {'q': f_qkv, 's': f_s, 'v': f_pv, 'o': f_o}[op](p)
        acc = st['acc']
        xbuf[pl.ds(r, SEG), :] = xbuf[pl.ds(r, SEG), :] + acc[MEM:, :]
        return acc[0:MEM, :]

    lane_h = jax.lax.broadcasted_iota(jnp.int32, (CH, 128), 1)

    def b1(c, carry):
        r = pl.multiple_of(c * CH, CH)
        x1 = xbuf[pl.ds(r, CH), :]
        y = _ln(x1)
        ybuf[pl.ds(r, CH), :] = y
        yy = _ln(y)
        hbuf[pl.ds(r + 8, CH), :] = _gelu(_dot(yy, w1[...]))
        return carry

    def b2(c, layer):
        r = pl.multiple_of(c * CH, CH)

        def sh(j, d):
            win = hbuf[pl.ds(r, CH + 16), j * 128:(j + 1) * 128]
            return win[8 + d:8 + d + CH, :]
        cols = [
            sh(0, -1),
            jnp.where(lane_h < 32, sh(1, -1), sh(1, 1)),
            jnp.where(lane_h < 64, sh(2, 1), sh(2, -2)),
            jnp.where(lane_h < 96, sh(3, -2), sh(3, 2)),
            sh(4, 2),
        ]
        hs_in = jnp.concatenate(cols, axis=1)
        y1 = ybuf[pl.ds(r, CH), :] + _dot(hs_in, w2[...])
        z = _ln(y1)
        g = _gelu(_dot(z, w3[...]))
        xn = xbuf[pl.ds(r, CH), :] + (y1 + _dot(g, w4[...]))
        xbuf[pl.ds(r, CH), :] = xn
        ybuf[pl.ds(r, CH), :] = _ln(xn)
        obuf[pl.ds(r, CH), :] = xn.astype(BF16)

        @pl.when(layer == 1)
        def _():
            pltpu.make_async_copy(obuf.at[pl.ds(r, CH), :], out_hbm.at[pl.ds(r, CH), :], sem_out.at[c]).start()
        return layer

    def layer_body(layer, carry):
        with _scope("A_pass"):
            jax.lax.fori_loop(0, NSEG, a_step, mem0[...].astype(F32))

        @pl.when(layer == 0)
        def _():
            cw1.wait()
            cw2.wait()
            cw3.wait()
            cw4.wait()
        with _scope("B1"):
            jax.lax.fori_loop(0, NCH, b1, 0)
        with _scope("B2"):
            jax.lax.fori_loop(0, NCH, b2, layer)
        return carry

    jax.lax.fori_loop(0, 2, layer_body, 0)
    for c in range(NCH):
        pltpu.make_async_copy(obuf.at[pl.ds(c * CH, CH), :], out_hbm.at[pl.ds(c * CH, CH), :], sem_out.at[c]).wait()


@jax.jit
def pallas_interleave_layers__memory_aug_recurrent_mem_tr__mixer_s_mlp__prompt_kernel(A_x, A_mem0, A_Wq, A_Wk, A_Wv, A_Wo, A_seg_len, B_x, B_w1, B_w2, B_w3, B_w4):
    del A_seg_len, B_x
    x2 = A_x.reshape(S_TOT, DM)
    m2 = A_mem0.reshape(MEM, DM)
    wqT = A_Wq.transpose(1, 2, 0).reshape(HD, DM)
    wkT = A_Wk.transpose(1, 2, 0).reshape(HD, DM)
    wvT = A_Wv.transpose(1, 2, 0).reshape(HD, DM)
    wo2 = A_Wo.reshape(HD, DM)
    any_spec = pl.BlockSpec(memory_space=pl.ANY)
    out = pl.pallas_call(
        _kernel,
        out_shape=jax.ShapeDtypeStruct((S_TOT, DM), BF16),
        in_specs=[any_spec] * 10,
        out_specs=any_spec,
        scratch_shapes=[
            pltpu.VMEM((NP, 9, DM // 2, 128), U32),
            pltpu.VMEM((5, HD // 2, 128), U32),
            pltpu.VMEM((S_TOT, DM), F32),
            pltpu.VMEM((S_TOT, DM), F32),
            pltpu.VMEM((S_TOT + 32, DM), F32),
            pltpu.VMEM((DM, DM), BF16),
            pltpu.VMEM((DM, DM), BF16),
            pltpu.VMEM((DM, FF), BF16),
            pltpu.VMEM((FF, DM), BF16),
            pltpu.VMEM((NSLOT, 4, PW, DM), BF16),
            pltpu.VMEM((S_TOT, DM), BF16),
            pltpu.VMEM((S_TOT, DM), BF16),
            pltpu.VMEM((MEM, DM), BF16),
            pltpu.SemaphoreType.DMA((NSLOT, 4)),
            pltpu.SemaphoreType.DMA((7,)),
            pltpu.SemaphoreType.DMA((NCH,)),
        ],
        compiler_params=pltpu.CompilerParams(vmem_limit_bytes=100 * 1024 * 1024),
    )(x2, m2, wqT, wkT, wvT, wo2, B_w1, B_w2, B_w3, B_w4)
    return out.reshape(1, S_TOT, DM)
```

```python
import contextlib
import jax
import jax.numpy as jnp
import numpy as np
import jax.experimental.pallas as pl
import jax.experimental.pallas.tpu as pltpu

F32 = jnp.float32
BF16 = jnp.bfloat16
U32 = jnp.uint32

S_TOT = 2048
DM = 640
NH = 32
DH = 192
HD = NH * DH
MEM = 8
SEG = 32
NSEG = S_TOT // SEG
L = MEM + SEG
NP = NH // 2
PW = 2 * DH
FF = 1536
CH = 256
NSLOT = 3
HB_DUMMY = S_TOT + 32
LOG2E = 1.4426950408889634
SCOPES = False


def _make_sched(lag_s=1, lag_v=2, lag_o=5, b_pos=None):
    ops = []
    i = 0
    done_o = 0
    while done_o < NP:
        if i < NP:
            ops.append(('q', i))
        if b_pos and i in b_pos:
            for b in b_pos[i]:
                ops.append((b, 0))
        if 0 <= i - lag_s < NP:
            ops.append(('s', i - lag_s))
        if 0 <= i - lag_o < NP:
            ops.append(('o', i - lag_o))
            done_o += 1
        if 0 <= i - lag_v < NP:
            ops.append(('v', i - lag_v))
        i += 1
    return ops


SCHED_A = _make_sched()
SCHED_AB = _make_sched(b_pos={1: ['b1'], 4: ['b2a'], 8: ['b2b'], 12: ['b2c']})


def _ln(x, eps=1e-5):
    m = jnp.mean(x, axis=-1, keepdims=True)
    xc = x - m
    v = jnp.mean(xc * xc, axis=-1, keepdims=True)
    return xc * jax.lax.rsqrt(v + eps)


def _gelu(x):
    return jax.nn.gelu(x, approximate=True)


def _dot(a, b):
    return jnp.dot(a, b, preferred_element_type=F32)


def _dot_nt(a, b):
    return jax.lax.dot_general(a, b, (((1,), (1,)), ((), ())), preferred_element_type=F32)


def _scope(name):
    return jax.named_scope(name) if SCOPES else contextlib.nullcontext()


def _wload(ref, ntile):
    return jnp.concatenate([pltpu.bitcast(ref[c], BF16) for c in range(ntile)], axis=1)


def _kernel(x_hbm, mem0_hbm, wq_hbm, wk_hbm, wv_hbm, wo_hbm, w1_hbm, w2_hbm, w3_hbm, w4_hbm,
            out_hbm,
            wqkv, wo, w1, w2, w3, w4, xbuf, ybuf, hbuf, obuf, stage, xin, w1s, w2s, w3s, w4s, mem0,
            sem_stage, sem_misc, sem_out):
    def stage_copies(p, slot):
        return [pltpu.make_async_copy(w.at[pl.ds(p * PW, PW), :], stage.at[slot, j], sem_stage.at[slot, j])
                for j, w in enumerate((wq_hbm, wk_hbm, wv_hbm, wo_hbm))]

    cx = pltpu.make_async_copy(x_hbm, xin, sem_misc.at[0])
    cm = pltpu.make_async_copy(mem0_hbm, mem0, sem_misc.at[1])
    cw = [pltpu.make_async_copy(a, b, sem_misc.at[2 + i])
          for i, (a, b) in enumerate(((w1_hbm, w1s), (w2_hbm, w2s), (w3_hbm, w3s), (w4_hbm, w4s)))]
    for p in range(NSLOT):
        for c in stage_copies(p, p):
            c.start()
    cx.start()
    cm.start()
    z32 = jnp.zeros((32, DM), F32)
    hbuf[pl.ds(0, 8), :] = z32[0:8]
    hbuf[pl.ds(8 + S_TOT, 8), :] = z32[0:8]
    hbuf[pl.ds(HB_DUMMY - 16, 32), :] = z32
    hbuf[pl.ds(HB_DUMMY + 16, 32), :] = z32
    xbuf[pl.ds(S_TOT, 32), :] = z32
    ybuf[pl.ds(S_TOT, 32), :] = z32
    cx.wait()
    cm.wait()

    def ln0(c, carry):
        r = pl.multiple_of(c * CH, CH)
        xv = xin[pl.ds(r, CH), :].astype(F32)
        xbuf[pl.ds(r, CH), :] = xv
        ybuf[pl.ds(r, CH), :] = _ln(xv)
        return carry
    jax.lax.fori_loop(0, S_TOT // CH, ln0, 0)

    for p in range(NP):
        slot = p % NSLOT
        for c in stage_copies(p, slot):
            c.wait()
        for j in range(3):
            wt = stage[slot, j].T
            for c in range(3):
                wqkv[p, 3 * j + c] = pltpu.bitcast(wt[:, c * 128:(c + 1) * 128], U32)
        for c in range(5):
            wo[c, pl.ds(p * (PW // 2), PW // 2), :] = pltpu.bitcast(stage[slot, 3, :, c * 128:(c + 1) * 128], U32)
        if p + NSLOT < NP:
            for c in stage_copies(p + NSLOT, slot):
                c.start()
        if p + NSLOT == NP:
            for c in cw:
                c.start()

    row = jax.lax.broadcasted_iota(jnp.int32, (L, 128), 0)
    lane = jax.lax.broadcasted_iota(jnp.int32, (L, 128), 1)
    NEG = np.float32(-1e30)
    MASKED = np.float32(-1e9 * LOG2E)
    realA = lane < L
    realB = (lane >= 64) & (lane < 64 + L)
    validA = realA & ((row < MEM) | (row >= lane))
    validB = realB & ((row < MEM) | (row >= lane - 64))
    fillA = jnp.where(realA, MASKED, NEG)
    fillB = jnp.where(realB, MASKED, NEG)
    isA = lane < 64
    SC = np.float32(DH ** -0.5 * LOG2E)
    lane48 = jax.lax.broadcasted_iota(jnp.int32, (48, 128), 1)
    lo48 = lane48 < 64
    lane_h = jax.lax.broadcasted_iota(jnp.int32, (SEG, 128), 1)

    def blk(t):
        tb = jnp.concatenate([t, jnp.zeros((8, PW), F32)], axis=0).astype(BF16)
        t0 = tb[:, 0:128]
        t1 = tb[:, 128:256]
        t2 = tb[:, 256:384]
        z16 = jnp.zeros((16, 128), BF16)
        z64 = jnp.zeros((64, 128), BF16)
        z80 = jnp.zeros((80, 128), BF16)
        zb = jnp.zeros((48, 128), BF16)
        c0 = jnp.concatenate([t0, z80], axis=0)
        c1 = jnp.concatenate([jnp.where(lo48, t1, zb), z16, jnp.where(lo48, zb, t1), z16], axis=0)
        c2 = jnp.concatenate([z64, t2, z16], axis=0)
        return jnp.concatenate([c0, c1, c2], axis=1)

    def run(sched, rA=None, mem=None, rB1=None, rB2=None, rH=None):
        st = {}
        if rA is not None:
            st['h'] = jnp.concatenate([mem, ybuf[pl.ds(rA, SEG), :]], axis=0)

        def f_qkv(p):
            qkv = _dot(st['h'], _wload(wqkv.at[p], 9))
            st['q', p] = qkv[:, 0:PW]
            st['k', p] = blk(qkv[:, PW:2 * PW])
            st['v', p] = blk(qkv[:, 2 * PW:3 * PW])

        def f_s(p):
            t = _dot_nt(st['q', p], st['k', p]) * SC
            sA = jnp.where(validA, t, fillA)
            sB = jnp.where(validB, t, fillB)
            mA = jnp.max(sA, axis=-1, keepdims=True)
            mB = jnp.max(sB, axis=-1, keepdims=True)
            e = jnp.exp2(jnp.where(isA, sA - mA, sB - mB))
            lA = jnp.sum(jnp.where(isA, e, 0.0), axis=-1, keepdims=True)
            lB = jnp.sum(jnp.where(isA, 0.0, e), axis=-1, keepdims=True)
            st['p', p] = e * jnp.where(isA, 1.0 / lA, 1.0 / lB)

        def f_pv(p):
            st['o', p] = _dot(st['p', p], st['v', p])

        def f_o(p):
            w = jnp.concatenate([pltpu.bitcast(wo[j, pl.ds(p * (PW // 2), PW // 2), :], BF16) for j in range(5)], axis=1)
            c = _dot(st['o', p], w)
            st['acc'] = c if 'acc' not in st else st['acc'] + c

        def f_b1(_):
            x1 = xbuf[pl.ds(rB1, SEG), :]
            y = _ln(x1)
            ybuf[pl.ds(rB1, SEG), :] = y
            hbuf[pl.ds(rB1 + 8, SEG), :] = _gelu(_dot(_ln(y), _wload(w1, 5)))

        def f_b2a(_):
            def sh(j, d):
                win = hbuf[pl.ds(rH, SEG + 16), j * 128:(j + 1) * 128]
                return win[8 + d:8 + d + SEG, :]
            cols = [
                sh(0, -1),
                jnp.where(lane_h < 32, sh(1, -1), sh(1, 1)),
                jnp.where(lane_h < 64, sh(2, 1), sh(2, -2)),
                jnp.where(lane_h < 96, sh(3, -2), sh(3, 2)),
                sh(4, 2),
            ]
            hs_in = jnp.concatenate(cols, axis=1)
            st['y1'] = ybuf[pl.ds(rB2, SEG), :] + _dot(hs_in, _wload(w2, 5))

        def f_b2b(_):
            st['g'] = _gelu(_dot(_ln(st['y1']), _wload(w3, 12)))

        def f_b2c(_):
            xn = xbuf[pl.ds(rB2, SEG), :] + (st['y1'] + _dot(st['g'], _wload(w4, 5)))
            xbuf[pl.ds(rB2, SEG), :] = xn
            ybuf[pl.ds(rB2, SEG), :] = _ln(xn)
            obuf[pl.ds(rB2, SEG), :] = xn.astype(BF16)

        fs = {'q': f_qkv, 's': f_s, 'v': f_pv, 'o': f_o, 'b1': f_b1, 'b2a': f_b2a, 'b2b': f_b2b, 'b2c': f_b2c}
        for op, p in sched:
            fs[op](p)
        if rA is not None:
            acc = st['acc']
            xbuf[pl.ds(rA, SEG), :] = xbuf[pl.ds(rA, SEG), :] + acc[MEM:, :]
            return acc[0:MEM, :]
        return None

    m0 = mem0[...].astype(F32)
    with _scope("step0"):
        mem1 = run(SCHED_A, rA=0, mem=m0)

    with _scope("bw"):
        for c in cw:
            c.wait()
        for src, dst, nt in ((w1s, w1, 5), (w2s, w2, 5), (w3s, w3, 12), (w4s, w4, 5)):
            for c in range(nt):
                dst[c] = pltpu.bitcast(src[:, c * 128:(c + 1) * 128], U32)

    def body(t, mem):
        segA = t & (NSEG - 1)
        segB1 = (t - 1) & (NSEG - 1)
        live2 = t >= 2
        segB2 = jnp.where(live2, (t - 2) & (NSEG - 1), NSEG)
        rA = pl.multiple_of(segA * SEG, SEG)
        rB1 = pl.multiple_of(segB1 * SEG, SEG)
        rB2 = pl.multiple_of(segB2 * SEG, SEG)
        rH = pl.multiple_of(jnp.where(live2, segB2 * SEG, HB_DUMMY), SEG)
        mem = jnp.where(t == NSEG, mem0[...].astype(F32), mem)
        mem = run(SCHED_AB, rA=rA, mem=mem, rB1=rB1, rB2=rB2, rH=rH)

        @pl.when(jnp.logical_and(t >= NSEG + 3, (t & 1) == 1))
        def _():
            ro = pl.multiple_of((t - (NSEG + 3)) * SEG, 2 * SEG)
            pltpu.make_async_copy(obuf.at[pl.ds(ro, 2 * SEG), :], out_hbm.at[pl.ds(ro, 2 * SEG), :], sem_out.at[0]).start()
        return mem

    with _scope("main"):
        jax.lax.fori_loop(1, 2 * NSEG, body, mem1)

    with _scope("epi"):
        r63 = (NSEG - 1) * SEG
        r62 = (NSEG - 2) * SEG
        run([('b1', 0), ('b2a', 0), ('b2b', 0), ('b2c', 0)], rB1=r63, rB2=r62, rH=r62)
        run([('b2a', 0), ('b2b', 0), ('b2c', 0)], rB2=r63, rH=r63)
        pltpu.make_async_copy(obuf.at[pl.ds(r62, 2 * SEG), :], out_hbm.at[pl.ds(r62, 2 * SEG), :], sem_out.at[0]).start()
        pltpu.make_async_copy(obuf.at[pl.ds(0, S_TOT), :], out_hbm, sem_out.at[0]).wait()


@jax.jit
def pallas_interleave_layers__memory_aug_recurrent_mem_tr__mixer_s_mlp__prompt_kernel(A_x, A_mem0, A_Wq, A_Wk, A_Wv, A_Wo, A_seg_len, B_x, B_w1, B_w2, B_w3, B_w4):
    del A_seg_len, B_x
    x2 = A_x.reshape(S_TOT, DM)
    m2 = A_mem0.reshape(MEM, DM)
    wqT = A_Wq.transpose(1, 2, 0).reshape(HD, DM)
    wkT = A_Wk.transpose(1, 2, 0).reshape(HD, DM)
    wvT = A_Wv.transpose(1, 2, 0).reshape(HD, DM)
    wo2 = A_Wo.reshape(HD, DM)
    any_spec = pl.BlockSpec(memory_space=pl.ANY)
    out = pl.pallas_call(
        _kernel,
        out_shape=jax.ShapeDtypeStruct((S_TOT, DM), BF16),
        in_specs=[any_spec] * 10,
        out_specs=any_spec,
        scratch_shapes=[
            pltpu.VMEM((NP, 9, DM // 2, 128), U32),
            pltpu.VMEM((5, HD // 2, 128), U32),
            pltpu.VMEM((5, DM // 2, 128), U32),
            pltpu.VMEM((5, DM // 2, 128), U32),
            pltpu.VMEM((12, DM // 2, 128), U32),
            pltpu.VMEM((5, FF // 2, 128), U32),
            pltpu.VMEM((S_TOT + 64, DM), F32),
            pltpu.VMEM((S_TOT + 64, DM), F32),
            pltpu.VMEM((S_TOT + 128, DM), F32),
            pltpu.VMEM((S_TOT + 64, DM), BF16),
            pltpu.VMEM((NSLOT, 4, PW, DM), BF16),
            pltpu.VMEM((S_TOT, DM), BF16),
            pltpu.VMEM((DM, DM), BF16),
            pltpu.VMEM((DM, DM), BF16),
            pltpu.VMEM((DM, FF), BF16),
            pltpu.VMEM((FF, DM), BF16),
            pltpu.VMEM((MEM, DM), BF16),
            pltpu.SemaphoreType.DMA((NSLOT, 4)),
            pltpu.SemaphoreType.DMA((6,)),
            pltpu.SemaphoreType.DMA((1,)),
        ],
        compiler_params=pltpu.CompilerParams(vmem_limit_bytes=100 * 1024 * 1024),
    )(x2, m2, wqT, wkT, wvT, wo2, B_w1, B_w2, B_w3, B_w4)
    return out.reshape(1, S_TOT, DM)
```

```python
import contextlib
import jax
import jax.numpy as jnp
import numpy as np
import jax.experimental.pallas as pl
import jax.experimental.pallas.tpu as pltpu

F32 = jnp.float32
BF16 = jnp.bfloat16
U32 = jnp.uint32

S_TOT = 2048
DM = 640
NH = 32
DH = 192
HD = NH * DH
MEM = 8
SEG = 32
NSEG = S_TOT // SEG
L = MEM + SEG
NP = NH // 2
PW = 2 * DH
FF = 1536
X0 = 2 * SEG
LOG2E = 1.4426950408889634
SCOPES = False
NB2C = 4


def _make_sched(lag_s=1, lag_v=2, lag_o=5, b_pos=None, tail=()):
    ops = []
    i = 0
    done_o = 0
    while done_o < NP:
        if i < NP:
            ops.append(('q', i))
        if b_pos and i in b_pos:
            for b in b_pos[i]:
                ops.append(b if isinstance(b, tuple) else (b, 0))
        if 0 <= i - lag_s < NP:
            ops.append(('s', i - lag_s))
        if 0 <= i - lag_o < NP:
            ops.append(('o', i - lag_o))
            done_o += 1
        if 0 <= i - lag_v < NP:
            ops.append(('v', i - lag_v))
        i += 1
    ops.append(('fin', 0))
    for b in tail:
        ops.append((b, 0))
    return ops


def _place(ops, places):
    out = []
    pl_ = {a: l for a, l in places}
    for o in ops:
        out.append(o)
        for b in pl_.get(o, ()):
            out.append(b if isinstance(b, tuple) else (b, 0))
    return out


def _sched0():
    ops = []
    for i in range(NP + 3):
        if i < NP:
            ops += [('wq', i), ('q', i)]
        if 0 <= i - 1 < NP:
            ops.append(('s', i - 1))
        if 0 <= i - 2 < NP:
            ops += [('wo', i - 2), ('v', i - 2)]
        if 0 <= i - 3 < NP:
            ops.append(('o', i - 3))
    ops.append(('fin', 0))
    return ops


SCHED_0 = _sched0()
SCHED_1 = _make_sched(b_pos={4: [('bw', 0)], 5: ['b1'], 7: [('x1', 0)], 8: [('ln0', 1)], 9: [('ln0', 2)],
                             10: [('ln0', 3)], 11: [('ln0', 4)], 12: [('ln0', 5)], 13: [('ln0', 6)],
                             14: [('ln0', 7), ('bw', 1)], 15: [('ln0', 8)]},
                      tail=[])
SCHED_A = _place(_make_sched(), [(('q', 1), ['b1']), (('q', 4), ['b2a']), (('q', 8), ['b2b']),
                                 (('s', 15), [('b2c', 0)]), (('v', 14), [('b2c', 1), 'pre']),
                                 (('fin', 0), [('b2c', 2), ('b2c', 3), 'b2d'])])
SCHED_B = _place(_make_sched(), [(('q', 1), ['b1']), (('q', 4), ['b2a']), (('q', 8), ['b2b']),
                                 (('q', 13), [('b2c', 0)]), (('s', 15), [('b2c', 1)]),
                                 (('v', 14), [('b2c', 2)]), (('o', 12), [('b2c', 3), 'b2d'])])
SCHED_E = [('b2a', 0), ('b2b', 0)] + [('b2c', i) for i in range(NB2C)] + [('b2d', 0)]


def _ln(x, eps=1e-5):
    m = jnp.mean(x, axis=-1, keepdims=True)
    xc = x - m
    v = jnp.mean(xc * xc, axis=-1, keepdims=True)
    return xc * jax.lax.rsqrt(v + eps)


def _gelu(x):
    return jax.nn.gelu(x, approximate=True)


def _dot(a, b):
    return jnp.dot(a, b, preferred_element_type=F32)


def _dot_nt(a, b):
    return jax.lax.dot_general(a, b, (((1,), (1,)), ((), ())), preferred_element_type=F32)


def _scope(name):
    return jax.named_scope(name) if SCOPES else contextlib.nullcontext()


def _wload(ref, ntile, k0=0, kn=None):
    if kn is None:
        return jnp.concatenate([pltpu.bitcast(ref[c], BF16) for c in range(ntile)], axis=1)
    return jnp.concatenate([pltpu.bitcast(ref[c, pl.ds(k0 // 2, kn // 2), :], BF16) for c in range(ntile)], axis=1)


def _kernel(x_hbm, mem0_hbm, wq_hbm, wk_hbm, wv_hbm, wo_hbm, w1_hbm, w2_hbm, w3_hbm, w4_hbm,
            out_hbm,
            wqkv, wo, w1, w2, w3, w4, xbuf, ybuf, hbuf, obuf, stage, xin, w1s, w2s, w3s, w4s, mem0,
            sem_stage, sem_misc, sem_out):
    w_hbm = (wq_hbm, wk_hbm, wv_hbm, wo_hbm)
    cst = {(p, j): pltpu.make_async_copy(w_hbm[j].at[pl.ds(p * PW, PW), :], stage.at[p, j], sem_stage.at[p, j])
           for p in range(NP) for j in range(4)}
    cm = pltpu.make_async_copy(mem0_hbm, mem0, sem_misc.at[0])
    cx0 = pltpu.make_async_copy(x_hbm.at[pl.ds(0, X0), :], xin.at[pl.ds(0, X0), :], sem_misc.at[1])
    cx1 = pltpu.make_async_copy(x_hbm.at[pl.ds(X0, S_TOT - X0), :], xin.at[pl.ds(X0, S_TOT - X0), :], sem_misc.at[2])
    cw = [pltpu.make_async_copy(a, b, sem_misc.at[3 + i])
          for i, (a, b) in enumerate(((w1_hbm, w1s), (w2_hbm, w2s), (w3_hbm, w3s), (w4_hbm, w4s)))]
    cm.start()
    cx0.start()
    for p in range(NP + 2):
        if p == 1:
            cm.wait()
            cx0.wait()
        if p < NP:
            for j in range(3):
                cst[p, j].start()
        if p >= 2:
            cst[p - 2, 3].start()
    cw[0].start()
    cx1.start()
    for c in cw[1:]:
        c.start()

    z8 = jnp.zeros((8, DM), F32)
    hbuf[pl.ds(0, 8), :] = z8
    hbuf[pl.ds(8 + S_TOT, 8), :] = z8

    def ln0(r, n):
        xv = xin[pl.ds(r, n), :].astype(F32)
        xbuf[pl.ds(r, n), :] = xv
        ybuf[pl.ds(r, n), :] = _ln(xv)
    ln0(0, X0)

    row = jax.lax.broadcasted_iota(jnp.int32, (L, 128), 0)
    lane = jax.lax.broadcasted_iota(jnp.int32, (L, 128), 1)
    NEG = np.float32(-1e30)
    MASKED = np.float32(-1e9 * LOG2E)
    realA = lane < L
    realB = (lane >= 64) & (lane < 64 + L)
    validA = realA & ((row < MEM) | (row >= lane))
    validB = realB & ((row < MEM) | (row >= lane - 64))
    valid = validA | validB
    fill = jnp.where(realA | realB, MASKED, NEG)
    isA = lane < 64
    SC = np.float32(DH ** -0.5 * LOG2E)
    lane48 = jax.lax.broadcasted_iota(jnp.int32, (48, 128), 1)
    lo48 = lane48 < 64
    lane_h = jax.lax.broadcasted_iota(jnp.int32, (SEG, 128), 1)

    def blk(t):
        tb = jnp.concatenate([t, jnp.zeros((8, PW), F32)], axis=0).astype(BF16)
        t0 = tb[:, 0:128]
        t1 = tb[:, 128:256]
        t2 = tb[:, 256:384]
        z16 = jnp.zeros((16, 128), BF16)
        z64 = jnp.zeros((64, 128), BF16)
        z80 = jnp.zeros((80, 128), BF16)
        zb = jnp.zeros((48, 128), BF16)
        c0 = jnp.concatenate([t0, z80], axis=0)
        c1 = jnp.concatenate([jnp.where(lo48, t1, zb), z16, jnp.where(lo48, zb, t1), z16], axis=0)
        c2 = jnp.concatenate([z64, t2, z16], axis=0)
        return jnp.concatenate([c0, c1, c2], axis=1)

    def run(sched, rA=None, mem=None, rB1=None, rB2=None, y=None, rPre=None):
        st = {}
        if rA is not None:
            if y is None:
                y = ybuf[pl.ds(rA, SEG), :]
            st['h'] = jnp.concatenate([mem, y], axis=0)

        def f_pre(_):
            st['ypre'] = ybuf[pl.ds(rPre, SEG), :]

        def f_wq(p):
            for j in range(3):
                cst[p, j].wait()
                wt = stage[p, j].T
                for c in range(3):
                    wqkv[p, 3 * j + c] = pltpu.bitcast(wt[:, c * 128:(c + 1) * 128], U32)

        def f_wo(p):
            cst[p, 3].wait()
            for c in range(5):
                wo[c, pl.ds(p * (PW // 2), PW // 2), :] = pltpu.bitcast(stage[p, 3, :, c * 128:(c + 1) * 128], U32)

        def f_bw(i):
            cw[i].wait()
            src, dst, nt = ((w1s, w1, 5), (w2s, w2, 5), (w3s, w3, 12), (w4s, w4, 5))[i]
            for c in range(nt):
                dst[c] = pltpu.bitcast(src[:, c * 128:(c + 1) * 128], U32)

        def f_x1(_):
            cx1.wait()

        def f_ln0(i):
            for r0 in range(max(X0, i * 256 - 256), i * 256, SEG):
                ln0(r0, SEG)

        def f_qkv(p):
            qkv = _dot(st['h'], _wload(wqkv.at[p], 9))
            st['q', p] = qkv[:, 0:PW]
            st['k', p] = blk(qkv[:, PW:2 * PW])
            st['v', p] = blk(qkv[:, 2 * PW:3 * PW])

        def f_s(p):
            t = _dot_nt(st['q', p], st['k', p]) * SC
            s = jnp.where(valid, t, fill)
            mA = jnp.max(jnp.where(isA, s, NEG), axis=-1, keepdims=True)
            mB = jnp.max(jnp.where(isA, NEG, s), axis=-1, keepdims=True)
            e = jnp.exp2(s - jnp.where(isA, mA, mB))
            lA = jnp.sum(jnp.where(isA, e, 0.0), axis=-1, keepdims=True)
            lB = jnp.sum(jnp.where(isA, 0.0, e), axis=-1, keepdims=True)
            l = jnp.where(isA, lA, lB)
            r = pl.reciprocal(l, approx=True)
            r = r * (2.0 - l * r)
            st['p', p] = e * r

        def f_pv(p):
            st['o', p] = _dot(st['p', p], st['v', p])

        def f_o(p):
            c = _dot(st['o', p], _wload(wo, 5, p * PW, PW))
            st['acc'] = c if 'acc' not in st else st['acc'] + c

        def f_fin(_):
            acc = st['acc']
            xbuf[pl.ds(rA, SEG), :] = xbuf[pl.ds(rA, SEG), :] + acc[MEM:, :]
            st['mem'] = acc[0:MEM, :]

        def f_b1(_):
            x1 = xbuf[pl.ds(rB1, SEG), :]
            y = _ln(x1)
            ybuf[pl.ds(rB1, SEG), :] = y
            hbuf[pl.ds(rB1 + 8, SEG), :] = _gelu(_dot(_ln(y), _wload(w1, 5)))

        def f_b2a(_):
            def sh(j, d):
                win = hbuf[pl.ds(rB2, SEG + 16), j * 128:(j + 1) * 128]
                return win[8 + d:8 + d + SEG, :]
            cols = [
                sh(0, -1),
                jnp.where(lane_h < 32, sh(1, -1), sh(1, 1)),
                jnp.where(lane_h < 64, sh(2, 1), sh(2, -2)),
                jnp.where(lane_h < 96, sh(3, -2), sh(3, 2)),
                sh(4, 2),
            ]
            hs_in = jnp.concatenate(cols, axis=1)
            st['y1'] = ybuf[pl.ds(rB2, SEG), :] + _dot(hs_in, _wload(w2, 5))

        def f_b2b(_):
            st['g'] = _gelu(_dot(_ln(st['y1']), _wload(w3, 12)))

        def f_b2c(i):
            kc = FF // NB2C
            c = _dot(st['g'][:, i * kc:(i + 1) * kc], _wload(w4, 5, i * kc, kc))
            st['h2'] = c if 'h2' not in st else st['h2'] + c

        def f_b2d(_):
            xn = xbuf[pl.ds(rB2, SEG), :] + (st['y1'] + st['h2'])
            xbuf[pl.ds(rB2, SEG), :] = xn
            ybuf[pl.ds(rB2, SEG), :] = _ln(xn)
            obuf[pl.ds(rB2, SEG), :] = xn.astype(BF16)

        fs = {'q': f_qkv, 's': f_s, 'v': f_pv, 'o': f_o, 'fin': f_fin, 'b1': f_b1, 'b2a': f_b2a, 'b2b': f_b2b,
              'b2c': f_b2c, 'b2d': f_b2d, 'wq': f_wq, 'wo': f_wo, 'bw': f_bw, 'x1': f_x1,
              'ln0': f_ln0, 'pre': f_pre}
        for op, p in sched:
            fs[op](p)
        return st.get('mem'), st.get('ypre')

    with _scope("step0"):
        mem, _ = run(SCHED_0, rA=0, mem=mem0[...].astype(F32))
    with _scope("step1"):
        mem, _ = run(SCHED_1, rA=SEG, mem=mem, rB1=0)
        run([('bw', 2), ('bw', 3)])

    def body(u, mem):
        t = 2 * u + 2
        rA = pl.multiple_of((t & (NSEG - 1)) * SEG, 2 * SEG)
        rA1 = pl.multiple_of(rA + SEG, SEG)
        rm1 = pl.multiple_of(((t - 1) & (NSEG - 1)) * SEG, SEG)
        rm2 = pl.multiple_of(((t - 2) & (NSEG - 1)) * SEG, 2 * SEG)
        mem = jnp.where(t == NSEG, mem0[...].astype(F32), mem)
        mem, y1 = run(SCHED_A, rA=rA, mem=mem, rB1=rm1, rB2=rm2, rPre=rA1)
        mem, _ = run(SCHED_B, rA=rA1, mem=mem, rB1=rA, rB2=rm1, y=y1)

        @pl.when(t >= NSEG + 2)
        def _():
            pltpu.make_async_copy(obuf.at[pl.ds(rm2, 2 * SEG), :], out_hbm.at[pl.ds(rm2, 2 * SEG), :], sem_out.at[0]).start()
        return mem

    with _scope("main"):
        jax.lax.fori_loop(0, NSEG - 1, body, mem)

    with _scope("epi"):
        r63 = (NSEG - 1) * SEG
        r62 = (NSEG - 2) * SEG
        run([('b1', 0)] + SCHED_E, rB1=r63, rB2=r62)
        run(SCHED_E, rB2=r63)
        pltpu.make_async_copy(obuf.at[pl.ds(r62, 2 * SEG), :], out_hbm.at[pl.ds(r62, 2 * SEG), :], sem_out.at[0]).start()
        pltpu.make_async_copy(obuf.at[pl.ds(0, S_TOT), :], out_hbm, sem_out.at[0]).wait()


@jax.jit
def pallas_interleave_layers__memory_aug_recurrent_mem_tr__mixer_s_mlp__prompt_kernel(A_x, A_mem0, A_Wq, A_Wk, A_Wv, A_Wo, A_seg_len, B_x, B_w1, B_w2, B_w3, B_w4):
    del A_seg_len, B_x
    x2 = A_x.reshape(S_TOT, DM)
    m2 = A_mem0.reshape(MEM, DM)
    wqT = A_Wq.transpose(1, 2, 0).reshape(HD, DM)
    wkT = A_Wk.transpose(1, 2, 0).reshape(HD, DM)
    wvT = A_Wv.transpose(1, 2, 0).reshape(HD, DM)
    wo2 = A_Wo.reshape(HD, DM)
    any_spec = pl.BlockSpec(memory_space=pl.ANY)
    out = pl.pallas_call(
        _kernel,
        out_shape=jax.ShapeDtypeStruct((S_TOT, DM), BF16),
        in_specs=[any_spec] * 10,
        out_specs=any_spec,
        scratch_shapes=[
            pltpu.VMEM((NP, 9, DM // 2, 128), U32),
            pltpu.VMEM((5, HD // 2, 128), U32),
            pltpu.VMEM((5, DM // 2, 128), U32),
            pltpu.VMEM((5, DM // 2, 128), U32),
            pltpu.VMEM((12, DM // 2, 128), U32),
            pltpu.VMEM((5, FF // 2, 128), U32),
            pltpu.VMEM((S_TOT + 64, DM), F32),
            pltpu.VMEM((S_TOT + 64, DM), F32),
            pltpu.VMEM((S_TOT + 64, DM), F32),
            pltpu.VMEM((S_TOT + 64, DM), BF16),
            pltpu.VMEM((NP, 4, PW, DM), BF16),
            pltpu.VMEM((S_TOT, DM), BF16),
            pltpu.VMEM((DM, DM), BF16),
            pltpu.VMEM((DM, DM), BF16),
            pltpu.VMEM((DM, FF), BF16),
            pltpu.VMEM((FF, DM), BF16),
            pltpu.VMEM((MEM, DM), BF16),
            pltpu.SemaphoreType.DMA((NP, 4)),
            pltpu.SemaphoreType.DMA((7,)),
            pltpu.SemaphoreType.DMA((1,)),
        ],
        compiler_params=pltpu.CompilerParams(vmem_limit_bytes=116 * 1024 * 1024),
    )(x2, m2, wqT, wkT, wvT, wo2, B_w1, B_w2, B_w3, B_w4)
    return out.reshape(1, S_TOT, DM)
```

```python
import contextlib
import jax
import jax.numpy as jnp
import numpy as np
import jax.experimental.pallas as pl
import jax.experimental.pallas.tpu as pltpu

F32 = jnp.float32
BF16 = jnp.bfloat16
U32 = jnp.uint32

S_TOT = 2048
DM = 640
NH = 32
DH = 192
HD = NH * DH
MEM = 8
SEG = 32
NSEG = S_TOT // SEG
L = MEM + SEG
NP = NH // 2
PW = 2 * DH
FF = 1536
XC = 256
LOG2E = 1.4426950408889634
SCOPES = False
NB2C = 4
UNROLL = 2
DMA_WINDOW = 6


def _make_sched(lag_s=1, lag_v=2, lag_o=5, b_pos=None, tail=()):
    ops = []
    i = 0
    done_o = 0
    while done_o < NP:
        if i < NP:
            ops.append(('q', i))
        if b_pos and i in b_pos:
            for b in b_pos[i]:
                ops.append(b if isinstance(b, tuple) else (b, 0))
        if 0 <= i - lag_s < NP:
            ops.append(('s', i - lag_s))
        if 0 <= i - lag_o < NP:
            ops.append(('o', i - lag_o))
            done_o += 1
        if 0 <= i - lag_v < NP:
            ops.append(('v', i - lag_v))
        i += 1
    ops.append(('fin', 0))
    for b in tail:
        ops.append((b, 0))
    return ops


XEARLY = {3: 1, 5: 2, 7: 3, 9: 4}


def _place(ops, places):
    out = []
    pl_ = {a: l for a, l in places}
    for o in ops:
        out.append(o)
        for b in pl_.get(o, ()):
            out.append(b if isinstance(b, tuple) else (b, 0))
    return out


def _sched0():
    ops = []
    for i in range(NP + 3):
        if i < NP:
            ops += [('wq', i), ('q', i)]
        if 0 <= i - 1 < NP:
            ops.append(('s', i - 1))
        if 0 <= i - 2 < NP:
            ops += [('wo', i - 2), ('v', i - 2)]
        if i in XEARLY:
            ops.append(('ln0', XEARLY[i]))
        if 0 <= i - 3 < NP:
            ops.append(('o', i - 3))
    ops.append(('fin', 0))
    return ops


SCHED_0 = _sched0()
SCHED_1 = _place(_make_sched(), [(('q', 3), [('bw', 0)]), (('q', 5), ['b1']), (('q', 6), [('ln0', 5)]),
                                 (('q', 9), [('ln0', 6)]), (('q', 12), [('ln0', 7)]), (('q', 14), [('bw', 1)])])
SCHED_A = _place(_make_sched(lag_v=2, lag_o=4),
                 [(('q', 2), ['b1']), (('q', 4), ['b2a']), (('q', 9), ['b2b']),
                  (('q', 14), ['pre', ('b2c', 0), ('b2c', 1)]), (('o', 13), [('b2c', 2)]),
                  (('fin', 0), [('b2c', 3), 'b2d'])])
SCHED_B = _place(_make_sched(lag_v=2, lag_o=5),
                 [(('q', 2), ['b1']), (('q', 4), ['b2a']), (('q', 9), ['b2b']), (('q', 14), [('b2c', 0)]),
                  (('s', 14), [('b2c', 1)]), (('o', 11), [('b2c', 2)]), (('v', 15), [('b2c', 3), 'b2d'])])
SCHED_E = [('b2a', 0), ('b2b', 0)] + [('b2c', i) for i in range(NB2C)] + [('b2d', 0)]


def _ln(x, eps=1e-5):
    m = jnp.mean(x, axis=-1, keepdims=True)
    xc = x - m
    v = jnp.mean(xc * xc, axis=-1, keepdims=True)
    return xc * jax.lax.rsqrt(v + eps)


def _gelu(x):
    return jax.nn.gelu(x, approximate=True)


def _dot(a, b):
    return jnp.dot(a, b, preferred_element_type=F32)


def _dot_nt(a, b):
    return jax.lax.dot_general(a, b, (((1,), (1,)), ((), ())), preferred_element_type=F32)


def _scope(name):
    return jax.named_scope(name) if SCOPES else contextlib.nullcontext()


def _wload(ref, ntile, k0=0, kn=None):
    if kn is None:
        return jnp.concatenate([pltpu.bitcast(ref[c], BF16) for c in range(ntile)], axis=1)
    return jnp.concatenate([pltpu.bitcast(ref[c, pl.ds(k0 // 2, kn // 2), :], BF16) for c in range(ntile)], axis=1)


def _kernel(x_hbm, mem0_hbm, wq_hbm, wk_hbm, wv_hbm, wo_hbm, w1_hbm, w2_hbm, w3_hbm, w4_hbm,
            out_hbm,
            wqkv, wo, w1b, w2b, w3b, w4b, xbuf, ybuf, hbuf, obuf, stage, xin, mem0,
            sem_stage, sem_misc, sem_x, sem_w, sem_out):
    w_hbm = (wq_hbm, wk_hbm, wv_hbm, wo_hbm)

    def cp_x(i):
        return [pltpu.make_async_copy(x_hbm.at[pl.ds(i * XC, XC), :], xin.at[pl.ds(i * XC, XC), :], sem_x.at[i])]

    def cp_w(i, src_ref, dst_ref, ntile):
        return [pltpu.make_async_copy(src_ref.at[:, pl.ds(c * 128, 128)], dst_ref.at[c], sem_w.at[i])
                for c in range(ntile)]

    cps = {'m': [pltpu.make_async_copy(mem0_hbm, mem0, sem_misc.at[0])], ('x', 0): cp_x(0)}
    for p in range(NP + 2):
        for j in ((0, 1, 2) if p < NP else ()) + ((3,) if p >= 2 else ()):
            pp = p - 2 if j == 3 else p
            cps[pp, j] = [pltpu.make_async_copy(w_hbm[j].at[pl.ds(pp * PW, PW), :], stage.at[pp, j], sem_stage.at[pp, j])]
        if p in XEARLY:
            cps['x', XEARLY[p]] = cp_x(XEARLY[p])
    cps['w', 0] = cp_w(0, w1_hbm, w1b, 5)
    for i in range(5, S_TOT // XC):
        cps['x', i] = cp_x(i)
    cps['w', 1] = cp_w(1, w2_hbm, w2b, 5)
    cps['w', 2] = cp_w(2, w3_hbm, w3b, 12)
    cps['w', 3] = cp_w(3, w4_hbm, w4b, 5)
    queue = list(cps)
    issued = [0]

    def start_next():
        if issued[0] < len(queue):
            for c in cps[queue[issued[0]]]:
                c.start()
            issued[0] += 1

    def arrive(key):
        for c in cps[key]:
            c.wait()
        start_next()

    for _ in range(DMA_WINDOW):
        start_next()
    w1, w2, w3, w4 = (r.bitcast(U32) for r in (w1b, w2b, w3b, w4b))

    z8 = jnp.zeros((8, DM), F32)
    hbuf[pl.ds(0, 8), :] = z8
    hbuf[pl.ds(8 + S_TOT, 8), :] = z8
    arrive('m')

    def ln0(i):
        arrive(('x', i))
        for r in range(i * XC, (i + 1) * XC, SEG):
            xv = xin[pl.ds(r, SEG), :].astype(F32)
            xbuf[pl.ds(r, SEG), :] = xv
            ybuf[pl.ds(r, SEG), :] = _ln(xv)
    ln0(0)

    row = jax.lax.broadcasted_iota(jnp.int32, (L, 128), 0)
    lane = jax.lax.broadcasted_iota(jnp.int32, (L, 128), 1)
    NEG = np.float32(-1e30)
    MASKED = np.float32(-1e9 * LOG2E)
    realA = lane < L
    realB = (lane >= 64) & (lane < 64 + L)
    validA = realA & ((row < MEM) | (row >= lane))
    validB = realB & ((row < MEM) | (row >= lane - 64))
    valid = validA | validB
    fill = jnp.where(realA | realB, MASKED, NEG)
    isA = lane < 64
    SC = np.float32(DH ** -0.5 * LOG2E)
    lane48 = jax.lax.broadcasted_iota(jnp.int32, (48, 128), 1)
    lo48 = lane48 < 64
    lane_h = jax.lax.broadcasted_iota(jnp.int32, (SEG, 128), 1)

    def blk(t):
        tb = jnp.concatenate([t, jnp.zeros((8, PW), F32)], axis=0).astype(BF16)
        t0 = tb[:, 0:128]
        t1 = tb[:, 128:256]
        t2 = tb[:, 256:384]
        z16 = jnp.zeros((16, 128), BF16)
        z64 = jnp.zeros((64, 128), BF16)
        z80 = jnp.zeros((80, 128), BF16)
        zb = jnp.zeros((48, 128), BF16)
        c0 = jnp.concatenate([t0, z80], axis=0)
        c1 = jnp.concatenate([jnp.where(lo48, t1, zb), z16, jnp.where(lo48, zb, t1), z16], axis=0)
        c2 = jnp.concatenate([z64, t2, z16], axis=0)
        return jnp.concatenate([c0, c1, c2], axis=1)

    def run(sched, rA=None, mem=None, rB1=None, rB2=None, y=None, rPre=None):
        st = {}
        if rA is not None:
            if y is None:
                y = ybuf[pl.ds(rA, SEG), :]
            st['h'] = jnp.concatenate([mem, y], axis=0)

        def f_pre(_):
            st['ypre'] = ybuf[pl.ds(rPre, SEG), :]

        def f_wq(p):
            for j in range(3):
                arrive((p, j))
                wt = stage[p, j].T
                for c in range(3):
                    wqkv[p, 3 * j + c] = pltpu.bitcast(wt[:, c * 128:(c + 1) * 128], U32)

        def f_wo(p):
            arrive((p, 3))
            for c in range(5):
                wo[c, pl.ds(p * (PW // 2), PW // 2), :] = pltpu.bitcast(stage[p, 3, :, c * 128:(c + 1) * 128], U32)

        def f_bw(i):
            arrive(('w', i))

        def f_qkv(p):
            qkv = _dot(st['h'], _wload(wqkv.at[p], 9))
            st['q', p] = qkv[:, 0:PW]
            st['k', p] = blk(qkv[:, PW:2 * PW])
            st['v', p] = blk(qkv[:, 2 * PW:3 * PW])

        def f_s(p):
            t = _dot_nt(st['q', p], st['k', p]) * SC
            s = jnp.where(valid, t, fill)
            mA = jnp.max(jnp.where(isA, s, NEG), axis=-1, keepdims=True)
            mB = jnp.max(jnp.where(isA, NEG, s), axis=-1, keepdims=True)
            e = jnp.exp2(s - jnp.where(isA, mA, mB))
            lA = jnp.sum(jnp.where(isA, e, 0.0), axis=-1, keepdims=True)
            lB = jnp.sum(jnp.where(isA, 0.0, e), axis=-1, keepdims=True)
            l = jnp.where(isA, lA, lB)
            r = pl.reciprocal(l, approx=True)
            r = r * (2.0 - l * r)
            st['p', p] = e * r

        def f_pv(p):
            st['o', p] = _dot(st['p', p], st['v', p])

        def f_o(p):
            c = _dot(st['o', p], _wload(wo, 5, p * PW, PW))
            st['acc'] = c if 'acc' not in st else st['acc'] + c

        def f_fin(_):
            acc = st['acc']
            xbuf[pl.ds(rA, SEG), :] = xbuf[pl.ds(rA, SEG), :] + acc[MEM:, :]
            st['mem'] = acc[0:MEM, :]

        def f_b1(_):
            x1 = xbuf[pl.ds(rB1, SEG), :]
            y = _ln(x1)
            ybuf[pl.ds(rB1, SEG), :] = y
            hbuf[pl.ds(rB1 + 8, SEG), :] = _gelu(_dot(_ln(y), _wload(w1, 5)))

        def f_b2a(_):
            def sh(j, d):
                win = hbuf[pl.ds(rB2, SEG + 16), j * 128:(j + 1) * 128]
                return win[8 + d:8 + d + SEG, :]
            cols = [
                sh(0, -1),
                jnp.where(lane_h < 32, sh(1, -1), sh(1, 1)),
                jnp.where(lane_h < 64, sh(2, 1), sh(2, -2)),
                jnp.where(lane_h < 96, sh(3, -2), sh(3, 2)),
                sh(4, 2),
            ]
            hs_in = jnp.concatenate(cols, axis=1)
            st['y1'] = ybuf[pl.ds(rB2, SEG), :] + _dot(hs_in, _wload(w2, 5))

        def f_b2b(_):
            st['g'] = _gelu(_dot(_ln(st['y1']), _wload(w3, 12)))

        def f_b2c(i):
            kc = FF // NB2C
            c = _dot(st['g'][:, i * kc:(i + 1) * kc], _wload(w4, 5, i * kc, kc))
            st['h2'] = c if 'h2' not in st else st['h2'] + c

        def f_b2d(_):
            xn = xbuf[pl.ds(rB2, SEG), :] + (st['y1'] + st['h2'])
            xbuf[pl.ds(rB2, SEG), :] = xn
            ybuf[pl.ds(rB2, SEG), :] = _ln(xn)
            obuf[pl.ds(rB2, SEG), :] = xn.astype(BF16)

        fs = {'q': f_qkv, 's': f_s, 'v': f_pv, 'o': f_o, 'fin': f_fin, 'b1': f_b1, 'b2a': f_b2a, 'b2b': f_b2b,
              'b2c': f_b2c, 'b2d': f_b2d, 'wq': f_wq, 'wo': f_wo, 'bw': f_bw,
              'ln0': ln0, 'pre': f_pre}
        for op, p in sched:
            fs[op](p)
        return st.get('mem'), st.get('ypre')

    with _scope("step0"):
        mem, _ = run(SCHED_0, rA=0, mem=mem0[...].astype(F32))
    with _scope("step1"):
        mem, _ = run(SCHED_1, rA=SEG, mem=mem, rB1=0)
        run([('bw', 2), ('bw', 3)])

    def seg_row(t):
        return pl.multiple_of((t & (NSEG - 1)) * SEG, SEG)

    def body(u, mem):
        t0 = UNROLL * u + 2
        y = None
        for k in range(UNROLL):
            t = t0 + k
            mem = jnp.where(t == NSEG, mem0[...].astype(F32), mem)
            last = k == UNROLL - 1
            mem, y = run(SCHED_B if last else SCHED_A, rA=seg_row(t), mem=mem, rB1=seg_row(t - 1), rB2=seg_row(t - 2),
                         y=y, rPre=None if last else seg_row(t + 1))
        for k in range(UNROLL):
            t = t0 + k

            @pl.when(t >= NSEG + 2)
            def _():
                r = seg_row(t - 2)
                pltpu.make_async_copy(obuf.at[pl.ds(r, SEG), :], out_hbm.at[pl.ds(r, SEG), :], sem_out.at[0]).start()
        return mem

    with _scope("main"):
        jax.lax.fori_loop(0, (2 * NSEG - 2) // UNROLL, body, mem)

    with _scope("epi"):
        r63 = (NSEG - 1) * SEG
        r62 = (NSEG - 2) * SEG
        run([('b1', 0)] + SCHED_E, rB1=r63, rB2=r62)
        run(SCHED_E, rB2=r63)
        pltpu.make_async_copy(obuf.at[pl.ds(r62, 2 * SEG), :], out_hbm.at[pl.ds(r62, 2 * SEG), :], sem_out.at[0]).start()
        pltpu.make_async_copy(obuf.at[pl.ds(0, S_TOT), :], out_hbm, sem_out.at[0]).wait()


@jax.jit
def pallas_interleave_layers__memory_aug_recurrent_mem_tr__mixer_s_mlp__prompt_kernel(A_x, A_mem0, A_Wq, A_Wk, A_Wv, A_Wo, A_seg_len, B_x, B_w1, B_w2, B_w3, B_w4):
    del A_seg_len, B_x
    x2 = A_x.reshape(S_TOT, DM)
    m2 = A_mem0.reshape(MEM, DM)
    wqT = A_Wq.transpose(1, 2, 0).reshape(HD, DM)
    wkT = A_Wk.transpose(1, 2, 0).reshape(HD, DM)
    wvT = A_Wv.transpose(1, 2, 0).reshape(HD, DM)
    wo2 = A_Wo.reshape(HD, DM)
    any_spec = pl.BlockSpec(memory_space=pl.ANY)
    out = pl.pallas_call(
        _kernel,
        out_shape=jax.ShapeDtypeStruct((S_TOT, DM), BF16),
        in_specs=[any_spec] * 10,
        out_specs=any_spec,
        scratch_shapes=[
            pltpu.VMEM((NP, 9, DM // 2, 128), U32),
            pltpu.VMEM((5, HD // 2, 128), U32),
            pltpu.VMEM((5, DM, 128), BF16),
            pltpu.VMEM((5, DM, 128), BF16),
            pltpu.VMEM((12, DM, 128), BF16),
            pltpu.VMEM((5, FF, 128), BF16),
            pltpu.VMEM((S_TOT + 64, DM), F32),
            pltpu.VMEM((S_TOT + 64, DM), F32),
            pltpu.VMEM((S_TOT + 64, DM), F32),
            pltpu.VMEM((S_TOT + 64, DM), BF16),
            pltpu.VMEM((NP, 4, PW, DM), BF16),
            pltpu.VMEM((S_TOT, DM), BF16),
            pltpu.VMEM((MEM, DM), BF16),
            pltpu.SemaphoreType.DMA((NP, 4)),
            pltpu.SemaphoreType.DMA((1,)),
            pltpu.SemaphoreType.DMA((S_TOT // XC,)),
            pltpu.SemaphoreType.DMA((4,)),
            pltpu.SemaphoreType.DMA((1,)),
        ],
        compiler_params=pltpu.CompilerParams(vmem_limit_bytes=116 * 1024 * 1024),
    )(x2, m2, wqT, wkT, wvT, wo2, B_w1, B_w2, B_w3, B_w4)
    return out.reshape(1, S_TOT, DM)
```

```python
import contextlib
import jax
import jax.numpy as jnp
import numpy as np
import jax.experimental.pallas as pl
import jax.experimental.pallas.tpu as pltpu

F32 = jnp.float32
BF16 = jnp.bfloat16
U32 = jnp.uint32

S_TOT = 2048
DM = 640
NH = 32
DH = 192
HD = NH * DH
MEM = 8
SEG = 32
NSEG = S_TOT // SEG
L = MEM + SEG
NP = NH // 2
PW = 2 * DH
QW = 3 * PW
FF = 1536
LOG2E = 1.4426950408889634
SCOPES = False
NB2C = 4
DMA_WINDOW = 7
NSLOT = 10

SH = 24
R0 = 280
TS = (R0 - SH) // (SEG - SH)
RING = 288
C0 = 72
XCH = [(0, 288), (288, 512)] + [(r, r + 256) for r in range(512, S_TOT, 256)]
XEARLY = {3: 1, 5: 2, 7: 3, 9: 4}


def _make_sched(lag_s=1, lag_v=2, lag_o=5):
    ops = []
    i = 0
    done_o = 0
    while done_o < NP:
        if i < NP:
            ops.append(('q', i))
        if 0 <= i - lag_s < NP:
            ops.append(('s', i - lag_s))
        if 0 <= i - lag_o < NP:
            ops.append(('o', i - lag_o))
            done_o += 1
        if 0 <= i - lag_v < NP:
            ops.append(('v', i - lag_v))
        i += 1
    ops.append(('fin', 0))
    return ops


def _place(ops, places):
    out = []
    pl_ = {a: l for a, l in places}
    for o in ops:
        out.append(o)
        for b in pl_.get(o, ()):
            out.append(b if isinstance(b, tuple) else (b, 0))
    return out


WO_LAG = 6


def _sched0():
    ops = [('wq', (0, 0)), ('wq', (0, 1)), ('wq', (0, 2))]
    for i in range(NP + WO_LAG + 1):
        q = i < NP
        nq = i + 1 < NP
        if q:
            ops.append(('q0', (i, 0)))
        if nq:
            ops.append(('wq', (i + 1, 0)))
        if 0 <= i - 1 < NP:
            ops.append(('s', i - 1))
        if q:
            ops.append(('q0', (i, 1)))
        if nq:
            ops.append(('wq', (i + 1, 1)))
        if 0 <= i - 2 < NP:
            ops.append(('v', i - 2))
        if q:
            ops.append(('q0', (i, 2)))
        if nq:
            ops.append(('wq', (i + 1, 2)))
        if 0 <= i - WO_LAG < NP:
            ops.append(('o', i - WO_LAG))
        if q:
            ops.append(('q0', (i, 3)))
        if 0 <= i + 1 - WO_LAG < NP:
            ops.append(('wo', i + 1 - WO_LAG))
        if i in XEARLY:
            ops.append(('ln0', XEARLY[i]))
    ops.append(('fin', 0))
    return ops


SCHED_0 = _sched0()
SCHED_1 = _place(_make_sched(), [(('q', 3), [('bw', 0)]), (('q', 5), ['b1']), (('q', 6), [('ln0', 5)]),
                                 (('q', 9), [('ln0', 6)]), (('q', 12), [('ln0', 7)]), (('q', 14), [('bw', 1)])])
SCHED_A = _place(_make_sched(lag_v=2, lag_o=4),
                 [(('q', 2), ['b1']), (('q', 4), ['b2a']), (('q', 9), ['b2b']),
                  (('q', 14), ['pre', ('b2c', 0), ('b2c', 1)]), (('o', 13), [('b2c', 2)]),
                  (('fin', 0), [('b2c', 3), 'b2d'])])
SCHED_B = _place(_make_sched(lag_v=2, lag_o=5),
                 [(('q', 2), ['b1']), (('q', 4), ['b2a']), (('q', 9), ['b2b']), (('q', 14), [('b2c', 0)]),
                  (('s', 14), [('b2c', 1)]), (('o', 11), [('b2c', 2)]), (('v', 15), [('b2c', 3), 'b2d'])])
SCHED_SA = SCHED_A
SCHED_SB = SCHED_B
SCHED_E = [('b2a', 0), ('b2b', 0)] + [('b2c', i) for i in range(NB2C)] + [('b2d', 0)]


def _ln(x, eps=1e-5):
    m = jnp.mean(x, axis=-1, keepdims=True)
    xc = x - m
    v = jnp.mean(xc * xc, axis=-1, keepdims=True)
    return xc * jax.lax.rsqrt(v + eps)


def _gelu(x):
    return jax.nn.gelu(x, approximate=True)


def _dot(a, b):
    return jnp.dot(a, b, preferred_element_type=F32)


def _dot_nt(a, b):
    return jax.lax.dot_general(a, b, (((1,), (1,)), ((), ())), preferred_element_type=F32)


def _scope(name):
    return jax.named_scope(name) if SCOPES else contextlib.nullcontext()


def _wload(ref, ntile, k0=0, kn=None):
    if kn is None:
        return jnp.concatenate([pltpu.bitcast(ref[c], BF16) for c in range(ntile)], axis=1)
    return jnp.concatenate([pltpu.bitcast(ref[c, pl.ds(k0 // 2, kn // 2), :], BF16) for c in range(ntile)], axis=1)


def _kernel(x_hbm, mem0_hbm, wq_hbm, wk_hbm, wv_hbm, wo_hbm, w1_hbm, w2_hbm, w3_hbm, w4_hbm,
            out_hbm,
            wqkv, wo, ring, w1b, w2b, w3b, w4b, xbuf, ybuf, hbuf, obuf, stage, xin, mem0,
            sem_stage, sem_misc, sem_x, sem_w, sem_out):
    w_hbm = (wq_hbm, wk_hbm, wv_hbm, wo_hbm)

    def cp_x(i):
        r0, r1 = XCH[i]
        return [pltpu.make_async_copy(x_hbm.at[pl.ds(r0, r1 - r0), :], xin.at[pl.ds(r0, r1 - r0), :], sem_x.at[i])]

    def cp_w(i, src_ref, dst_ref, ntile):
        return [pltpu.make_async_copy(src_ref.at[:, pl.ds(c * 128, 128)], dst_ref.at[c], sem_w.at[i])
                for c in range(ntile)]

    cps = {'m': [pltpu.make_async_copy(mem0_hbm, mem0, sem_misc.at[0])], ('x', 0): cp_x(0)}
    slot_of = {}
    for p in range(NP + WO_LAG):
        for j in ((0, 1, 2) if p < NP else ()) + ((3,) if p >= WO_LAG else ()):
            pp = p - WO_LAG if j == 3 else p
            slot_of[pp, j] = len(slot_of) % NSLOT
            cps[pp, j] = [pltpu.make_async_copy(w_hbm[j].at[pl.ds(pp * PW, PW), :], stage.at[slot_of[pp, j]],
                                                sem_stage.at[pp, j])]
        if p - 1 in XEARLY:
            cps['x', XEARLY[p - 1]] = cp_x(XEARLY[p - 1])
    cps['w', 0] = cp_w(0, w1_hbm, w1b, 5)
    for i in range(5, len(XCH)):
        cps['x', i] = cp_x(i)
    cps['w', 1] = cp_w(1, w2_hbm, w2b, 5)
    cps['w', 2] = cp_w(2, w3_hbm, w3b, 12)
    cps['w', 3] = cp_w(3, w4_hbm, w4b, 5)
    queue = list(cps)
    issued = [0]

    def start_next():
        if issued[0] < len(queue):
            for c in cps[queue[issued[0]]]:
                c.start()
            issued[0] += 1

    def arrive(key):
        for c in cps[key]:
            c.wait()
        start_next()

    for _ in range(DMA_WINDOW):
        start_next()
    w1, w2, w3, w4 = (r.bitcast(U32) for r in (w1b, w2b, w3b, w4b))

    z8 = jnp.zeros((8, DM), F32)
    hbuf[pl.ds(0, 8), :] = z8
    hbuf[pl.ds(8 + S_TOT, 8), :] = z8
    arrive('m')

    def ln0(i):
        arrive(('x', i))
        for r in range(XCH[i][0], XCH[i][1], SEG):
            xv = xin[pl.ds(r, SEG), :].astype(F32)
            xbuf[pl.ds(r, SEG), :] = xv
            ybuf[pl.ds(r, SEG), :] = _ln(xv)
    ln0(0)

    row = jax.lax.broadcasted_iota(jnp.int32, (L, 128), 0)
    lane = jax.lax.broadcasted_iota(jnp.int32, (L, 128), 1)
    NEG = np.float32(-1e30)
    MASKED = np.float32(-1e9 * LOG2E)
    realA = lane < L
    realB = (lane >= 64) & (lane < 64 + L)
    validA = realA & ((row < MEM) | (row >= lane))
    validB = realB & ((row < MEM) | (row >= lane - 64))
    valid = validA | validB
    fill = jnp.where(realA | realB, MASKED, NEG)
    isA = lane < 64
    SC = np.float32(DH ** -0.5 * LOG2E)
    lane48 = jax.lax.broadcasted_iota(jnp.int32, (48, 128), 1)
    lo48 = lane48 < 64
    lane_h = jax.lax.broadcasted_iota(jnp.int32, (SEG, 128), 1)

    def blk(t):
        tb = jnp.concatenate([t, jnp.zeros((8, PW), F32)], axis=0).astype(BF16)
        t0 = tb[:, 0:128]
        t1 = tb[:, 128:256]
        t2 = tb[:, 256:384]
        z16 = jnp.zeros((16, 128), BF16)
        z64 = jnp.zeros((64, 128), BF16)
        z80 = jnp.zeros((80, 128), BF16)
        zb = jnp.zeros((48, 128), BF16)
        c0 = jnp.concatenate([t0, z80], axis=0)
        c1 = jnp.concatenate([jnp.where(lo48, t1, zb), z16, jnp.where(lo48, zb, t1), z16], axis=0)
        c2 = jnp.concatenate([z64, t2, z16], axis=0)
        return jnp.concatenate([c0, c1, c2], axis=1)

    def run(sched, rA=None, mem=None, rB1=None, rB2=None, y=None, yPre=None, short=None):
        st = {}
        if rA is not None and sched is not SCHED_0:
            yv = ybuf[pl.ds(y[0], y[1]), :] if isinstance(y, tuple) else y
            st['h'] = jnp.concatenate([mem, yv], axis=0)

        def f_pre(_):
            st['ypre'] = ybuf[pl.ds(yPre[0], yPre[1]), :]

        def f_wq(pj):
            p, j = pj
            arrive((p, j))
            wt = stage[slot_of[p, j]].T
            for c in range(3):
                wqkv[p, 3 * j + c] = pltpu.bitcast(wt[:, c * 128:(c + 1) * 128], U32)

        def f_wo(p):
            arrive((p, 3))
            for c in range(5):
                wo[c, pl.ds(p * (PW // 2), PW // 2), :] = pltpu.bitcast(
                    stage[slot_of[p, 3], :, c * 128:(c + 1) * 128], U32)

        def f_bw(i):
            arrive(('w', i))

        def split_qkv(p, qkv):
            st['q', p] = qkv[:, 0:PW]
            st['k', p] = blk(qkv[:, PW:2 * PW])
            st['v', p] = blk(qkv[:, 2 * PW:3 * PW])

        def f_qkv0(pc):
            p, c = pc
            if c == 0:
                lhs = jnp.concatenate([mem, ybuf[pl.ds(0, C0 - MEM), :]], axis=0)
            else:
                lhs = ybuf[pl.ds(c * C0 - MEM, C0), :]
            res = _dot(lhs, _wload(wqkv.at[p], 9))
            if c == 0:
                split_qkv(p, res[0:L])
                ring[pl.ds(SEG, C0 - L), p * QW:(p + 1) * QW] = res[L:]
            else:
                ring[pl.ds(c * C0 - MEM, C0), p * QW:(p + 1) * QW] = res

        def f_qkv(p):
            res = _dot(st['h'], _wload(wqkv.at[p], 9))
            if short is not None:
                groups, rseg = short
                for g in range(SH // 8):
                    ring[pl.ds(groups[g], 8), p * QW:(p + 1) * QW] = res[MEM + 8 * g:MEM + 8 * g + 8]
                res = jnp.concatenate([res[0:MEM], ring[pl.ds(rseg, SEG), p * QW:(p + 1) * QW]], axis=0)
            split_qkv(p, res)

        def f_s(p):
            t = _dot_nt(st['q', p], st['k', p]) * SC
            s = jnp.where(valid, t, fill)
            mA = jnp.max(jnp.where(isA, s, NEG), axis=-1, keepdims=True)
            mB = jnp.max(jnp.where(isA, NEG, s), axis=-1, keepdims=True)
            e = jnp.exp2(s - jnp.where(isA, mA, mB))
            lA = jnp.sum(jnp.where(isA, e, 0.0), axis=-1, keepdims=True)
            lB = jnp.sum(jnp.where(isA, 0.0, e), axis=-1, keepdims=True)
            l = jnp.where(isA, lA, lB)
            r = pl.reciprocal(l, approx=True)
            r = r * (2.0 - l * r)
            st['p', p] = e * r

        def f_pv(p):
            st['o', p] = _dot(st['p', p], st['v', p])

        def f_o(p):
            c = _dot(st['o', p], _wload(wo, 5, p * PW, PW))
            st['acc'] = c if 'acc' not in st else st['acc'] + c

        def f_fin(_):
            acc = st['acc']
            xbuf[pl.ds(rA, SEG), :] = xbuf[pl.ds(rA, SEG), :] + acc[MEM:, :]
            st['mem'] = acc[0:MEM, :]

        def f_b1(_):
            x1 = xbuf[pl.ds(rB1, SEG), :]
            y = _ln(x1)
            ybuf[pl.ds(rB1, SEG), :] = y
            hbuf[pl.ds(rB1 + 8, SEG), :] = _gelu(_dot(_ln(y), _wload(w1, 5)))

        def f_b2a(_):
            def sh(j, d):
                win = hbuf[pl.ds(rB2, SEG + 16), j * 128:(j + 1) * 128]
                return win[8 + d:8 + d + SEG, :]
            cols = [
                sh(0, -1),
                jnp.where(lane_h < 32, sh(1, -1), sh(1, 1)),
                jnp.where(lane_h < 64, sh(2, 1), sh(2, -2)),
                jnp.where(lane_h < 96, sh(3, -2), sh(3, 2)),
                sh(4, 2),
            ]
            hs_in = jnp.concatenate(cols, axis=1)
            st['y1'] = ybuf[pl.ds(rB2, SEG), :] + _dot(hs_in, _wload(w2, 5))

        def f_b2b(_):
            st['g'] = _gelu(_dot(_ln(st['y1']), _wload(w3, 12)))

        def f_b2c(i):
            kc = FF // NB2C
            c = _dot(st['g'][:, i * kc:(i + 1) * kc], _wload(w4, 5, i * kc, kc))
            st['h2'] = c if 'h2' not in st else st['h2'] + c

        def f_b2d(_):
            xn = xbuf[pl.ds(rB2, SEG), :] + (st['y1'] + st['h2'])
            xbuf[pl.ds(rB2, SEG), :] = xn
            ybuf[pl.ds(rB2, SEG), :] = _ln(xn)
            obuf[pl.ds(rB2, SEG), :] = xn.astype(BF16)

        fs = {'q': f_qkv, 'q0': f_qkv0, 's': f_s, 'v': f_pv, 'o': f_o, 'fin': f_fin, 'b1': f_b1, 'b2a': f_b2a,
              'b2b': f_b2b, 'b2c': f_b2c, 'b2d': f_b2d, 'wq': f_wq, 'wo': f_wo, 'bw': f_bw, 'ln0': ln0,
              'pre': f_pre}
        for op, p in sched:
            fs[op](p)
        return st.get('mem'), st.get('ypre')

    def seg_row(t):
        return pl.multiple_of((t & (NSEG - 1)) * SEG, SEG)

    def new_rows(t):
        return R0 + SH * (t - 1)

    with _scope("step0"):
        mem, _ = run(SCHED_0, rA=0, mem=mem0[...].astype(F32))
    with _scope("step1"):
        mem, _ = run(SCHED_1, rA=SEG, mem=mem, rB1=0, y=(new_rows(1), SH),
                     short=([(new_rows(1) + 8 * g) % RING for g in range(SH // 8)], SEG))
        run([('bw', 2), ('bw', 3)])

    def short_body(u, mem):
        t0 = 2 * u + 2
        y = (pl.multiple_of(new_rows(t0), 8), SH)
        for k in range(2):
            t = t0 + k
            groups = [pl.multiple_of(jax.lax.rem(new_rows(t) + 8 * g, RING), 8) for g in range(SH // 8)]
            rseg = pl.multiple_of(jax.lax.rem(t * SEG, RING), SEG)
            mem, y = run(SCHED_SB if k else SCHED_SA, rA=seg_row(t), mem=mem, rB1=seg_row(t - 1), rB2=seg_row(t - 2),
                         y=y, yPre=None if k else (pl.multiple_of(new_rows(t + 1), 8), SH), short=(groups, rseg))
        return mem

    with _scope("short"):
        mem = jax.lax.fori_loop(0, (TS - 2) // 2, short_body, mem)

    def body(u, mem):
        t0 = 2 * u + TS
        y = (seg_row(t0), SEG)
        mem = jnp.where(t0 == NSEG, mem0[...].astype(F32), mem)
        for k in range(2):
            t = t0 + k
            mem, y = run(SCHED_B if k else SCHED_A, rA=seg_row(t), mem=mem, rB1=seg_row(t - 1), rB2=seg_row(t - 2),
                         y=y, yPre=None if k else (seg_row(t + 1), SEG))

        @pl.when(t0 >= NSEG + 2)
        def _():
            r = pl.multiple_of((t0 - NSEG - 2) * SEG, 2 * SEG)
            pltpu.make_async_copy(obuf.at[pl.ds(r, 2 * SEG), :], out_hbm.at[pl.ds(r, 2 * SEG), :], sem_out.at[0]).start()
        return mem

    with _scope("main"):
        jax.lax.fori_loop(0, (2 * NSEG - TS) // 2, body, mem)

    with _scope("epi"):
        r63 = (NSEG - 1) * SEG
        r62 = (NSEG - 2) * SEG
        run([('b1', 0)] + SCHED_E, rB1=r63, rB2=r62)
        run(SCHED_E, rB2=r63)
        pltpu.make_async_copy(obuf.at[pl.ds(r62, 2 * SEG), :], out_hbm.at[pl.ds(r62, 2 * SEG), :], sem_out.at[0]).start()
        pltpu.make_async_copy(obuf.at[pl.ds(0, S_TOT), :], out_hbm, sem_out.at[0]).wait()


@jax.jit
def pallas_interleave_layers__memory_aug_recurrent_mem_tr__mixer_s_mlp__prompt_kernel(A_x, A_mem0, A_Wq, A_Wk, A_Wv, A_Wo, A_seg_len, B_x, B_w1, B_w2, B_w3, B_w4):
    del A_seg_len, B_x
    x2 = A_x.reshape(S_TOT, DM)
    m2 = A_mem0.reshape(MEM, DM)
    wqT = A_Wq.transpose(1, 2, 0).reshape(HD, DM)
    wkT = A_Wk.transpose(1, 2, 0).reshape(HD, DM)
    wvT = A_Wv.transpose(1, 2, 0).reshape(HD, DM)
    wo2 = A_Wo.reshape(HD, DM)
    any_spec = pl.BlockSpec(memory_space=pl.ANY)
    out = pl.pallas_call(
        _kernel,
        out_shape=jax.ShapeDtypeStruct((S_TOT, DM), BF16),
        in_specs=[any_spec] * 10,
        out_specs=any_spec,
        scratch_shapes=[
            pltpu.VMEM((NP, 9, DM // 2, 128), U32),
            pltpu.VMEM((5, HD // 2, 128), U32),
            pltpu.VMEM((RING, NP * QW), F32),
            pltpu.VMEM((5, DM, 128), BF16),
            pltpu.VMEM((5, DM, 128), BF16),
            pltpu.VMEM((12, DM, 128), BF16),
            pltpu.VMEM((5, FF, 128), BF16),
            pltpu.VMEM((S_TOT + 64, DM), F32),
            pltpu.VMEM((S_TOT + 64, DM), F32),
            pltpu.VMEM((S_TOT + 64, DM), F32),
            pltpu.VMEM((S_TOT + 64, DM), BF16),
            pltpu.VMEM((NSLOT, PW, DM), BF16),
            pltpu.VMEM((S_TOT, DM), BF16),
            pltpu.VMEM((MEM, DM), BF16),
            pltpu.SemaphoreType.DMA((NP, 4)),
            pltpu.SemaphoreType.DMA((1,)),
            pltpu.SemaphoreType.DMA((len(XCH),)),
            pltpu.SemaphoreType.DMA((4,)),
            pltpu.SemaphoreType.DMA((1,)),
        ],
        compiler_params=pltpu.CompilerParams(vmem_limit_bytes=116 * 1024 * 1024),
    )(x2, m2, wqT, wkT, wvT, wo2, B_w1, B_w2, B_w3, B_w4)
    return out.reshape(1, S_TOT, DM)
```

```python
import contextlib
import jax
import jax.numpy as jnp
import numpy as np
import jax.experimental.pallas as pl
import jax.experimental.pallas.tpu as pltpu

F32 = jnp.float32
BF16 = jnp.bfloat16
U32 = jnp.uint32

S_TOT = 2048
DM = 640
NH = 32
DH = 192
HD = NH * DH
MEM = 8
SEG = 32
NSEG = S_TOT // SEG
L = MEM + SEG
NP = NH // 2
PW = 2 * DH
QW = 3 * PW
FF = 1536
LOG2E = 1.4426950408889634
SCOPES = False
NB2C = 4

SH = 24
R0 = 344
TS = (R0 - SH) // (SEG - SH)
RING = (R0 + 31) // 32 * 32
C0 = (R0 + MEM) // 4
XCH = [(0, RING), (RING, 512)] + [(r, r + 256) for r in range(512, S_TOT, 256)]
NSEM = 64
DMA_DEPTH = 3
GROUPS = [((0, 1), None, ()), ((1, 2), None, ()), ((2, 3), None, ()), ((3, 4), None, (1,)), ((4, 6), None, ()),
          ((6, 8), None, (2,)), ((8, 10), None, (3,)), ((10, 12), None, (4,)), ((12, 14), None, ()),
          ((14, 16), None, ()), (None, (0, 4), ()), (None, (4, 8), ()), (None, (8, 12), ()), (None, (12, 16), ())]
O_SLOTS = {10: (14, 7), 11: (15, 4)}


def _make_sched(lag_s=1, lag_v=2, lag_o=5):
    ops = []
    i = 0
    done_o = 0
    while done_o < NP:
        if i < NP:
            ops.append(('q', i))
        if 0 <= i - lag_s < NP:
            ops.append(('s', i - lag_s))
        if 0 <= i - lag_o < NP:
            ops.append(('o', i - lag_o))
            done_o += 1
        if 0 <= i - lag_v < NP:
            ops.append(('v', i - lag_v))
        i += 1
    ops.append(('fin', 0))
    return ops


def _place(ops, places):
    out = []
    pl_ = {a: l for a, l in places}
    for o in ops:
        out.append(o)
        for b in pl_.get(o, ()):
            out.append(b if isinstance(b, tuple) else (b, 0))
    return out


def _sched0():
    first = {q[0]: g for g, (q, _, _) in enumerate(GROUPS) if q}
    ops = [('wq', 0)] + [('tr', (0, j, c)) for j in range(3) for c in range(3)]
    todo_x = []
    o_at = {}
    for g, (i, k) in O_SLOTS.items():
        o_at[i, k] = [('wq', g)]
        for n, p in enumerate(range(*GROUPS[g][1])):
            o_at.setdefault((i, k + n), []).append(('o', p))
    for i in range(NP + 2):
        mm = [('q0', (i, c, j)) for c in range(4) for j in range(3)] if i < NP else []
        side = {k: [] for k in range(12)}
        if i + 1 < NP:
            if i + 1 in first:
                g = first[i + 1]
                side[0] += [('wq', g)]
                todo_x += list(GROUPS[g][2])
            for k in range(9):
                side[k] += [('tr', (i + 1, k // 3, k % 3))]
        if 0 <= i - 1 < NP:
            side[2] += [('s', i - 1)]
        if 0 <= i - 2 < NP:
            side[5] += [('v', i - 2)]
        if todo_x:
            side[9] += [('ln0', todo_x.pop(0))]
        for k in range(12):
            if mm:
                ops.append(mm[k])
            ops += side[k] + o_at.get((i, k), [])
    for g, (q, wo_, _) in enumerate(GROUPS):
        if not q and g not in O_SLOTS:
            ops += [('wq', g)] + [('o', p) for p in range(*wo_)]
    ops.append(('fin', 0))
    return ops


SCHED_0 = _sched0()
SCHED_1 = _place(_make_sched(), [(('q', 4), [('bw', 0)]), (('q', 5), ['b1']), (('q', 6), [('ln0', 5)]),
                                 (('q', 9), [('ln0', 6)]), (('q', 12), [('ln0', 7)]), (('q', 14), [('bw', 1)])])
SCHED_A = _place(_make_sched(lag_v=2, lag_o=4),
                 [(('q', 2), ['b1']), (('q', 4), ['b2a']), (('q', 9), ['b2b']),
                  (('q', 14), ['pre', ('b2c', 0), ('b2c', 1)]), (('o', 13), [('b2c', 2)]),
                  (('fin', 0), [('b2c', 3), 'b2d'])])
SCHED_B = _place(_make_sched(lag_v=2, lag_o=5),
                 [(('q', 2), ['b1']), (('q', 4), ['b2a']), (('q', 9), ['b2b']), (('q', 14), [('b2c', 0)]),
                  (('s', 14), [('b2c', 1)]), (('o', 11), [('b2c', 2)]), (('v', 15), [('b2c', 3), 'b2d'])])
SCHED_SA = SCHED_A
SCHED_SB = SCHED_B
SCHED_E = [('b2a', 0), ('b2b', 0)] + [('b2c', i) for i in range(NB2C)] + [('b2d', 0)]


def _ln(x, eps=1e-5):
    m = jnp.mean(x, axis=-1, keepdims=True)
    xc = x - m
    v = jnp.mean(xc * xc, axis=-1, keepdims=True)
    return xc * jax.lax.rsqrt(v + eps)


def _gelu(x):
    return jax.nn.gelu(x, approximate=True)


def _dot(a, b):
    return jnp.dot(a, b, preferred_element_type=F32)


def _dot_nt(a, b):
    return jax.lax.dot_general(a, b, (((1,), (1,)), ((), ())), preferred_element_type=F32)


def _scope(name):
    return jax.named_scope(name) if SCOPES else contextlib.nullcontext()


def _wload(ref, ntile, k0=0, kn=None):
    if kn is None:
        return jnp.concatenate([pltpu.bitcast(ref[c], BF16) for c in range(ntile)], axis=1)
    return jnp.concatenate([pltpu.bitcast(ref[c, pl.ds(k0 // 2, kn // 2), :], BF16) for c in range(ntile)], axis=1)


def _kernel(x_hbm, mem0_hbm, wq_hbm, wk_hbm, wv_hbm, wo_hbm, w1_hbm, w2_hbm, w3_hbm, w4_hbm,
            out_hbm,
            wqkv, wob, ring, w1b, w2b, w3b, w4b, xbuf, ybuf, hbuf, obuf, stage, xin, mem0,
            sem_in, sem_out):
    w_hbm = (wq_hbm, wk_hbm, wv_hbm, wo_hbm)
    nsem = [0]

    def new_sem():
        nsem[0] += 1
        return sem_in.at[nsem[0] - 1]

    def cp_x(i):
        r0, r1 = XCH[i]
        return [pltpu.make_async_copy(x_hbm.at[pl.ds(r0, r1 - r0), :], xin.at[pl.ds(r0, r1 - r0), :], new_sem())]

    def cp_w(src_ref, dst_ref, ntile):
        sem = new_sem()
        return [pltpu.make_async_copy(src_ref.at[:, pl.ds(c * 128, 128)], dst_ref.at[c], sem) for c in range(ntile)]

    def cp_rows(j, p0, p1):
        rows = pl.ds(p0 * PW, (p1 - p0) * PW)
        sem = new_sem()
        if j < 3:
            return [pltpu.make_async_copy(w_hbm[j].at[rows, :], stage.at[j, rows, :], sem)]
        return [pltpu.make_async_copy(w_hbm[j].at[rows, pl.ds(c * 128, 128)], wob.at[c, rows, :], sem)
                for c in range(5)]

    cps = {'m': [pltpu.make_async_copy(mem0_hbm, mem0, new_sem())] + cp_x(0)}
    for g, (qkv, wo_, xc) in enumerate(GROUPS):
        cps['g', g] = []
        if qkv:
            cps['g', g] += [c for j in range(3) for c in cp_rows(j, *qkv)]
        if wo_:
            cps['g', g] += cp_rows(3, *wo_)
        for i in xc:
            cps['g', g] += cp_x(i)
    cps['w', 0] = cp_w(w1_hbm, w1b, 5) + [c for i in range(5, len(XCH)) for c in cp_x(i)]
    cps['w', 1] = cp_w(w2_hbm, w2b, 5)
    cps['w', 2] = cp_w(w3_hbm, w3b, 12)
    cps['w', 3] = cp_w(w4_hbm, w4b, 5)
    assert nsem[0] <= NSEM
    queue = list(cps)
    pos = {'started': 0, 'done': 0}

    def top_up(limit=DMA_DEPTH):
        while pos['started'] < min(len(queue), pos['done'] + limit):
            for c in cps[queue[pos['started']]]:
                c.start()
            pos['started'] += 1

    def arrive(key):
        assert key == queue[pos['done']]
        for c in cps[key]:
            c.wait()
        pos['done'] += 1
        top_up()

    top_up(2)
    wo, w1, w2, w3, w4 = (r.bitcast(U32) for r in (wob, w1b, w2b, w3b, w4b))

    z8 = jnp.zeros((8, DM), F32)
    hbuf[pl.ds(0, 8), :] = z8
    hbuf[pl.ds(8 + S_TOT, 8), :] = z8
    arrive('m')

    def ln0(i):
        for r in range(XCH[i][0], XCH[i][1], SEG):
            xv = xin[pl.ds(r, SEG), :].astype(F32)
            xbuf[pl.ds(r, SEG), :] = xv
            ybuf[pl.ds(r, SEG), :] = _ln(xv)
    ln0(0)

    row = jax.lax.broadcasted_iota(jnp.int32, (L, 128), 0)
    lane = jax.lax.broadcasted_iota(jnp.int32, (L, 128), 1)
    NEG = np.float32(-1e30)
    MASKED = np.float32(-1e9 * LOG2E)
    realA = lane < L
    realB = (lane >= 64) & (lane < 64 + L)
    validA = realA & ((row < MEM) | (row >= lane))
    validB = realB & ((row < MEM) | (row >= lane - 64))
    valid = validA | validB
    fill = jnp.where(realA | realB, MASKED, NEG)
    isA = lane < 64
    SC = np.float32(DH ** -0.5 * LOG2E)
    lane48 = jax.lax.broadcasted_iota(jnp.int32, (48, 128), 1)
    lo48 = lane48 < 64
    lane_h = jax.lax.broadcasted_iota(jnp.int32, (SEG, 128), 1)

    def blk(t):
        tb = jnp.concatenate([t, jnp.zeros((8, PW), F32)], axis=0).astype(BF16)
        t0 = tb[:, 0:128]
        t1 = tb[:, 128:256]
        t2 = tb[:, 256:384]
        z16 = jnp.zeros((16, 128), BF16)
        z64 = jnp.zeros((64, 128), BF16)
        z80 = jnp.zeros((80, 128), BF16)
        zb = jnp.zeros((48, 128), BF16)
        c0 = jnp.concatenate([t0, z80], axis=0)
        c1 = jnp.concatenate([jnp.where(lo48, t1, zb), z16, jnp.where(lo48, zb, t1), z16], axis=0)
        c2 = jnp.concatenate([z64, t2, z16], axis=0)
        return jnp.concatenate([c0, c1, c2], axis=1)

    def run(sched, rA=None, mem=None, rB1=None, rB2=None, y=None, yPre=None, short=None):
        st = {}
        if rA is not None and sched is not SCHED_0:
            yv = ybuf[pl.ds(y[0], y[1]), :] if isinstance(y, tuple) else y
            st['h'] = jnp.concatenate([mem, yv], axis=0)

        def f_pre(_):
            st['ypre'] = ybuf[pl.ds(yPre[0], yPre[1]), :]

        def f_wq(g):
            arrive(('g', g))

        def f_tr(pjc):
            p, j, c = pjc
            for m in range(5):
                blk_ = stage[j, pl.ds(p * PW + c * 128, 128), pl.ds(m * 128, 128)]
                wqkv[p, 3 * j + c, pl.ds(m * 64, 64), :] = pltpu.bitcast(blk_.T, U32)

        def f_bw(i):
            arrive(('w', i))

        def split_qkv(p, qkv):
            st['q', p] = qkv[:, 0:PW]
            st['k', p] = blk(qkv[:, PW:2 * PW])
            st['v', p] = blk(qkv[:, 2 * PW:3 * PW])

        def f_qkv0(pcj):
            p, c, j = pcj
            if c == 0:
                lhs = jnp.concatenate([mem, ybuf[pl.ds(0, C0 - MEM), :]], axis=0)
            else:
                lhs = ybuf[pl.ds(c * C0 - MEM, C0), :]
            res = _dot(lhs, _wload(wqkv.at[p, pl.ds(3 * j, 3)], 3))
            col = p * QW + j * PW
            if c == 0:
                st['qkv'[j], p] = res[0:L] if j == 0 else blk(res[0:L])
                ring[pl.ds(SEG, C0 - L), col:col + PW] = res[L:]
            else:
                ring[pl.ds(c * C0 - MEM, C0), col:col + PW] = res

        def f_qkv(p):
            res = _dot(st['h'], _wload(wqkv.at[p], 9))
            if short is not None:
                groups, rseg = short
                for g in range(SH // 8):
                    ring[pl.ds(groups[g], 8), p * QW:(p + 1) * QW] = res[MEM + 8 * g:MEM + 8 * g + 8]
                res = jnp.concatenate([res[0:MEM], ring[pl.ds(rseg, SEG), p * QW:(p + 1) * QW]], axis=0)
            split_qkv(p, res)

        def f_s(p):
            t = _dot_nt(st['q', p], st['k', p]) * SC
            s = jnp.where(valid, t, fill)
            mA = jnp.max(jnp.where(isA, s, NEG), axis=-1, keepdims=True)
            mB = jnp.max(jnp.where(isA, NEG, s), axis=-1, keepdims=True)
            e = jnp.exp2(s - jnp.where(isA, mA, mB))
            lA = jnp.sum(jnp.where(isA, e, 0.0), axis=-1, keepdims=True)
            lB = jnp.sum(jnp.where(isA, 0.0, e), axis=-1, keepdims=True)
            l = jnp.where(isA, lA, lB)
            r = pl.reciprocal(l, approx=True)
            r = r * (2.0 - l * r)
            st['p', p] = e * r

        def f_pv(p):
            st['o', p] = _dot(st['p', p], st['v', p])

        def f_o(p):
            c = _dot(st['o', p], _wload(wo, 5, p * PW, PW))
            st['acc'] = c if 'acc' not in st else st['acc'] + c

        def f_fin(_):
            acc = st['acc']
            xbuf[pl.ds(rA, SEG), :] = xbuf[pl.ds(rA, SEG), :] + acc[MEM:, :]
            st['mem'] = acc[0:MEM, :]

        def f_b1(_):
            x1 = xbuf[pl.ds(rB1, SEG), :]
            y = _ln(x1)
            ybuf[pl.ds(rB1, SEG), :] = y
            hbuf[pl.ds(rB1 + 8, SEG), :] = _gelu(_dot(_ln(y), _wload(w1, 5)))

        def f_b2a(_):
            def sh(j, d):
                win = hbuf[pl.ds(rB2, SEG + 16), j * 128:(j + 1) * 128]
                return win[8 + d:8 + d + SEG, :]
            cols = [
                sh(0, -1),
                jnp.where(lane_h < 32, sh(1, -1), sh(1, 1)),
                jnp.where(lane_h < 64, sh(2, 1), sh(2, -2)),
                jnp.where(lane_h < 96, sh(3, -2), sh(3, 2)),
                sh(4, 2),
            ]
            hs_in = jnp.concatenate(cols, axis=1)
            st['y1'] = ybuf[pl.ds(rB2, SEG), :] + _dot(hs_in, _wload(w2, 5))

        def f_b2b(_):
            st['g'] = _gelu(_dot(_ln(st['y1']), _wload(w3, 12)))

        def f_b2c(i):
            kc = FF // NB2C
            c = _dot(st['g'][:, i * kc:(i + 1) * kc], _wload(w4, 5, i * kc, kc))
            st['h2'] = c if 'h2' not in st else st['h2'] + c

        def f_b2d(_):
            xn = xbuf[pl.ds(rB2, SEG), :] + (st['y1'] + st['h2'])
            xbuf[pl.ds(rB2, SEG), :] = xn
            ybuf[pl.ds(rB2, SEG), :] = _ln(xn)
            obuf[pl.ds(rB2, SEG), :] = xn.astype(BF16)

        fs = {'q': f_qkv, 'q0': f_qkv0, 's': f_s, 'v': f_pv, 'o': f_o, 'fin': f_fin, 'b1': f_b1, 'b2a': f_b2a,
              'b2b': f_b2b, 'b2c': f_b2c, 'b2d': f_b2d, 'wq': f_wq, 'tr': f_tr, 'bw': f_bw, 'ln0': ln0,
              'pre': f_pre}
        for op, p in sched:
            fs[op](p)
        return st.get('mem'), st.get('ypre')

    def seg_row(t):
        return pl.multiple_of((t & (NSEG - 1)) * SEG, SEG)

    def new_rows(t):
        return R0 + SH * (t - 1)

    with _scope("step0"):
        mem, _ = run(SCHED_0, rA=0, mem=mem0[...].astype(F32))
    with _scope("step1"):
        mem, _ = run(SCHED_1, rA=SEG, mem=mem, rB1=0, y=(new_rows(1), SH),
                     short=([(new_rows(1) + 8 * g) % RING for g in range(SH // 8)], SEG))
        run([('bw', 2), ('bw', 3)])

    def short_body(u, mem):
        t0 = 2 * u + 2
        y = (pl.multiple_of(new_rows(t0), 8), SH)
        for k in range(2):
            t = t0 + k
            groups = [pl.multiple_of(jax.lax.rem(new_rows(t) + 8 * g, RING), 8) for g in range(SH // 8)]
            rseg = pl.multiple_of(jax.lax.rem(t * SEG, RING), SEG)
            mem, y = run(SCHED_SB if k else SCHED_SA, rA=seg_row(t), mem=mem, rB1=seg_row(t - 1), rB2=seg_row(t - 2),
                         y=y, yPre=None if k else (pl.multiple_of(new_rows(t + 1), 8), SH), short=(groups, rseg))
        return mem

    with _scope("short"):
        mem = jax.lax.fori_loop(0, (TS - 2) // 2, short_body, mem)

    def body(u, mem):
        t0 = 2 * u + TS
        y = (seg_row(t0), SEG)
        mem = jnp.where(t0 == NSEG, mem0[...].astype(F32), mem)
        for k in range(2):
            t = t0 + k
            mem, y = run(SCHED_B if k else SCHED_A, rA=seg_row(t), mem=mem, rB1=seg_row(t - 1), rB2=seg_row(t - 2),
                         y=y, yPre=None if k else (seg_row(t + 1), SEG))

        @pl.when(t0 >= NSEG + 2)
        def _():
            r = pl.multiple_of((t0 - NSEG - 2) * SEG, 2 * SEG)
            pltpu.make_async_copy(obuf.at[pl.ds(r, 2 * SEG), :], out_hbm.at[pl.ds(r, 2 * SEG), :], sem_out.at[0]).start()
        return mem

    with _scope("main"):
        jax.lax.fori_loop(0, (2 * NSEG - TS) // 2, body, mem)

    with _scope("epi"):
        r63 = (NSEG - 1) * SEG
        r62 = (NSEG - 2) * SEG
        run([('b1', 0)] + SCHED_E, rB1=r63, rB2=r62)
        run(SCHED_E, rB2=r63)
        pltpu.make_async_copy(obuf.at[pl.ds(r62, 2 * SEG), :], out_hbm.at[pl.ds(r62, 2 * SEG), :], sem_out.at[0]).start()
        pltpu.make_async_copy(obuf.at[pl.ds(0, S_TOT), :], out_hbm, sem_out.at[0]).wait()


@jax.jit
def pallas_interleave_layers__memory_aug_recurrent_mem_tr__mixer_s_mlp__prompt_kernel(A_x, A_mem0, A_Wq, A_Wk, A_Wv, A_Wo, A_seg_len, B_x, B_w1, B_w2, B_w3, B_w4):
    del A_seg_len, B_x
    x2 = A_x.reshape(S_TOT, DM)
    m2 = A_mem0.reshape(MEM, DM)
    wqT = A_Wq.transpose(1, 2, 0).reshape(HD, DM)
    wkT = A_Wk.transpose(1, 2, 0).reshape(HD, DM)
    wvT = A_Wv.transpose(1, 2, 0).reshape(HD, DM)
    wo2 = A_Wo.reshape(HD, DM)
    any_spec = pl.BlockSpec(memory_space=pl.ANY)
    out = pl.pallas_call(
        _kernel,
        out_shape=jax.ShapeDtypeStruct((S_TOT, DM), BF16),
        in_specs=[any_spec] * 10,
        out_specs=any_spec,
        scratch_shapes=[
            pltpu.VMEM((NP, 9, DM // 2, 128), U32),
            pltpu.VMEM((5, HD, 128), BF16),
            pltpu.VMEM((RING, NP * QW), F32),
            pltpu.VMEM((5, DM, 128), BF16),
            pltpu.VMEM((5, DM, 128), BF16),
            pltpu.VMEM((12, DM, 128), BF16),
            pltpu.VMEM((5, FF, 128), BF16),
            pltpu.VMEM((S_TOT + 64, DM), F32),
            pltpu.VMEM((S_TOT + 64, DM), F32),
            pltpu.VMEM((S_TOT + 64, DM), F32),
            pltpu.VMEM((S_TOT + 64, DM), BF16),
            pltpu.VMEM((3, HD, DM), BF16),
            pltpu.VMEM((S_TOT, DM), BF16),
            pltpu.VMEM((MEM, DM), BF16),
            pltpu.SemaphoreType.DMA((NSEM,)),
            pltpu.SemaphoreType.DMA((1,)),
        ],
        compiler_params=pltpu.CompilerParams(vmem_limit_bytes=120 * 1024 * 1024),
    )(x2, m2, wqT, wkT, wvT, wo2, B_w1, B_w2, B_w3, B_w4)
    return out.reshape(1, S_TOT, DM)
```

```python
import contextlib
import jax
import jax.numpy as jnp
import numpy as np
import jax.experimental.pallas as pl
import jax.experimental.pallas.tpu as pltpu

F32 = jnp.float32
BF16 = jnp.bfloat16
U32 = jnp.uint32

S_TOT = 2048
DM = 640
NH = 32
DH = 192
HD = NH * DH
MEM = 8
SEG = 32
NSEG = S_TOT // SEG
L = MEM + SEG
NP = NH // 2
PW = 2 * DH
QW = 3 * PW
FF = 1536
LOG2E = 1.4426950408889634
SCOPES = False
NB2C = 4

SH = 24
R0 = 344
TS = (R0 - SH) // (SEG - SH)
RING = (R0 + 31) // 32 * 32
C0 = (R0 + MEM) // 4
XCH = [(0, RING), (RING, 512)] + [(r, r + 256) for r in range(512, S_TOT, 256)]
NSEM = 64
DMA_DEPTH = 3
GROUPS = [((0, 1), None, ()), ((1, 2), None, ()), ((2, 3), None, ()), ((3, 4), None, (1,)), ((4, 6), None, ()),
          ((6, 8), None, (2,)), ((8, 10), None, (3,)), ((10, 12), None, (4,)), ((12, 14), None, ()),
          ((14, 16), None, ()), (None, (0, 4), ()), (None, (4, 8), ()), (None, (8, 12), ()), (None, (12, 16), ())]
O_SLOTS = {10: (14, 7), 11: (15, 4)}


def _make_sched(lag_s=1, lag_v=2, lag_o=5):
    ops = []
    i = 0
    done_o = 0
    while done_o < NP:
        if i < NP:
            ops.append(('q', i))
        if 0 <= i - lag_s < NP:
            ops.append(('s', i - lag_s))
        if 0 <= i - lag_o < NP:
            ops.append(('o', i - lag_o))
            done_o += 1
        if 0 <= i - lag_v < NP:
            ops.append(('v', i - lag_v))
        i += 1
    ops.append(('fin', 0))
    return ops


def _place(ops, places):
    out = []
    pl_ = {a: l for a, l in places}
    for o in ops:
        out.append(o)
        for b in pl_.get(o, ()):
            out.append(b if isinstance(b, tuple) else (b, 0))
    return out


def _sched0():
    first = {q[0]: g for g, (q, _, _) in enumerate(GROUPS) if q}
    ops = [('wq', 0)] + [('tr', (0, j, c)) for j in range(3) for c in range(3)]
    todo_x = []
    o_at = {}
    for g, (i, k) in O_SLOTS.items():
        o_at[i, k] = [('wq', g)]
        for n, p in enumerate(range(*GROUPS[g][1])):
            o_at.setdefault((i, k + n), []).append(('o', p))
    for i in range(NP + 2):
        mm = [('q0', (i, c, j)) for c in range(4) for j in range(3)] if i < NP else []
        side = {k: [] for k in range(12)}
        if i + 1 < NP:
            if i + 1 in first:
                g = first[i + 1]
                side[0] += [('wq', g)]
                todo_x += list(GROUPS[g][2])
            for k in range(9):
                side[k] += [('tr', (i + 1, k // 3, k % 3))]
        if 0 <= i - 1 < NP:
            side[2] += [('s', i - 1)]
        if 0 <= i - 2 < NP:
            side[5] += [('v', i - 2)]
        if todo_x:
            side[9] += [('ln0', todo_x.pop(0))]
        for k in range(12):
            if mm:
                ops.append(mm[k])
            ops += side[k] + o_at.get((i, k), [])
    for g, (q, wo_, _) in enumerate(GROUPS):
        if not q and g not in O_SLOTS:
            ops += [('wq', g)] + [('o', p) for p in range(*wo_)]
    ops.append(('fin', 0))
    return ops


SCHED_0 = _sched0()
SCHED_1 = _place(_make_sched(), [(('q', 4), [('bw', 0)]), (('q', 5), ['b1']), (('q', 6), [('ln0', 5)]),
                                 (('q', 9), [('ln0', 6)]), (('q', 12), [('ln0', 7)]), (('q', 14), [('bw', 1)])])
SCHED_A = _place(_make_sched(lag_v=2, lag_o=4),
                 [(('q', 2), ['b1']), (('q', 4), ['b2a']), (('q', 9), ['b2b']),
                  (('q', 14), ['pre', ('b2c', 0), ('b2c', 1)]), (('o', 13), [('b2c', 2)]),
                  (('fin', 0), [('b2c', 3), 'b2d'])])
SCHED_B = _place(_make_sched(lag_v=2, lag_o=5),
                 [(('q', 2), ['b1']), (('q', 4), ['b2a']), (('q', 9), ['b2b']), (('q', 14), [('b2c', 0)]),
                  (('s', 14), [('b2c', 1)]), (('o', 11), [('b2c', 2)]), (('v', 15), [('b2c', 3), 'b2d'])])
SCHED_SA = _place(_make_sched(lag_v=2, lag_o=7),
                  [(('q', 2), ['b1']), (('q', 6), ['b2a']), (('q', 9), ['b2b']), (('s', 15), [('b2c', 0)]),
                   (('o', 9), [('b2c', 1)]), (('o', 14), ['pre', ('b2c', 2)]), (('fin', 0), [('b2c', 3), 'b2d'])])
SCHED_SB = _place(_make_sched(lag_v=2, lag_o=4),
                  [(('q', 2), ['b1']), (('q', 4), ['b2a']), (('q', 7), ['b2b']), (('q', 10), [('b2c', 0)]),
                   (('v', 13), [('b2c', 1), ('b2c', 2)]), (('o', 12), [('b2c', 3), 'b2d'])])
SCHED_E = [('b2a', 0), ('b2b', 0)] + [('b2c', i) for i in range(NB2C)] + [('b2d', 0)]


def _ln(x, eps=1e-5):
    m = jnp.mean(x, axis=-1, keepdims=True)
    xc = x - m
    v = jnp.mean(xc * xc, axis=-1, keepdims=True)
    return xc * jax.lax.rsqrt(v + eps)


def _gelu(x):
    return jax.nn.gelu(x, approximate=True)


def _dot(a, b):
    return jnp.dot(a, b, preferred_element_type=F32)


def _dot_nt(a, b):
    return jax.lax.dot_general(a, b, (((1,), (1,)), ((), ())), preferred_element_type=F32)


def _scope(name):
    return jax.named_scope(name) if SCOPES else contextlib.nullcontext()


def _wload(ref, ntile, k0=0, kn=None):
    if kn is None:
        return jnp.concatenate([pltpu.bitcast(ref[c], BF16) for c in range(ntile)], axis=1)
    return jnp.concatenate([pltpu.bitcast(ref[c, pl.ds(k0 // 2, kn // 2), :], BF16) for c in range(ntile)], axis=1)


def _kernel(x_hbm, mem0_hbm, wq_hbm, wk_hbm, wv_hbm, wo_hbm, w1_hbm, w2_hbm, w3_hbm, w4_hbm,
            out_hbm,
            wqkv, wob, ring, w1b, w2b, w3b, w4b, xbuf, ybuf, hbuf, obuf, stage, xin, mem0,
            sem_in, sem_out):
    w_hbm = (wq_hbm, wk_hbm, wv_hbm, wo_hbm)
    nsem = [0]

    def new_sem():
        nsem[0] += 1
        return sem_in.at[nsem[0] - 1]

    def cp_x(i):
        r0, r1 = XCH[i]
        return [pltpu.make_async_copy(x_hbm.at[pl.ds(r0, r1 - r0), :], xin.at[pl.ds(r0, r1 - r0), :], new_sem())]

    def cp_w(src_ref, dst_ref, ntile):
        sem = new_sem()
        return [pltpu.make_async_copy(src_ref.at[:, pl.ds(c * 128, 128)], dst_ref.at[c], sem) for c in range(ntile)]

    def cp_rows(j, p0, p1):
        rows = pl.ds(p0 * PW, (p1 - p0) * PW)
        sem = new_sem()
        if j < 3:
            return [pltpu.make_async_copy(w_hbm[j].at[rows, :], stage.at[j, rows, :], sem)]
        return [pltpu.make_async_copy(w_hbm[j].at[rows, pl.ds(c * 128, 128)], wob.at[c, rows, :], sem)
                for c in range(5)]

    cps = {'m': [pltpu.make_async_copy(mem0_hbm, mem0, new_sem())] + cp_x(0)}
    for g, (qkv, wo_, xc) in enumerate(GROUPS):
        cps['g', g] = []
        if qkv:
            cps['g', g] += [c for j in range(3) for c in cp_rows(j, *qkv)]
        if wo_:
            cps['g', g] += cp_rows(3, *wo_)
        for i in xc:
            cps['g', g] += cp_x(i)
    cps['w', 0] = cp_w(w1_hbm, w1b, 5) + [c for i in range(5, len(XCH)) for c in cp_x(i)]
    cps['w', 1] = cp_w(w2_hbm, w2b, 5)
    cps['w', 2] = cp_w(w3_hbm, w3b, 12)
    cps['w', 3] = cp_w(w4_hbm, w4b, 5)
    assert nsem[0] <= NSEM
    queue = list(cps)
    pos = {'started': 0, 'done': 0}

    def top_up(limit=DMA_DEPTH):
        while pos['started'] < min(len(queue), pos['done'] + limit):
            for c in cps[queue[pos['started']]]:
                c.start()
            pos['started'] += 1

    def arrive(key):
        assert key == queue[pos['done']]
        for c in cps[key]:
            c.wait()
        pos['done'] += 1
        top_up()

    top_up(2)
    wo, w1, w2, w3, w4 = (r.bitcast(U32) for r in (wob, w1b, w2b, w3b, w4b))

    z8 = jnp.zeros((8, DM), F32)
    hbuf[pl.ds(0, 8), :] = z8
    hbuf[pl.ds(8 + S_TOT, 8), :] = z8
    arrive('m')

    def ln0(i):
        for r in range(XCH[i][0], XCH[i][1], SEG):
            xv = xin[pl.ds(r, SEG), :].astype(F32)
            xbuf[pl.ds(r, SEG), :] = xv
            ybuf[pl.ds(r, SEG), :] = _ln(xv)
    ln0(0)

    row = jax.lax.broadcasted_iota(jnp.int32, (L, 128), 0)
    lane = jax.lax.broadcasted_iota(jnp.int32, (L, 128), 1)
    NEG = np.float32(-1e30)
    MASKED = np.float32(-1e9 * LOG2E)
    realA = lane < L
    realB = (lane >= 64) & (lane < 64 + L)
    validA = realA & ((row < MEM) | (row >= lane))
    validB = realB & ((row < MEM) | (row >= lane - 64))
    valid = validA | validB
    fill = jnp.where(realA | realB, MASKED, NEG)
    isA = lane < 64
    SC = np.float32(DH ** -0.5 * LOG2E)
    lane48 = jax.lax.broadcasted_iota(jnp.int32, (48, 128), 1)
    lo48 = lane48 < 64
    lane_h = jax.lax.broadcasted_iota(jnp.int32, (SEG, 128), 1)

    def blk(t):
        tb = jnp.concatenate([t, jnp.zeros((8, PW), F32)], axis=0).astype(BF16)
        t0 = tb[:, 0:128]
        t1 = tb[:, 128:256]
        t2 = tb[:, 256:384]
        z16 = jnp.zeros((16, 128), BF16)
        z64 = jnp.zeros((64, 128), BF16)
        z80 = jnp.zeros((80, 128), BF16)
        zb = jnp.zeros((48, 128), BF16)
        c0 = jnp.concatenate([t0, z80], axis=0)
        c1 = jnp.concatenate([jnp.where(lo48, t1, zb), z16, jnp.where(lo48, zb, t1), z16], axis=0)
        c2 = jnp.concatenate([z64, t2, z16], axis=0)
        return jnp.concatenate([c0, c1, c2], axis=1)

    def run(sched, rA=None, mem=None, rB1=None, rB2=None, y=None, yPre=None, short=None):
        st = {}
        if rA is not None and sched is not SCHED_0:
            yv = ybuf[pl.ds(y[0], y[1]), :] if isinstance(y, tuple) else y
            st['h'] = jnp.concatenate([mem, yv], axis=0)

        def f_pre(_):
            st['ypre'] = ybuf[pl.ds(yPre[0], yPre[1]), :]

        def f_wq(g):
            arrive(('g', g))

        def f_tr(pjc):
            p, j, c = pjc
            for m in range(5):
                blk_ = stage[j, pl.ds(p * PW + c * 128, 128), pl.ds(m * 128, 128)]
                wqkv[p, 3 * j + c, pl.ds(m * 64, 64), :] = pltpu.bitcast(blk_.T, U32)

        def f_bw(i):
            arrive(('w', i))

        def split_qkv(p, qkv):
            st['q', p] = qkv[:, 0:PW]
            st['k', p] = blk(qkv[:, PW:2 * PW])
            st['v', p] = blk(qkv[:, 2 * PW:3 * PW])

        def f_qkv0(pcj):
            p, c, j = pcj
            if c == 0:
                lhs = jnp.concatenate([mem, ybuf[pl.ds(0, C0 - MEM), :]], axis=0)
            else:
                lhs = ybuf[pl.ds(c * C0 - MEM, C0), :]
            res = _dot(lhs, _wload(wqkv.at[p, pl.ds(3 * j, 3)], 3))
            col = p * QW + j * PW
            if c == 0:
                st['qkv'[j], p] = res[0:L] if j == 0 else blk(res[0:L])
                ring[pl.ds(SEG, C0 - L), col:col + PW] = res[L:]
            else:
                ring[pl.ds(c * C0 - MEM, C0), col:col + PW] = res

        def f_qkv(p):
            res = _dot(st['h'], _wload(wqkv.at[p], 9))
            if short is not None:
                groups, rseg = short
                for g in range(SH // 8):
                    ring[pl.ds(groups[g], 8), p * QW:(p + 1) * QW] = res[MEM + 8 * g:MEM + 8 * g + 8]
                res = jnp.concatenate([res[0:MEM], ring[pl.ds(rseg, SEG), p * QW:(p + 1) * QW]], axis=0)
            split_qkv(p, res)

        def f_s(p):
            t = _dot_nt(st['q', p], st['k', p]) * SC
            s = jnp.where(valid, t, fill)
            mA = jnp.max(jnp.where(isA, s, NEG), axis=-1, keepdims=True)
            mB = jnp.max(jnp.where(isA, NEG, s), axis=-1, keepdims=True)
            e = jnp.exp2(s - jnp.where(isA, mA, mB))
            lA = jnp.sum(jnp.where(isA, e, 0.0), axis=-1, keepdims=True)
            lB = jnp.sum(jnp.where(isA, 0.0, e), axis=-1, keepdims=True)
            l = jnp.where(isA, lA, lB)
            r = pl.reciprocal(l, approx=True)
            r = r * (2.0 - l * r)
            st['p', p] = e * r

        def f_pv(p):
            st['o', p] = _dot(st['p', p], st['v', p])

        def f_o(p):
            c = _dot(st['o', p], _wload(wo, 5, p * PW, PW))
            st['acc'] = c if 'acc' not in st else st['acc'] + c

        def f_fin(_):
            acc = st['acc']
            xbuf[pl.ds(rA, SEG), :] = xbuf[pl.ds(rA, SEG), :] + acc[MEM:, :]
            st['mem'] = acc[0:MEM, :]

        def f_b1(_):
            x1 = xbuf[pl.ds(rB1, SEG), :]
            y = _ln(x1)
            ybuf[pl.ds(rB1, SEG), :] = y
            hbuf[pl.ds(rB1 + 8, SEG), :] = _gelu(_dot(_ln(y), _wload(w1, 5)))

        def f_b2a(_):
            def sh(j, d):
                win = hbuf[pl.ds(rB2, SEG + 16), j * 128:(j + 1) * 128]
                return win[8 + d:8 + d + SEG, :]
            cols = [
                sh(0, -1),
                jnp.where(lane_h < 32, sh(1, -1), sh(1, 1)),
                jnp.where(lane_h < 64, sh(2, 1), sh(2, -2)),
                jnp.where(lane_h < 96, sh(3, -2), sh(3, 2)),
                sh(4, 2),
            ]
            hs_in = jnp.concatenate(cols, axis=1)
            st['y1'] = ybuf[pl.ds(rB2, SEG), :] + _dot(hs_in, _wload(w2, 5))

        def f_b2b(_):
            st['g'] = _gelu(_dot(_ln(st['y1']), _wload(w3, 12)))

        def f_b2c(i):
            kc = FF // NB2C
            c = _dot(st['g'][:, i * kc:(i + 1) * kc], _wload(w4, 5, i * kc, kc))
            st['h2'] = c if 'h2' not in st else st['h2'] + c

        def f_b2d(_):
            xn = xbuf[pl.ds(rB2, SEG), :] + (st['y1'] + st['h2'])
            xbuf[pl.ds(rB2, SEG), :] = xn
            ybuf[pl.ds(rB2, SEG), :] = _ln(xn)
            obuf[pl.ds(rB2, SEG), :] = xn.astype(BF16)

        fs = {'q': f_qkv, 'q0': f_qkv0, 's': f_s, 'v': f_pv, 'o': f_o, 'fin': f_fin, 'b1': f_b1, 'b2a': f_b2a,
              'b2b': f_b2b, 'b2c': f_b2c, 'b2d': f_b2d, 'wq': f_wq, 'tr': f_tr, 'bw': f_bw, 'ln0': ln0,
              'pre': f_pre}
        for op, p in sched:
            fs[op](p)
        return st.get('mem'), st.get('ypre')

    def seg_row(t):
        return pl.multiple_of((t & (NSEG - 1)) * SEG, SEG)

    def new_rows(t):
        return R0 + SH * (t - 1)

    with _scope("step0"):
        mem, _ = run(SCHED_0, rA=0, mem=mem0[...].astype(F32))
    with _scope("step1"):
        mem, _ = run(SCHED_1, rA=SEG, mem=mem, rB1=0, y=(new_rows(1), SH),
                     short=([(new_rows(1) + 8 * g) % RING for g in range(SH // 8)], SEG))
        run([('bw', 2), ('bw', 3)])

    def short_body(u, mem):
        t0 = 2 * u + 2
        y = (pl.multiple_of(new_rows(t0), 8), SH)
        for k in range(2):
            t = t0 + k
            groups = [pl.multiple_of(jax.lax.rem(new_rows(t) + 8 * g, RING), 8) for g in range(SH // 8)]
            rseg = pl.multiple_of(jax.lax.rem(t * SEG, RING), SEG)
            mem, y = run(SCHED_SB if k else SCHED_SA, rA=seg_row(t), mem=mem, rB1=seg_row(t - 1), rB2=seg_row(t - 2),
                         y=y, yPre=None if k else (pl.multiple_of(new_rows(t + 1), 8), SH), short=(groups, rseg))
        return mem

    with _scope("short"):
        mem = jax.lax.fori_loop(0, (TS - 2) // 2, short_body, mem)

    def body(u, mem):
        t0 = 2 * u + TS
        y = (seg_row(t0), SEG)
        mem = jnp.where(t0 == NSEG, mem0[...].astype(F32), mem)
        for k in range(2):
            t = t0 + k
            mem, y = run(SCHED_B if k else SCHED_A, rA=seg_row(t), mem=mem, rB1=seg_row(t - 1), rB2=seg_row(t - 2),
                         y=y, yPre=None if k else (seg_row(t + 1), SEG))

        @pl.when(t0 >= NSEG + 2)
        def _():
            r = pl.multiple_of((t0 - NSEG - 2) * SEG, 2 * SEG)
            pltpu.make_async_copy(obuf.at[pl.ds(r, 2 * SEG), :], out_hbm.at[pl.ds(r, 2 * SEG), :], sem_out.at[0]).start()
        return mem

    with _scope("main"):
        jax.lax.fori_loop(0, (2 * NSEG - TS) // 2, body, mem)

    with _scope("epi"):
        r63 = (NSEG - 1) * SEG
        r62 = (NSEG - 2) * SEG
        run([('b1', 0)] + SCHED_E, rB1=r63, rB2=r62)
        run(SCHED_E, rB2=r63)
        pltpu.make_async_copy(obuf.at[pl.ds(r62, 2 * SEG), :], out_hbm.at[pl.ds(r62, 2 * SEG), :], sem_out.at[0]).start()
        pltpu.make_async_copy(obuf.at[pl.ds(0, S_TOT), :], out_hbm, sem_out.at[0]).wait()


@jax.jit
def pallas_interleave_layers__memory_aug_recurrent_mem_tr__mixer_s_mlp__prompt_kernel(A_x, A_mem0, A_Wq, A_Wk, A_Wv, A_Wo, A_seg_len, B_x, B_w1, B_w2, B_w3, B_w4):
    del A_seg_len, B_x
    x2 = A_x.reshape(S_TOT, DM)
    m2 = A_mem0.reshape(MEM, DM)
    wqT = A_Wq.transpose(1, 2, 0).reshape(HD, DM)
    wkT = A_Wk.transpose(1, 2, 0).reshape(HD, DM)
    wvT = A_Wv.transpose(1, 2, 0).reshape(HD, DM)
    wo2 = A_Wo.reshape(HD, DM)
    any_spec = pl.BlockSpec(memory_space=pl.ANY)
    out = pl.pallas_call(
        _kernel,
        out_shape=jax.ShapeDtypeStruct((S_TOT, DM), BF16),
        in_specs=[any_spec] * 10,
        out_specs=any_spec,
        scratch_shapes=[
            pltpu.VMEM((NP, 9, DM // 2, 128), U32),
            pltpu.VMEM((5, HD, 128), BF16),
            pltpu.VMEM((RING, NP * QW), F32),
            pltpu.VMEM((5, DM, 128), BF16),
            pltpu.VMEM((5, DM, 128), BF16),
            pltpu.VMEM((12, DM, 128), BF16),
            pltpu.VMEM((5, FF, 128), BF16),
            pltpu.VMEM((S_TOT + 64, DM), F32),
            pltpu.VMEM((S_TOT + 64, DM), F32),
            pltpu.VMEM((S_TOT + 64, DM), F32),
            pltpu.VMEM((S_TOT + 64, DM), BF16),
            pltpu.VMEM((3, HD, DM), BF16),
            pltpu.VMEM((S_TOT, DM), BF16),
            pltpu.VMEM((MEM, DM), BF16),
            pltpu.SemaphoreType.DMA((NSEM,)),
            pltpu.SemaphoreType.DMA((1,)),
        ],
        compiler_params=pltpu.CompilerParams(vmem_limit_bytes=120 * 1024 * 1024),
    )(x2, m2, wqT, wkT, wvT, wo2, B_w1, B_w2, B_w3, B_w4)
    return out.reshape(1, S_TOT, DM)
```

```python
import contextlib
import jax
import jax.numpy as jnp
import numpy as np
import jax.experimental.pallas as pl
import jax.experimental.pallas.tpu as pltpu

F32 = jnp.float32
BF16 = jnp.bfloat16
U32 = jnp.uint32

S_TOT = 2048
DM = 640
NH = 32
DH = 192
HD = NH * DH
MEM = 8
SEG = 32
NSEG = S_TOT // SEG
L = MEM + SEG
NP = NH // 2
PW = 2 * DH
QW = 3 * PW
FF = 1536
LOG2E = 1.4426950408889634
SCOPES = False
NB2C = 4

SH = 24
R0 = 344
TS = (R0 - SH) // (SEG - SH)
RING = (R0 + 31) // 32 * 32
C0 = (R0 + MEM) // 4
XCH = [(0, RING), (RING, 512)] + [(r, r + 256) for r in range(512, S_TOT, 256)]
NSEM = 64
DMA_DEPTH = 3
GROUPS = [((0, 1), None, ()), ((1, 2), None, ()), ((2, 3), None, ()), ((3, 4), None, ()), ((4, 5), None, ()),
          ((5, 6), None, (1,)), ((6, 7), None, ()), ((7, 9), None, (2, 3)), ((9, 11), None, (4, 5)),
          ((11, 13), None, (6,)), ((13, 16), None, (7,)),
          (None, (0, 4), ()), (None, (4, 8), ()), (None, (8, 12), ()), (None, (12, 16), ())]
BAR_POS = {1: 7, 2: 3}
O_SLOTS = {11: (13, 6), 12: (15, 0)}


def _make_sched(lag_s=1, lag_v=2, lag_o=5):
    ops = []
    i = 0
    done_o = 0
    while done_o < NP:
        if i < NP:
            ops.append(('q', i))
        if 0 <= i - lag_s < NP:
            ops.append(('s', i - lag_s))
        if 0 <= i - lag_o < NP:
            ops.append(('o', i - lag_o))
            done_o += 1
        if 0 <= i - lag_v < NP:
            ops.append(('v', i - lag_v))
        i += 1
    ops.append(('fin', 0))
    return ops


def _place(ops, places):
    out = []
    pl_ = {a: l for a, l in places}
    for o in ops:
        out.append(o)
        for b in pl_.get(o, ()):
            out.append(b if isinstance(b, tuple) else (b, 0))
    return out


def _sched0():
    first = {q[0]: g for g, (q, _, _) in enumerate(GROUPS) if q}
    ops = [('wq', 0)]
    tr = [('tr', (0, j, c)) for j in range(3) for c in range(3)]
    todo_x, todo_o = [], []
    for i in range(NP + 2):
        mm = [('q0', (i, c, j)) for c in range(4) for j in range(3)] if i < NP else []
        for k in range(12):
            if mm:
                if k < 3:
                    while tr and tr[0][1][:2] <= (i, k):
                        ops.append(tr.pop(0))
                ops.append(mm[k])
            if i + 1 < NP and k == BAR_POS.get(i + 1, 0):
                if i + 1 in first:
                    g = first[i + 1]
                    ops.append(('wq', g))
                    todo_x += list(GROUPS[g][2])
                tr += [('tr', (i + 1, j, c)) for j in range(3) for c in range(3)]
            if tr:
                ops.append(tr.pop(0))
            if k == 2 and 0 <= i - 1 < NP:
                ops.append(('s', i - 1))
            if k == 5 and 0 <= i - 2 < NP:
                ops.append(('v', i - 2))
            for g, pos_ in O_SLOTS.items():
                if pos_ == (i, k):
                    ops.append(('wq', g))
                    todo_o += list(range(*GROUPS[g][1]))
            if todo_o and k in (3, 4, 7, 8, 10, 11) and todo_o[0] <= i - 3:
                ops.append(('o', todo_o.pop(0)))
            if todo_x and k == 9:
                ops.append(('ln0', todo_x.pop(0)))
    assert not tr and not todo_x
    ops += [('o', p) for p in todo_o]
    for g, (q, wo_, _) in enumerate(GROUPS):
        if not q and g not in O_SLOTS:
            ops += [('wq', g)] + [('o', p) for p in range(*wo_)]
    ops.append(('fin', 0))
    return ops


SCHED_0 = _sched0()
SCHED_1 = _place(_make_sched(lag_o=7), [(('q', 4), [('bw', 0)]), (('s', 15), ['b1'])])
SCHED_A = _place(_make_sched(lag_v=2, lag_o=4),
                 [(('q', 2), ['b1']), (('q', 4), ['b2a']), (('q', 9), ['b2b']),
                  (('q', 14), ['pre', ('b2c', 0), ('b2c', 1)]), (('o', 13), [('b2c', 2)]),
                  (('fin', 0), [('b2c', 3), 'b2d'])])
SCHED_B = _place(_make_sched(lag_v=2, lag_o=5),
                 [(('q', 2), ['b1']), (('q', 4), ['b2a']), (('q', 9), ['b2b']), (('q', 14), [('b2c', 0)]),
                  (('s', 14), [('b2c', 1)]), (('o', 11), [('b2c', 2)]), (('v', 15), [('b2c', 3), 'b2d'])])
SCHED_SA = _place(_make_sched(lag_v=2, lag_o=7),
                  [(('q', 2), ['b1']), (('q', 6), ['b2a']), (('q', 9), ['b2b']), (('s', 15), [('b2c', 0)]),
                   (('o', 9), [('b2c', 1)]), (('o', 14), ['pre', ('b2c', 2)]), (('fin', 0), [('b2c', 3), 'b2d'])])
SCHED_SB = _place(_make_sched(lag_v=2, lag_o=4),
                  [(('q', 2), ['b1']), (('q', 4), ['b2a']), (('q', 7), ['b2b']), (('q', 10), [('b2c', 0)]),
                   (('v', 13), [('b2c', 1), ('b2c', 2)]), (('o', 12), [('b2c', 3), 'b2d'])])
SCHED_S2 = []
for _op in SCHED_SA:
    if _op[0] in ('b2a', 'b2b') or _op == ('b2c', 0):
        SCHED_S2.append(('bw', {'b2a': 1, 'b2b': 2, 'b2c': 3}[_op[0]]))
    SCHED_S2.append(_op)
SCHED_E = [('b2a', 0), ('b2b', 0)] + [('b2c', i) for i in range(NB2C)] + [('b2d', 0)]


def _ln(x, eps=1e-5):
    m = jnp.mean(x, axis=-1, keepdims=True)
    xc = x - m
    v = jnp.mean(xc * xc, axis=-1, keepdims=True)
    return xc * jax.lax.rsqrt(v + eps)


def _gelu(x):
    return jax.nn.gelu(x, approximate=True)


def _dot(a, b):
    return jnp.dot(a, b, preferred_element_type=F32)


def _dot_nt(a, b):
    return jax.lax.dot_general(a, b, (((1,), (1,)), ((), ())), preferred_element_type=F32)


def _scope(name):
    return jax.named_scope(name) if SCOPES else contextlib.nullcontext()


def _wload(ref, ntile, k0=0, kn=None):
    if kn is None:
        return jnp.concatenate([pltpu.bitcast(ref[c], BF16) for c in range(ntile)], axis=1)
    return jnp.concatenate([pltpu.bitcast(ref[c, pl.ds(k0 // 2, kn // 2), :], BF16) for c in range(ntile)], axis=1)


def _kernel(x_hbm, mem0_hbm, wq_hbm, wk_hbm, wv_hbm, wo_hbm, w1_hbm, w2_hbm, w3_hbm, w4_hbm,
            out_hbm,
            wqkv, wob, ring, w1b, w2b, w3b, w4b, xbuf, ybuf, hbuf, obuf, stage, xin, mem0,
            sem_in, sem_out):
    w_hbm = (wq_hbm, wk_hbm, wv_hbm, wo_hbm)
    nsem = [0]

    def new_sem():
        nsem[0] += 1
        return sem_in.at[nsem[0] - 1]

    def cp_x(i):
        r0, r1 = XCH[i]
        return [pltpu.make_async_copy(x_hbm.at[pl.ds(r0, r1 - r0), :], xin.at[pl.ds(r0, r1 - r0), :], new_sem())]

    def cp_w(src_ref, dst_ref, ntile):
        sem = new_sem()
        return [pltpu.make_async_copy(src_ref.at[:, pl.ds(c * 128, 128)], dst_ref.at[c], sem) for c in range(ntile)]

    def cp_rows(j, p0, p1):
        rows = pl.ds(p0 * PW, (p1 - p0) * PW)
        sem = new_sem()
        if j < 3:
            return [pltpu.make_async_copy(w_hbm[j].at[rows, :], stage.at[j, rows, :], sem)]
        return [pltpu.make_async_copy(w_hbm[j].at[rows, pl.ds(c * 128, 128)], wob.at[c, rows, :], sem)
                for c in range(5)]

    cps = {'m': [pltpu.make_async_copy(mem0_hbm, mem0, new_sem())] + cp_x(0)}
    for g, (qkv, wo_, xc) in enumerate(GROUPS):
        cps['g', g] = []
        if qkv:
            cps['g', g] += [c for j in range(3) for c in cp_rows(j, *qkv)]
        if wo_:
            cps['g', g] += cp_rows(3, *wo_)
        for i in xc:
            cps['g', g] += cp_x(i)
    cps['w', 0] = cp_w(w1_hbm, w1b, 5)
    cps['w', 1] = cp_w(w2_hbm, w2b, 5)
    cps['w', 2] = cp_w(w3_hbm, w3b, 12)
    cps['w', 3] = cp_w(w4_hbm, w4b, 5)
    assert nsem[0] <= NSEM
    queue = list(cps)
    pos = {'started': 0, 'done': 0}

    def top_up(limit=DMA_DEPTH):
        while pos['started'] < min(len(queue), pos['done'] + limit):
            for c in cps[queue[pos['started']]]:
                c.start()
            pos['started'] += 1

    def arrive(key):
        assert key == queue[pos['done']]
        for c in cps[key]:
            c.wait()
        pos['done'] += 1
        top_up()

    top_up(2)
    wo, w1, w2, w3, w4 = (r.bitcast(U32) for r in (wob, w1b, w2b, w3b, w4b))

    z8 = jnp.zeros((8, DM), F32)
    hbuf[pl.ds(0, 8), :] = z8
    hbuf[pl.ds(8 + S_TOT, 8), :] = z8
    arrive('m')

    def ln0(i):
        for r in range(XCH[i][0], XCH[i][1], SEG):
            xv = xin[pl.ds(r, SEG), :].astype(F32)
            xbuf[pl.ds(r, SEG), :] = xv
            ybuf[pl.ds(r, SEG), :] = _ln(xv)
    ln0(0)

    row = jax.lax.broadcasted_iota(jnp.int32, (L, 128), 0)
    lane = jax.lax.broadcasted_iota(jnp.int32, (L, 128), 1)
    NEG = np.float32(-1e30)
    MASKED = np.float32(-1e9 * LOG2E)
    realA = lane < L
    realB = (lane >= 64) & (lane < 64 + L)
    validA = realA & ((row < MEM) | (row >= lane))
    validB = realB & ((row < MEM) | (row >= lane - 64))
    valid = validA | validB
    fill = jnp.where(realA | realB, MASKED, NEG)
    isA = lane < 64
    SC = np.float32(DH ** -0.5 * LOG2E)
    lane48 = jax.lax.broadcasted_iota(jnp.int32, (48, 128), 1)
    lo48 = lane48 < 64
    lane_h = jax.lax.broadcasted_iota(jnp.int32, (SEG, 128), 1)

    def blk(t):
        tb = jnp.concatenate([t, jnp.zeros((8, PW), F32)], axis=0).astype(BF16)
        t0 = tb[:, 0:128]
        t1 = tb[:, 128:256]
        t2 = tb[:, 256:384]
        z16 = jnp.zeros((16, 128), BF16)
        z64 = jnp.zeros((64, 128), BF16)
        z80 = jnp.zeros((80, 128), BF16)
        zb = jnp.zeros((48, 128), BF16)
        c0 = jnp.concatenate([t0, z80], axis=0)
        c1 = jnp.concatenate([jnp.where(lo48, t1, zb), z16, jnp.where(lo48, zb, t1), z16], axis=0)
        c2 = jnp.concatenate([z64, t2, z16], axis=0)
        return jnp.concatenate([c0, c1, c2], axis=1)

    def run(sched, rA=None, mem=None, rB1=None, rB2=None, y=None, yPre=None, short=None):
        st = {}
        if rA is not None and sched is not SCHED_0:
            yv = ybuf[pl.ds(y[0], y[1]), :] if isinstance(y, tuple) else y
            st['h'] = jnp.concatenate([mem, yv], axis=0)

        def f_pre(_):
            st['ypre'] = ybuf[pl.ds(yPre[0], yPre[1]), :]

        def f_wq(g):
            arrive(('g', g))

        def f_tr(pjc):
            p, j, c = pjc
            for m in range(5):
                blk_ = stage[j, pl.ds(p * PW + c * 128, 128), pl.ds(m * 128, 128)]
                wqkv[p, 3 * j + c, pl.ds(m * 64, 64), :] = pltpu.bitcast(blk_.T, U32)

        def f_bw(i):
            arrive(('w', i))

        def split_qkv(p, qkv):
            st['q', p] = qkv[:, 0:PW]
            st['k', p] = blk(qkv[:, PW:2 * PW])
            st['v', p] = blk(qkv[:, 2 * PW:3 * PW])

        def f_qkv0(pcj):
            p, c, j = pcj
            if c == 0:
                lhs = jnp.concatenate([mem, ybuf[pl.ds(0, C0 - MEM), :]], axis=0)
            else:
                lhs = ybuf[pl.ds(c * C0 - MEM, C0), :]
            res = _dot(lhs, _wload(wqkv.at[p, pl.ds(3 * j, 3)], 3))
            col = p * QW + j * PW
            if c == 0:
                st['qkv'[j], p] = res[0:L] if j == 0 else blk(res[0:L])
                ring[pl.ds(SEG, C0 - L), col:col + PW] = res[L:]
            else:
                ring[pl.ds(c * C0 - MEM, C0), col:col + PW] = res

        def f_qkv(p):
            res = _dot(st['h'], _wload(wqkv.at[p], 9))
            if short is not None:
                groups, rseg = short
                for g in range(SH // 8):
                    ring[pl.ds(groups[g], 8), p * QW:(p + 1) * QW] = res[MEM + 8 * g:MEM + 8 * g + 8]
                res = jnp.concatenate([res[0:MEM], ring[pl.ds(rseg, SEG), p * QW:(p + 1) * QW]], axis=0)
            split_qkv(p, res)

        def f_s(p):
            t = _dot_nt(st['q', p], st['k', p]) * SC
            s = jnp.where(valid, t, fill)
            mA = jnp.max(jnp.where(isA, s, NEG), axis=-1, keepdims=True)
            mB = jnp.max(jnp.where(isA, NEG, s), axis=-1, keepdims=True)
            e = jnp.exp2(s - jnp.where(isA, mA, mB))
            lA = jnp.sum(jnp.where(isA, e, 0.0), axis=-1, keepdims=True)
            lB = jnp.sum(jnp.where(isA, 0.0, e), axis=-1, keepdims=True)
            l = jnp.where(isA, lA, lB)
            r = pl.reciprocal(l, approx=True)
            r = r * (2.0 - l * r)
            st['p', p] = e * r

        def f_pv(p):
            st['o', p] = _dot(st['p', p], st['v', p])

        def f_o(p):
            c = _dot(st['o', p], _wload(wo, 5, p * PW, PW))
            st['acc'] = c if 'acc' not in st else st['acc'] + c

        def f_fin(_):
            acc = st['acc']
            xbuf[pl.ds(rA, SEG), :] = xbuf[pl.ds(rA, SEG), :] + acc[MEM:, :]
            st['mem'] = acc[0:MEM, :]

        def f_b1(_):
            x1 = xbuf[pl.ds(rB1, SEG), :]
            y = _ln(x1)
            ybuf[pl.ds(rB1, SEG), :] = y
            hbuf[pl.ds(rB1 + 8, SEG), :] = _gelu(_dot(_ln(y), _wload(w1, 5)))

        def f_b2a(_):
            def sh(j, d):
                win = hbuf[pl.ds(rB2, SEG + 16), j * 128:(j + 1) * 128]
                return win[8 + d:8 + d + SEG, :]
            cols = [
                sh(0, -1),
                jnp.where(lane_h < 32, sh(1, -1), sh(1, 1)),
                jnp.where(lane_h < 64, sh(2, 1), sh(2, -2)),
                jnp.where(lane_h < 96, sh(3, -2), sh(3, 2)),
                sh(4, 2),
            ]
            hs_in = jnp.concatenate(cols, axis=1)
            st['y1'] = ybuf[pl.ds(rB2, SEG), :] + _dot(hs_in, _wload(w2, 5))

        def f_b2b(_):
            st['g'] = _gelu(_dot(_ln(st['y1']), _wload(w3, 12)))

        def f_b2c(i):
            kc = FF // NB2C
            c = _dot(st['g'][:, i * kc:(i + 1) * kc], _wload(w4, 5, i * kc, kc))
            st['h2'] = c if 'h2' not in st else st['h2'] + c

        def f_b2d(_):
            xn = xbuf[pl.ds(rB2, SEG), :] + (st['y1'] + st['h2'])
            xbuf[pl.ds(rB2, SEG), :] = xn
            ybuf[pl.ds(rB2, SEG), :] = _ln(xn)
            obuf[pl.ds(rB2, SEG), :] = xn.astype(BF16)

        fs = {'q': f_qkv, 'q0': f_qkv0, 's': f_s, 'v': f_pv, 'o': f_o, 'fin': f_fin, 'b1': f_b1, 'b2a': f_b2a,
              'b2b': f_b2b, 'b2c': f_b2c, 'b2d': f_b2d, 'wq': f_wq, 'tr': f_tr, 'bw': f_bw, 'ln0': ln0,
              'pre': f_pre}
        for op, p in sched:
            fs[op](p)
        return st.get('mem'), st.get('ypre')

    def seg_row(t):
        return pl.multiple_of((t & (NSEG - 1)) * SEG, SEG)

    def new_rows(t):
        return R0 + SH * (t - 1)

    with _scope("step0"):
        mem, _ = run(SCHED_0, rA=0, mem=mem0[...].astype(F32))
    with _scope("step1"):
        mem, _ = run(SCHED_1, rA=SEG, mem=mem, rB1=0, y=(new_rows(1), SH),
                     short=([(new_rows(1) + 8 * g) % RING for g in range(SH // 8)], SEG))

    def short_body(u, mem, first=False):
        t0 = 2 * u + 2
        y = (pl.multiple_of(new_rows(t0), 8), SH)
        for k in range(2):
            t = t0 + k
            groups = [pl.multiple_of(jax.lax.rem(new_rows(t) + 8 * g, RING), 8) for g in range(SH // 8)]
            rseg = pl.multiple_of(jax.lax.rem(t * SEG, RING), SEG)
            mem, y = run(SCHED_SB if k else (SCHED_S2 if first else SCHED_SA), rA=seg_row(t), mem=mem, rB1=seg_row(t - 1), rB2=seg_row(t - 2),
                         y=y, yPre=None if k else (pl.multiple_of(new_rows(t + 1), 8), SH), short=(groups, rseg))
        return mem

    with _scope("short"):
        mem = short_body(jnp.int32(0), mem, first=True)
        mem = jax.lax.fori_loop(1, (TS - 2) // 2, short_body, mem)

    def body(u, mem):
        t0 = 2 * u + TS
        y = (seg_row(t0), SEG)
        mem = jnp.where(t0 == NSEG, mem0[...].astype(F32), mem)
        for k in range(2):
            t = t0 + k
            mem, y = run(SCHED_B if k else SCHED_A, rA=seg_row(t), mem=mem, rB1=seg_row(t - 1), rB2=seg_row(t - 2),
                         y=y, yPre=None if k else (seg_row(t + 1), SEG))

        @pl.when(t0 >= NSEG + 2)
        def _():
            r = pl.multiple_of((t0 - NSEG - 2) * SEG, 2 * SEG)
            pltpu.make_async_copy(obuf.at[pl.ds(r, 2 * SEG), :], out_hbm.at[pl.ds(r, 2 * SEG), :], sem_out.at[0]).start()
        return mem

    with _scope("main"):
        jax.lax.fori_loop(0, (2 * NSEG - TS) // 2, body, mem)

    with _scope("epi"):
        r63 = (NSEG - 1) * SEG
        r62 = (NSEG - 2) * SEG
        run([('b1', 0)] + SCHED_E, rB1=r63, rB2=r62)
        run(SCHED_E, rB2=r63)
        pltpu.make_async_copy(obuf.at[pl.ds(r62, 2 * SEG), :], out_hbm.at[pl.ds(r62, 2 * SEG), :], sem_out.at[0]).start()
        pltpu.make_async_copy(obuf.at[pl.ds(0, S_TOT), :], out_hbm, sem_out.at[0]).wait()


@jax.jit
def pallas_interleave_layers__memory_aug_recurrent_mem_tr__mixer_s_mlp__prompt_kernel(A_x, A_mem0, A_Wq, A_Wk, A_Wv, A_Wo, A_seg_len, B_x, B_w1, B_w2, B_w3, B_w4):
    del A_seg_len, B_x
    x2 = A_x.reshape(S_TOT, DM)
    m2 = A_mem0.reshape(MEM, DM)
    wqT = A_Wq.transpose(1, 2, 0).reshape(HD, DM)
    wkT = A_Wk.transpose(1, 2, 0).reshape(HD, DM)
    wvT = A_Wv.transpose(1, 2, 0).reshape(HD, DM)
    wo2 = A_Wo.reshape(HD, DM)
    any_spec = pl.BlockSpec(memory_space=pl.ANY)
    out = pl.pallas_call(
        _kernel,
        out_shape=jax.ShapeDtypeStruct((S_TOT, DM), BF16),
        in_specs=[any_spec] * 10,
        out_specs=any_spec,
        scratch_shapes=[
            pltpu.VMEM((NP, 9, DM // 2, 128), U32),
            pltpu.VMEM((5, HD, 128), BF16),
            pltpu.VMEM((RING, NP * QW), F32),
            pltpu.VMEM((5, DM, 128), BF16),
            pltpu.VMEM((5, DM, 128), BF16),
            pltpu.VMEM((12, DM, 128), BF16),
            pltpu.VMEM((5, FF, 128), BF16),
            pltpu.VMEM((S_TOT + 64, DM), F32),
            pltpu.VMEM((S_TOT + 64, DM), F32),
            pltpu.VMEM((S_TOT + 64, DM), F32),
            pltpu.VMEM((S_TOT + 64, DM), BF16),
            pltpu.VMEM((3, HD, DM), BF16),
            pltpu.VMEM((S_TOT, DM), BF16),
            pltpu.VMEM((MEM, DM), BF16),
            pltpu.SemaphoreType.DMA((NSEM,)),
            pltpu.SemaphoreType.DMA((1,)),
        ],
        compiler_params=pltpu.CompilerParams(vmem_limit_bytes=120 * 1024 * 1024),
    )(x2, m2, wqT, wkT, wvT, wo2, B_w1, B_w2, B_w3, B_w4)
    return out.reshape(1, S_TOT, DM)
```

```python
import contextlib
import jax
import jax.numpy as jnp
import numpy as np
import jax.experimental.pallas as pl
import jax.experimental.pallas.tpu as pltpu

F32 = jnp.float32
BF16 = jnp.bfloat16
U32 = jnp.uint32

S_TOT = 2048
DM = 640
NH = 32
DH = 192
HD = NH * DH
MEM = 8
SEG = 32
NSEG = S_TOT // SEG
L = MEM + SEG
NP = NH // 2
PW = 2 * DH
QW = 3 * PW
FF = 1536
LOG2E = 1.4426950408889634
SCOPES = False
NB2C = 4

SH = 24
R0 = 344
TS = (R0 - SH) // (SEG - SH)
RING = (R0 + 31) // 32 * 32
C0 = (R0 + MEM) // 4
XCH = [(0, RING), (RING, 512)] + [(r, r + 256) for r in range(512, S_TOT, 256)]
DMA_DEPTH = 3
GROUPS = [((0, 1), None, ()), ((1, 2), None, ()), ((2, 3), None, ()), ((3, 4), None, ()), ((4, 5), None, ()),
          ((5, 6), None, (1,)), ((6, 7), None, ()), ((7, 9), None, (2, 3)), ((9, 11), None, (4, 5)),
          ((11, 13), None, (6,)), ((13, 16), None, (7,)),
          (None, (0, 4), ()), (None, (4, 8), ()), (None, (8, 12), ()), (None, (12, 16), ())]
BAR_POS = {1: 7, 2: 3}
O_SLOTS = {11: (13, 6), 12: (15, 0)}


def _make_sched(lag_s=1, lag_v=2, lag_o=5):
    ops = []
    i = 0
    done_o = 0
    while done_o < NP:
        if i < NP:
            ops.append(('q', i))
        if 0 <= i - lag_s < NP:
            ops.append(('s', i - lag_s))
        if 0 <= i - lag_o < NP:
            ops.append(('o', i - lag_o))
            done_o += 1
        if 0 <= i - lag_v < NP:
            ops.append(('v', i - lag_v))
        i += 1
    ops.append(('fin', 0))
    return ops


def _place(ops, places):
    out = []
    pl_ = {a: l for a, l in places}
    for o in ops:
        out.append(o)
        for b in pl_.get(o, ()):
            out.append(b if isinstance(b, tuple) else (b, 0))
    return out


def _sched0():
    first = {q[0]: g for g, (q, _, _) in enumerate(GROUPS) if q}
    ops = [('wq', 0)]
    tr = [('tr', (0, j, c)) for j in range(3) for c in range(3)]
    todo_x, todo_o = [], []
    for i in range(NP + 2):
        mm = [('q0', (i, c, j)) for c in range(4) for j in range(3)] if i < NP else []
        for k in range(12):
            if mm:
                if k < 3:
                    while tr and tr[0][1][:2] <= (i, k):
                        ops.append(tr.pop(0))
                ops.append(mm[k])
            if i + 1 < NP and k == BAR_POS.get(i + 1, 0):
                if i + 1 in first:
                    g = first[i + 1]
                    ops.append(('wq', g))
                    todo_x += list(GROUPS[g][2])
                tr += [('tr', (i + 1, j, c)) for j in range(3) for c in range(3)]
            if tr:
                ops.append(tr.pop(0))
            if k == 2 and 0 <= i - 1 < NP:
                ops.append(('s', i - 1))
            if k == 5 and 0 <= i - 2 < NP:
                ops.append(('v', i - 2))
            for g, pos_ in O_SLOTS.items():
                if pos_ == (i, k):
                    ops.append(('wq', g))
                    todo_o += list(range(*GROUPS[g][1]))
            if todo_o and k in (3, 4, 7, 8, 10, 11) and todo_o[0] <= i - 3:
                ops.append(('o', todo_o.pop(0)))
            if todo_x and k == 9:
                ops.append(('ln0', todo_x.pop(0)))
    assert not tr and not todo_x
    ops += [('o', p) for p in todo_o]
    for g, (q, wo_, _) in enumerate(GROUPS):
        if not q and g not in O_SLOTS:
            ops += [('wq', g)] + [('o', p) for p in range(*wo_)]
    ops.append(('fin', 0))
    return ops


SCHED_0 = _sched0()
SCHED_1 = _place(_make_sched(lag_o=7), [(('q', 4), [('bw', 0)]), (('s', 15), ['b1'])])
SCHED_A = _place(_make_sched(lag_v=2, lag_o=4),
                 [(('q', 2), ['b1']), (('q', 4), ['b2a']), (('q', 9), ['b2b']),
                  (('q', 14), ['pre', ('b2c', 0), ('b2c', 1)]), (('o', 13), [('b2c', 2)]),
                  (('fin', 0), [('b2c', 3), 'b2d'])])
SCHED_B = _place(_make_sched(lag_v=2, lag_o=5),
                 [(('q', 2), ['b1']), (('q', 4), ['b2a']), (('q', 9), ['b2b']), (('q', 14), [('b2c', 0)]),
                  (('s', 14), [('b2c', 1)]), (('o', 11), [('b2c', 2)]), (('v', 15), [('b2c', 3), 'b2d'])])
SCHED_SA = _place(_make_sched(lag_v=2, lag_o=7),
                  [(('q', 2), ['b1']), (('q', 6), ['b2a']), (('q', 9), ['b2b']), (('s', 15), [('b2c', 0)]),
                   (('o', 9), [('b2c', 1)]), (('o', 14), ['pre', ('b2c', 2)]), (('fin', 0), [('b2c', 3), 'b2d'])])
SCHED_SB = _place(_make_sched(lag_v=2, lag_o=4),
                  [(('q', 2), ['b1']), (('q', 4), ['b2a']), (('q', 7), ['b2b']), (('q', 10), [('b2c', 0)]),
                   (('v', 13), [('b2c', 1), ('b2c', 2)]), (('o', 12), [('b2c', 3), 'b2d'])])
SCHED_S2 = []
for _op in SCHED_SA:
    if _op[0] in ('b2a', 'b2b') or _op == ('b2c', 0):
        SCHED_S2.append(('bw', {'b2a': 1, 'b2b': 2, 'b2c': 3}[_op[0]]))
    SCHED_S2.append(_op)
SCHED_E = [('b2a', 0), ('b2b', 0)] + [('b2c', i) for i in range(NB2C)] + [('b2d', 0)]


def _ln(x, eps=1e-5):
    m = jnp.mean(x, axis=-1, keepdims=True)
    xc = x - m
    v = jnp.mean(xc * xc, axis=-1, keepdims=True)
    return xc * jax.lax.rsqrt(v + eps)


def _gelu(x):
    return jax.nn.gelu(x, approximate=True)


def _dot(a, b):
    return jnp.dot(a, b, preferred_element_type=F32)


def _dot_nt(a, b):
    return jax.lax.dot_general(a, b, (((1,), (1,)), ((), ())), preferred_element_type=F32)


def _scope(name):
    return jax.named_scope(name) if SCOPES else contextlib.nullcontext()


def _wload(ref, ntile, k0=0, kn=None):
    if kn is None:
        return jnp.concatenate([pltpu.bitcast(ref[c], BF16) for c in range(ntile)], axis=1)
    return jnp.concatenate([pltpu.bitcast(ref[c, pl.ds(k0 // 2, kn // 2), :], BF16) for c in range(ntile)], axis=1)


def _kernel(x_hbm, mem0_hbm, wq_hbm, wk_hbm, wv_hbm, wo_hbm, w1_hbm, w2_hbm, w3_hbm, w4_hbm,
            out_hbm,
            wqkv, wob, ring, w1b, w2b, w3b, w4b, xbuf, ybuf, hbuf, obuf, stage, xin, mem0,
            sem_in, sem_out):
    w_hbm = (wq_hbm, wk_hbm, wv_hbm, wo_hbm)
    def cp_x(i, sem):
        r0, r1 = XCH[i]
        return [pltpu.make_async_copy(x_hbm.at[pl.ds(r0, r1 - r0), :], xin.at[pl.ds(r0, r1 - r0), :], sem)]

    def cp_w(src_ref, dst_ref, ntile, sem):
        return [pltpu.make_async_copy(src_ref.at[:, pl.ds(c * 128, 128)], dst_ref.at[c], sem) for c in range(ntile)]

    def cp_rows(j, p0, p1, sem):
        rows = pl.ds(p0 * PW, (p1 - p0) * PW)
        if j < 3:
            return [pltpu.make_async_copy(w_hbm[j].at[rows, :], stage.at[j, rows, :], sem)]
        return [pltpu.make_async_copy(w_hbm[j].at[rows, pl.ds(c * 128, 128)], wob.at[c, rows, :], sem)
                for c in range(5)]

    cps = {'m': [pltpu.make_async_copy(mem0_hbm, mem0, sem_in.at[0])] + cp_x(0, sem_in.at[0])}
    for g, (qkv, wo_, xc) in enumerate(GROUPS):
        sem = sem_in.at[1 + g]
        cps['g', g] = []
        if qkv:
            cps['g', g] += [c for j in range(3) for c in cp_rows(j, *qkv, sem)]
        if wo_:
            cps['g', g] += cp_rows(3, *wo_, sem)
        for i in xc:
            cps['g', g] += cp_x(i, sem)
    for i, (src_ref, dst_ref, nt) in enumerate(((w1_hbm, w1b, 5), (w2_hbm, w2b, 5), (w3_hbm, w3b, 12),
                                                (w4_hbm, w4b, 5))):
        cps['w', i] = cp_w(src_ref, dst_ref, nt, sem_in.at[1 + len(GROUPS) + i])
    queue = list(cps)
    pos = {'started': 0, 'done': 0}

    def top_up(limit=DMA_DEPTH):
        while pos['started'] < min(len(queue), pos['done'] + limit):
            for c in cps[queue[pos['started']]]:
                c.start()
            pos['started'] += 1

    def arrive(key):
        assert key == queue[pos['done']]
        for c in cps[key]:
            c.wait()
        pos['done'] += 1
        top_up()

    top_up(2)
    wo, w1, w2, w3, w4 = (r.bitcast(U32) for r in (wob, w1b, w2b, w3b, w4b))

    z8 = jnp.zeros((8, DM), F32)
    hbuf[pl.ds(0, 8), :] = z8
    hbuf[pl.ds(8 + S_TOT, 8), :] = z8
    arrive('m')

    def ln0(i):
        for r in range(XCH[i][0], XCH[i][1], SEG):
            xv = xin[pl.ds(r, SEG), :].astype(F32)
            xbuf[pl.ds(r, SEG), :] = xv
            ybuf[pl.ds(r, SEG), :] = _ln(xv)
    ln0(0)

    row = jax.lax.broadcasted_iota(jnp.int32, (L, 128), 0)
    lane = jax.lax.broadcasted_iota(jnp.int32, (L, 128), 1)
    NEG = np.float32(-1e30)
    MASKED = np.float32(-1e9 * LOG2E)
    realA = lane < L
    realB = (lane >= 64) & (lane < 64 + L)
    validA = realA & ((row < MEM) | (row >= lane))
    validB = realB & ((row < MEM) | (row >= lane - 64))
    valid = validA | validB
    fill = jnp.where(realA | realB, MASKED, NEG)
    isA = lane < 64
    SC = np.float32(DH ** -0.5 * LOG2E)
    lane48 = jax.lax.broadcasted_iota(jnp.int32, (48, 128), 1)
    lo48 = lane48 < 64

    def blk(t):
        tb = jnp.concatenate([t, jnp.zeros((8, PW), F32)], axis=0).astype(BF16)
        t0 = tb[:, 0:128]
        t1 = tb[:, 128:256]
        t2 = tb[:, 256:384]
        z16 = jnp.zeros((16, 128), BF16)
        z64 = jnp.zeros((64, 128), BF16)
        z80 = jnp.zeros((80, 128), BF16)
        zb = jnp.zeros((48, 128), BF16)
        c0 = jnp.concatenate([t0, z80], axis=0)
        c1 = jnp.concatenate([jnp.where(lo48, t1, zb), z16, jnp.where(lo48, zb, t1), z16], axis=0)
        c2 = jnp.concatenate([z64, t2, z16], axis=0)
        return jnp.concatenate([c0, c1, c2], axis=1)

    def run(sched, rA=None, mem=None, rB1=None, rB2=None, y=None, yPre=None, short=None, nB=SEG, final=False):
        st = {}
        if rA is not None and sched is not SCHED_0:
            yv = ybuf[pl.ds(y[0], y[1]), :] if isinstance(y, tuple) else y
            st['h'] = jnp.concatenate([mem, yv], axis=0)

        def f_pre(_):
            st['ypre'] = ybuf[pl.ds(yPre[0], yPre[1]), :]

        def f_wq(g):
            arrive(('g', g))

        def f_tr(pjc):
            p, j, c = pjc
            for m in range(5):
                blk_ = stage[j, pl.ds(p * PW + c * 128, 128), pl.ds(m * 128, 128)]
                wqkv[p, 3 * j + c, pl.ds(m * 64, 64), :] = pltpu.bitcast(blk_.T, U32)

        def f_bw(i):
            arrive(('w', i))

        def split_qkv(p, qkv):
            st['q', p] = qkv[:, 0:PW]
            st['k', p] = blk(qkv[:, PW:2 * PW])
            st['v', p] = blk(qkv[:, 2 * PW:3 * PW])

        def f_qkv0(pcj):
            p, c, j = pcj
            if c == 0:
                lhs = jnp.concatenate([mem, ybuf[pl.ds(0, C0 - MEM), :]], axis=0)
            else:
                lhs = ybuf[pl.ds(c * C0 - MEM, C0), :]
            res = _dot(lhs, _wload(wqkv.at[p, pl.ds(3 * j, 3)], 3))
            col = p * QW + j * PW
            if c == 0:
                st['qkv'[j], p] = res[0:L] if j == 0 else blk(res[0:L])
                ring[pl.ds(SEG, C0 - L), col:col + PW] = res[L:]
            else:
                ring[pl.ds(c * C0 - MEM, C0), col:col + PW] = res

        def f_qkv(p):
            res = _dot(st['h'], _wload(wqkv.at[p], 9))
            if short is not None:
                groups, rseg = short
                for g in range(SH // 8):
                    ring[pl.ds(groups[g], 8), p * QW:(p + 1) * QW] = res[MEM + 8 * g:MEM + 8 * g + 8]
                res = jnp.concatenate([res[0:MEM], ring[pl.ds(rseg, SEG), p * QW:(p + 1) * QW]], axis=0)
            split_qkv(p, res)

        def f_s(p):
            t = _dot_nt(st['q', p], st['k', p]) * SC
            s = jnp.where(valid, t, fill)
            mA = jnp.max(jnp.where(isA, s, NEG), axis=-1, keepdims=True)
            mB = jnp.max(jnp.where(isA, NEG, s), axis=-1, keepdims=True)
            e = jnp.exp2(s - jnp.where(isA, mA, mB))
            lA = jnp.sum(jnp.where(isA, e, 0.0), axis=-1, keepdims=True)
            lB = jnp.sum(jnp.where(isA, 0.0, e), axis=-1, keepdims=True)
            l = jnp.where(isA, lA, lB)
            r = pl.reciprocal(l, approx=True)
            r = r * (2.0 - l * r)
            st['p', p] = e * r

        def f_pv(p):
            st['o', p] = _dot(st['p', p], st['v', p])

        def f_o(p):
            c = _dot(st['o', p], _wload(wo, 5, p * PW, PW))
            st['acc'] = c if 'acc' not in st else st['acc'] + c

        def f_fin(_):
            acc = st['acc']
            xbuf[pl.ds(rA, SEG), :] = xbuf[pl.ds(rA, SEG), :] + acc[MEM:, :]
            st['mem'] = acc[0:MEM, :]

        def f_b1(_):
            x1 = xbuf[pl.ds(rB1, SEG), :]
            y = _ln(x1)
            ybuf[pl.ds(rB1, SEG), :] = y
            hbuf[pl.ds(rB1 + 8, SEG), :] = _gelu(_dot(_ln(y), _wload(w1, 5)))

        def f_b2a(_):
            lane_h = jax.lax.broadcasted_iota(jnp.int32, (nB, 128), 1)

            def sh(j, d):
                win = hbuf[pl.ds(rB2, nB + 16), j * 128:(j + 1) * 128]
                return win[8 + d:8 + d + nB, :]
            cols = [
                sh(0, -1),
                jnp.where(lane_h < 32, sh(1, -1), sh(1, 1)),
                jnp.where(lane_h < 64, sh(2, 1), sh(2, -2)),
                jnp.where(lane_h < 96, sh(3, -2), sh(3, 2)),
                sh(4, 2),
            ]
            hs_in = jnp.concatenate(cols, axis=1)
            st['y1'] = ybuf[pl.ds(rB2, nB), :] + _dot(hs_in, _wload(w2, 5))

        def f_b2b(_):
            st['g'] = _gelu(_dot(_ln(st['y1']), _wload(w3, 12)))

        def f_b2c(i):
            kc = FF // NB2C
            c = _dot(st['g'][:, i * kc:(i + 1) * kc], _wload(w4, 5, i * kc, kc))
            st['h2'] = c if 'h2' not in st else st['h2'] + c

        def f_b2d(_):
            xn = xbuf[pl.ds(rB2, nB), :] + (st['y1'] + st['h2'])
            if not final:
                xbuf[pl.ds(rB2, nB), :] = xn
                ybuf[pl.ds(rB2, nB), :] = _ln(xn)
            obuf[pl.ds(rB2, nB), :] = xn.astype(BF16)

        fs = {'q': f_qkv, 'q0': f_qkv0, 's': f_s, 'v': f_pv, 'o': f_o, 'fin': f_fin, 'b1': f_b1, 'b2a': f_b2a,
              'b2b': f_b2b, 'b2c': f_b2c, 'b2d': f_b2d, 'wq': f_wq, 'tr': f_tr, 'bw': f_bw, 'ln0': ln0,
              'pre': f_pre}
        for op, p in sched:
            fs[op](p)
        return st.get('mem'), st.get('ypre')

    def seg_row(t):
        return pl.multiple_of((t & (NSEG - 1)) * SEG, SEG)

    def new_rows(t):
        return R0 + SH * (t - 1)

    with _scope("step0"):
        mem, _ = run(SCHED_0, rA=0, mem=mem0[...].astype(F32))
    with _scope("step1"):
        mem, _ = run(SCHED_1, rA=SEG, mem=mem, rB1=0, y=(new_rows(1), SH),
                     short=([(new_rows(1) + 8 * g) % RING for g in range(SH // 8)], SEG))

    def short_body(u, mem, first=False):
        t0 = 2 * u + 2
        y = (pl.multiple_of(new_rows(t0), 8), SH)
        for k in range(2):
            t = t0 + k
            groups = [pl.multiple_of(jax.lax.rem(new_rows(t) + 8 * g, RING), 8) for g in range(SH // 8)]
            rseg = pl.multiple_of(jax.lax.rem(t * SEG, RING), SEG)
            mem, y = run(SCHED_SB if k else (SCHED_S2 if first else SCHED_SA), rA=seg_row(t), mem=mem, rB1=seg_row(t - 1), rB2=seg_row(t - 2),
                         y=y, yPre=None if k else (pl.multiple_of(new_rows(t + 1), 8), SH), short=(groups, rseg))
        return mem

    with _scope("short"):
        mem = short_body(jnp.int32(0), mem, first=True)
        mem = jax.lax.fori_loop(1, (TS - 2) // 2, short_body, mem)

    def body(u, mem):
        t0 = 2 * u + TS
        y = (seg_row(t0), SEG)
        mem = jnp.where(t0 == NSEG, mem0[...].astype(F32), mem)
        for k in range(2):
            t = t0 + k
            mem, y = run(SCHED_B if k else SCHED_A, rA=seg_row(t), mem=mem, rB1=seg_row(t - 1), rB2=seg_row(t - 2),
                         y=y, yPre=None if k else (seg_row(t + 1), SEG))

        @pl.when(t0 >= NSEG + 2)
        def _():
            r = pl.multiple_of((t0 - NSEG - 2) * SEG, 2 * SEG)
            pltpu.make_async_copy(obuf.at[pl.ds(r, 2 * SEG), :], out_hbm.at[pl.ds(r, 2 * SEG), :], sem_out.at[0]).start()
        return mem

    with _scope("main"):
        jax.lax.fori_loop(0, (2 * NSEG - TS) // 2, body, mem)

    with _scope("epi"):
        r63 = (NSEG - 1) * SEG
        r62 = (NSEG - 2) * SEG
        run([('b1', 0)] + SCHED_E, rB1=r63, rB2=r62, nB=2 * SEG, final=True)
        pltpu.make_async_copy(obuf.at[pl.ds(r62, 2 * SEG), :], out_hbm.at[pl.ds(r62, 2 * SEG), :], sem_out.at[0]).start()
        pltpu.make_async_copy(obuf.at[pl.ds(0, S_TOT), :], out_hbm, sem_out.at[0]).wait()


@jax.jit
def pallas_interleave_layers__memory_aug_recurrent_mem_tr__mixer_s_mlp__prompt_kernel(A_x, A_mem0, A_Wq, A_Wk, A_Wv, A_Wo, A_seg_len, B_x, B_w1, B_w2, B_w3, B_w4):
    del A_seg_len, B_x
    x2 = A_x.reshape(S_TOT, DM)
    m2 = A_mem0.reshape(MEM, DM)
    wqT = A_Wq.transpose(1, 2, 0).reshape(HD, DM)
    wkT = A_Wk.transpose(1, 2, 0).reshape(HD, DM)
    wvT = A_Wv.transpose(1, 2, 0).reshape(HD, DM)
    wo2 = A_Wo.reshape(HD, DM)
    any_spec = pl.BlockSpec(memory_space=pl.ANY)
    out = pl.pallas_call(
        _kernel,
        out_shape=jax.ShapeDtypeStruct((S_TOT, DM), BF16),
        in_specs=[any_spec] * 10,
        out_specs=any_spec,
        scratch_shapes=[
            pltpu.VMEM((NP, 9, DM // 2, 128), U32),
            pltpu.VMEM((5, HD, 128), BF16),
            pltpu.VMEM((RING, NP * QW), F32),
            pltpu.VMEM((5, DM, 128), BF16),
            pltpu.VMEM((5, DM, 128), BF16),
            pltpu.VMEM((12, DM, 128), BF16),
            pltpu.VMEM((5, FF, 128), BF16),
            pltpu.VMEM((S_TOT + 64, DM), F32),
            pltpu.VMEM((S_TOT + 64, DM), F32),
            pltpu.VMEM((S_TOT + 64, DM), F32),
            pltpu.VMEM((S_TOT + 64, DM), BF16),
            pltpu.VMEM((3, HD, DM), BF16),
            pltpu.VMEM((S_TOT, DM), BF16),
            pltpu.VMEM((MEM, DM), BF16),
            pltpu.SemaphoreType.DMA((len(GROUPS) + 5,)),
            pltpu.SemaphoreType.DMA((1,)),
        ],
        compiler_params=pltpu.CompilerParams(vmem_limit_bytes=120 * 1024 * 1024),
    )(x2, m2, wqT, wkT, wvT, wo2, B_w1, B_w2, B_w3, B_w4)
    return out.reshape(1, S_TOT, DM)
```

```python
import contextlib
import jax
import jax.numpy as jnp
import numpy as np
import jax.experimental.pallas as pl
import jax.experimental.pallas.tpu as pltpu

F32 = jnp.float32
BF16 = jnp.bfloat16
U32 = jnp.uint32

S_TOT = 2048
DM = 640
NH = 32
DH = 192
HD = NH * DH
MEM = 8
SEG = 32
NSEG = S_TOT // SEG
L = MEM + SEG
NP = NH // 2
PW = 2 * DH
QW = 3 * PW
FF = 1536
LOG2E = 1.4426950408889634
SCOPES = False
NB2C = 4

SH = 24
R0 = 344
TS = (R0 - SH) // (SEG - SH)
RING = (R0 + 31) // 32 * 32
C0 = (R0 + MEM) // 4
XCH = [(0, RING), (RING, 512)] + [(r, r + 256) for r in range(512, S_TOT, 256)]
DMA_DEPTH = 3
GROUPS = [((0, 1), None, ()), ((1, 2), None, ()), ((2, 3), None, ()), ((3, 4), None, ()), ((4, 5), None, ()),
          ((5, 6), None, (1,)), ((6, 7), None, ()), ((7, 9), None, (2, 3)), ((9, 11), None, (4, 5)),
          ((11, 13), None, (6,)), ((13, 16), None, (7,)),
          (None, (0, 4), ()), (None, (4, 8), ()), (None, (8, 12), ()), (None, (12, 16), ())]
BAR_POS = {1: 7, 2: 3}
O_SLOTS = {11: (13, 6), 12: (15, 0)}


def _make_sched(lag_s=1, lag_v=2, lag_o=5, order='qsov'):
    ops = []
    i = 0
    done_o = 0
    while done_o < NP:
        for o in order:
            j = i - {'q': 0, 's': lag_s, 'o': lag_o, 'v': lag_v}[o]
            if 0 <= j < NP:
                ops.append((o, j))
                done_o += o == 'o'
        i += 1
    ops.append(('fin', 0))
    return ops


def _place(ops, places):
    out = []
    pl_ = {a: l for a, l in places}
    for o in ops:
        out.append(o)
        for b in pl_.get(o, ()):
            out.append(b if isinstance(b, tuple) else (b, 0))
    return out


def _sched0():
    first = {q[0]: g for g, (q, _, _) in enumerate(GROUPS) if q}
    ops = [('wq', 0)]
    tr = [('tr', (0, j, c)) for j in range(3) for c in range(3)]
    todo_x, todo_o = [], []
    for i in range(NP + 2):
        mm = [('q0', (i, c, j)) for c in range(4) for j in range(3)] if i < NP else []
        for k in range(12):
            if mm:
                if k < 3:
                    while tr and tr[0][1][:2] <= (i, k):
                        ops.append(tr.pop(0))
                ops.append(mm[k])
            if i + 1 < NP and k == BAR_POS.get(i + 1, 0):
                if i + 1 in first:
                    g = first[i + 1]
                    ops.append(('wq', g))
                    todo_x += list(GROUPS[g][2])
                tr += [('tr', (i + 1, j, c)) for j in range(3) for c in range(3)]
            if tr:
                ops.append(tr.pop(0))
            if k == 2 and 0 <= i - 1 < NP:
                ops.append(('s', i - 1))
            if k == 5 and 0 <= i - 2 < NP:
                ops.append(('v', i - 2))
            for g, pos_ in O_SLOTS.items():
                if pos_ == (i, k):
                    ops.append(('wq', g))
                    todo_o += list(range(*GROUPS[g][1]))
            if todo_o and k in (3, 4, 7, 8, 10, 11) and todo_o[0] <= i - 3:
                ops.append(('o', todo_o.pop(0)))
            if todo_x and k == 9:
                ops.append(('ln0', todo_x.pop(0)))
    assert not tr and not todo_x
    ops += [('o', p) for p in todo_o]
    for g, (q, wo_, _) in enumerate(GROUPS):
        if not q and g not in O_SLOTS:
            ops += [('wq', g)] + [('o', p) for p in range(*wo_)]
    ops.append(('fin', 0))
    return ops


SCHED_0 = _sched0()
SCHED_1 = _place(_make_sched(lag_o=7), [(('q', 4), [('bw', 0)]), (('s', 15), ['b1'])])
SCHED_A = _place(_make_sched(lag_s=1, lag_v=3, lag_o=5, order='qsvo'),
                 [(('q', 1), ['b1']), (('q', 4), ['b2a']), (('q', 9), ['b2b']), (('q', 12), [('b2c', 0)]),
                  (('v', 13), [('b2c', 1)]), (('o', 13), ['pre', ('b2c', 2)]), (('fin', 0), [('b2c', 3), 'b2d'])])
SCHED_B = _place(_make_sched(lag_s=1, lag_v=3, lag_o=5, order='qvso'),
                 [(('q', 3), ['b1']), (('q', 6), ['b2a']), (('q', 11), ['b2b']),
                  (('s', 15), [('b2c', 0), ('b2c', 1)]), (('v', 14), [('b2c', 2), ('b2c', 3), 'b2d'])])
SCHED_SA = _place(_make_sched(lag_s=2, lag_v=3, lag_o=7, order='sqov'),
                  [(('q', 1), ['b1']), (('q', 5), ['b2a']), (('q', 8), ['b2b']), (('q', 14), [('b2c', 0)]),
                   (('o', 10), ['pre', ('b2c', 1)]), (('o', 13), [('b2c', 2)]), (('fin', 0), [('b2c', 3), 'b2d'])])
SCHED_SB = _place(_make_sched(lag_s=1, lag_v=3, lag_o=6, order='qvso'),
                  [(('q', 1), ['b1']), (('q', 3), ['b2a']), (('q', 7), ['b2b']), (('q', 13), [('b2c', 0)]),
                   (('q', 14), [('b2c', 1)]), (('s', 15), [('b2c', 2)]), (('v', 15), [('b2c', 3), 'b2d'])])
SCHED_S2 = []
for _op in SCHED_SA:
    if _op[0] in ('b2a', 'b2b') or _op == ('b2c', 0):
        SCHED_S2.append(('bw', {'b2a': 1, 'b2b': 2, 'b2c': 3}[_op[0]]))
    SCHED_S2.append(_op)
SCHED_E = [('b2a', 0), ('b2b', 0)] + [('b2c', i) for i in range(NB2C)] + [('b2d', 0)]


def _ln(x, eps=1e-5):
    m = jnp.mean(x, axis=-1, keepdims=True)
    xc = x - m
    v = jnp.mean(xc * xc, axis=-1, keepdims=True)
    return xc * jax.lax.rsqrt(v + eps)


def _gelu(x):
    return jax.nn.gelu(x, approximate=True)


def _dot(a, b):
    return jnp.dot(a, b, preferred_element_type=F32)


def _dot_nt(a, b):
    return jax.lax.dot_general(a, b, (((1,), (1,)), ((), ())), preferred_element_type=F32)


def _scope(name):
    return jax.named_scope(name) if SCOPES else contextlib.nullcontext()


def _wload(ref, ntile, k0=0, kn=None):
    if kn is None:
        return jnp.concatenate([pltpu.bitcast(ref[c], BF16) for c in range(ntile)], axis=1)
    return jnp.concatenate([pltpu.bitcast(ref[c, pl.ds(k0 // 2, kn // 2), :], BF16) for c in range(ntile)], axis=1)


def _kernel(x_hbm, mem0_hbm, wq_hbm, wk_hbm, wv_hbm, wo_hbm, w1_hbm, w2_hbm, w3_hbm, w4_hbm,
            out_hbm,
            wqkv, wob, ring, w1b, w2b, w3b, w4b, xbuf, ybuf, hbuf, obuf, stage, xin, mem0,
            sem_in, sem_out):
    w_hbm = (wq_hbm, wk_hbm, wv_hbm, wo_hbm)
    def cp_x(i, sem):
        r0, r1 = XCH[i]
        return [pltpu.make_async_copy(x_hbm.at[pl.ds(r0, r1 - r0), :], xin.at[pl.ds(r0, r1 - r0), :], sem)]

    def cp_w(src_ref, dst_ref, ntile, sem):
        return [pltpu.make_async_copy(src_ref.at[:, pl.ds(c * 128, 128)], dst_ref.at[c], sem) for c in range(ntile)]

    def cp_rows(j, p0, p1, sem):
        rows = pl.ds(p0 * PW, (p1 - p0) * PW)
        if j < 3:
            return [pltpu.make_async_copy(w_hbm[j].at[rows, :], stage.at[j, rows, :], sem)]
        return [pltpu.make_async_copy(w_hbm[j].at[rows, pl.ds(c * 128, 128)], wob.at[c, rows, :], sem)
                for c in range(5)]

    cps = {'m': [pltpu.make_async_copy(mem0_hbm, mem0, sem_in.at[0])] + cp_x(0, sem_in.at[0])}
    for g, (qkv, wo_, xc) in enumerate(GROUPS):
        sem = sem_in.at[1 + g]
        cps['g', g] = []
        if qkv:
            cps['g', g] += [c for j in range(3) for c in cp_rows(j, *qkv, sem)]
        if wo_:
            cps['g', g] += cp_rows(3, *wo_, sem)
        for i in xc:
            cps['g', g] += cp_x(i, sem)
    for i, (src_ref, dst_ref, nt) in enumerate(((w1_hbm, w1b, 5), (w2_hbm, w2b, 5), (w3_hbm, w3b, 12),
                                                (w4_hbm, w4b, 5))):
        cps['w', i] = cp_w(src_ref, dst_ref, nt, sem_in.at[1 + len(GROUPS) + i])
    queue = list(cps)
    pos = {'started': 0, 'done': 0}

    def top_up(limit=DMA_DEPTH):
        while pos['started'] < min(len(queue), pos['done'] + limit):
            for c in cps[queue[pos['started']]]:
                c.start()
            pos['started'] += 1

    def arrive(key):
        assert key == queue[pos['done']]
        for c in cps[key]:
            c.wait()
        pos['done'] += 1
        top_up()

    top_up(2)
    wo, w1, w2, w3, w4 = (r.bitcast(U32) for r in (wob, w1b, w2b, w3b, w4b))

    z8 = jnp.zeros((8, DM), F32)
    hbuf[pl.ds(0, 8), :] = z8
    hbuf[pl.ds(8 + S_TOT, 8), :] = z8
    arrive('m')

    def ln0(i):
        for r in range(XCH[i][0], XCH[i][1], SEG):
            xv = xin[pl.ds(r, SEG), :].astype(F32)
            xbuf[pl.ds(r, SEG), :] = xv
            ybuf[pl.ds(r, SEG), :] = _ln(xv)
    ln0(0)

    row = jax.lax.broadcasted_iota(jnp.int32, (L, 128), 0)
    lane = jax.lax.broadcasted_iota(jnp.int32, (L, 128), 1)
    NEG = np.float32(-1e30)
    MASKED = np.float32(-1e9 * LOG2E)
    realA = lane < L
    realB = (lane >= 64) & (lane < 64 + L)
    validA = realA & ((row < MEM) | (row >= lane))
    validB = realB & ((row < MEM) | (row >= lane - 64))
    valid = validA | validB
    fill = jnp.where(realA | realB, MASKED, NEG)
    isA = lane < 64
    SC = np.float32(DH ** -0.5 * LOG2E)
    lane48 = jax.lax.broadcasted_iota(jnp.int32, (48, 128), 1)
    lo48 = lane48 < 64

    def blk(t):
        tb = jnp.concatenate([t, jnp.zeros((8, PW), F32)], axis=0).astype(BF16)
        t0 = tb[:, 0:128]
        t1 = tb[:, 128:256]
        t2 = tb[:, 256:384]
        z16 = jnp.zeros((16, 128), BF16)
        z64 = jnp.zeros((64, 128), BF16)
        z80 = jnp.zeros((80, 128), BF16)
        zb = jnp.zeros((48, 128), BF16)
        c0 = jnp.concatenate([t0, z80], axis=0)
        c1 = jnp.concatenate([jnp.where(lo48, t1, zb), z16, jnp.where(lo48, zb, t1), z16], axis=0)
        c2 = jnp.concatenate([z64, t2, z16], axis=0)
        return jnp.concatenate([c0, c1, c2], axis=1)

    def run(sched, rA=None, mem=None, rB1=None, rB2=None, y=None, yPre=None, short=None, nB=SEG, final=False):
        st = {}
        if rA is not None and sched is not SCHED_0:
            yv = ybuf[pl.ds(y[0], y[1]), :] if isinstance(y, tuple) else y
            st['h'] = jnp.concatenate([mem, yv], axis=0)

        def f_pre(_):
            st['ypre'] = ybuf[pl.ds(yPre[0], yPre[1]), :]

        def f_wq(g):
            arrive(('g', g))

        def f_tr(pjc):
            p, j, c = pjc
            for m in range(5):
                blk_ = stage[j, pl.ds(p * PW + c * 128, 128), pl.ds(m * 128, 128)]
                wqkv[p, 3 * j + c, pl.ds(m * 64, 64), :] = pltpu.bitcast(blk_.T, U32)

        def f_bw(i):
            arrive(('w', i))

        def split_qkv(p, qkv):
            st['q', p] = qkv[:, 0:PW]
            st['k', p] = blk(qkv[:, PW:2 * PW])
            st['v', p] = blk(qkv[:, 2 * PW:3 * PW])

        def f_qkv0(pcj):
            p, c, j = pcj
            if c == 0:
                lhs = jnp.concatenate([mem, ybuf[pl.ds(0, C0 - MEM), :]], axis=0)
            else:
                lhs = ybuf[pl.ds(c * C0 - MEM, C0), :]
            res = _dot(lhs, _wload(wqkv.at[p, pl.ds(3 * j, 3)], 3))
            col = p * QW + j * PW
            if c == 0:
                st['qkv'[j], p] = res[0:L] if j == 0 else blk(res[0:L])
                ring[pl.ds(SEG, C0 - L), col:col + PW] = res[L:]
            else:
                ring[pl.ds(c * C0 - MEM, C0), col:col + PW] = res

        def f_qkv(p):
            res = _dot(st['h'], _wload(wqkv.at[p], 9))
            if short is not None:
                groups, rseg = short
                for g in range(SH // 8):
                    ring[pl.ds(groups[g], 8), p * QW:(p + 1) * QW] = res[MEM + 8 * g:MEM + 8 * g + 8]
                res = jnp.concatenate([res[0:MEM], ring[pl.ds(rseg, SEG), p * QW:(p + 1) * QW]], axis=0)
            split_qkv(p, res)

        def f_s(p):
            t = _dot_nt(st['q', p], st['k', p]) * SC
            s = jnp.where(valid, t, fill)
            mA = jnp.max(jnp.where(isA, s, NEG), axis=-1, keepdims=True)
            mB = jnp.max(jnp.where(isA, NEG, s), axis=-1, keepdims=True)
            e = jnp.exp2(s - jnp.where(isA, mA, mB))
            lA = jnp.sum(jnp.where(isA, e, 0.0), axis=-1, keepdims=True)
            lB = jnp.sum(jnp.where(isA, 0.0, e), axis=-1, keepdims=True)
            l = jnp.where(isA, lA, lB)
            r = pl.reciprocal(l, approx=True)
            r = r * (2.0 - l * r)
            st['p', p] = e * r

        def f_pv(p):
            st['o', p] = _dot(st['p', p], st['v', p])

        def f_o(p):
            c = _dot(st['o', p], _wload(wo, 5, p * PW, PW))
            st['acc'] = c if 'acc' not in st else st['acc'] + c

        def f_fin(_):
            acc = st['acc']
            xbuf[pl.ds(rA, SEG), :] = xbuf[pl.ds(rA, SEG), :] + acc[MEM:, :]
            st['mem'] = acc[0:MEM, :]

        def f_b1(_):
            x1 = xbuf[pl.ds(rB1, SEG), :]
            y = _ln(x1)
            ybuf[pl.ds(rB1, SEG), :] = y
            hbuf[pl.ds(rB1 + 8, SEG), :] = _gelu(_dot(_ln(y), _wload(w1, 5)))

        def f_b2a(_):
            lane_h = jax.lax.broadcasted_iota(jnp.int32, (nB, 128), 1)

            def sh(j, d):
                win = hbuf[pl.ds(rB2, nB + 16), j * 128:(j + 1) * 128]
                return win[8 + d:8 + d + nB, :]
            cols = [
                sh(0, -1),
                jnp.where(lane_h < 32, sh(1, -1), sh(1, 1)),
                jnp.where(lane_h < 64, sh(2, 1), sh(2, -2)),
                jnp.where(lane_h < 96, sh(3, -2), sh(3, 2)),
                sh(4, 2),
            ]
            hs_in = jnp.concatenate(cols, axis=1)
            st['y1'] = ybuf[pl.ds(rB2, nB), :] + _dot(hs_in, _wload(w2, 5))

        def f_b2b(_):
            st['g'] = _gelu(_dot(_ln(st['y1']), _wload(w3, 12)))

        def f_b2c(i):
            kc = FF // NB2C
            c = _dot(st['g'][:, i * kc:(i + 1) * kc], _wload(w4, 5, i * kc, kc))
            st['h2'] = c if 'h2' not in st else st['h2'] + c

        def f_b2d(_):
            xn = xbuf[pl.ds(rB2, nB), :] + (st['y1'] + st['h2'])
            if not final:
                xbuf[pl.ds(rB2, nB), :] = xn
                ybuf[pl.ds(rB2, nB), :] = _ln(xn)
            obuf[pl.ds(rB2, nB), :] = xn.astype(BF16)

        fs = {'q': f_qkv, 'q0': f_qkv0, 's': f_s, 'v': f_pv, 'o': f_o, 'fin': f_fin, 'b1': f_b1, 'b2a': f_b2a,
              'b2b': f_b2b, 'b2c': f_b2c, 'b2d': f_b2d, 'wq': f_wq, 'tr': f_tr, 'bw': f_bw, 'ln0': ln0,
              'pre': f_pre}
        for op, p in sched:
            fs[op](p)
        return st.get('mem'), st.get('ypre')

    def seg_row(t):
        return pl.multiple_of((t & (NSEG - 1)) * SEG, SEG)

    def new_rows(t):
        return R0 + SH * (t - 1)

    with _scope("step0"):
        mem, _ = run(SCHED_0, rA=0, mem=mem0[...].astype(F32))
    with _scope("step1"):
        mem, _ = run(SCHED_1, rA=SEG, mem=mem, rB1=0, y=(new_rows(1), SH),
                     short=([(new_rows(1) + 8 * g) % RING for g in range(SH // 8)], SEG))

    def short_body(u, mem, first=False):
        t0 = 2 * u + 2
        y = (pl.multiple_of(new_rows(t0), 8), SH)
        for k in range(2):
            t = t0 + k
            groups = [pl.multiple_of(jax.lax.rem(new_rows(t) + 8 * g, RING), 8) for g in range(SH // 8)]
            rseg = pl.multiple_of(jax.lax.rem(t * SEG, RING), SEG)
            mem, y = run(SCHED_SB if k else (SCHED_S2 if first else SCHED_SA), rA=seg_row(t), mem=mem, rB1=seg_row(t - 1), rB2=seg_row(t - 2),
                         y=y, yPre=None if k else (pl.multiple_of(new_rows(t + 1), 8), SH), short=(groups, rseg))
        return mem

    with _scope("short"):
        mem = short_body(jnp.int32(0), mem, first=True)
        mem = jax.lax.fori_loop(1, (TS - 2) // 2, short_body, mem)

    def body(u, mem):
        t0 = 2 * u + TS
        y = (seg_row(t0), SEG)
        mem = jnp.where(t0 == NSEG, mem0[...].astype(F32), mem)
        for k in range(2):
            t = t0 + k
            mem, y = run(SCHED_B if k else SCHED_A, rA=seg_row(t), mem=mem, rB1=seg_row(t - 1), rB2=seg_row(t - 2),
                         y=y, yPre=None if k else (seg_row(t + 1), SEG))

        @pl.when(t0 >= NSEG + 2)
        def _():
            r = pl.multiple_of((t0 - NSEG - 2) * SEG, 2 * SEG)
            pltpu.make_async_copy(obuf.at[pl.ds(r, 2 * SEG), :], out_hbm.at[pl.ds(r, 2 * SEG), :], sem_out.at[0]).start()
        return mem

    with _scope("main"):
        jax.lax.fori_loop(0, (2 * NSEG - TS) // 2, body, mem)

    with _scope("epi"):
        r63 = (NSEG - 1) * SEG
        r62 = (NSEG - 2) * SEG
        run([('b1', 0)] + SCHED_E, rB1=r63, rB2=r62, nB=2 * SEG, final=True)
        pltpu.make_async_copy(obuf.at[pl.ds(r62, 2 * SEG), :], out_hbm.at[pl.ds(r62, 2 * SEG), :], sem_out.at[0]).start()
        pltpu.make_async_copy(obuf.at[pl.ds(0, S_TOT), :], out_hbm, sem_out.at[0]).wait()


@jax.jit
def pallas_interleave_layers__memory_aug_recurrent_mem_tr__mixer_s_mlp__prompt_kernel(A_x, A_mem0, A_Wq, A_Wk, A_Wv, A_Wo, A_seg_len, B_x, B_w1, B_w2, B_w3, B_w4):
    del A_seg_len, B_x
    x2 = A_x.reshape(S_TOT, DM)
    m2 = A_mem0.reshape(MEM, DM)
    wqT = A_Wq.transpose(1, 2, 0).reshape(HD, DM)
    wkT = A_Wk.transpose(1, 2, 0).reshape(HD, DM)
    wvT = A_Wv.transpose(1, 2, 0).reshape(HD, DM)
    wo2 = A_Wo.reshape(HD, DM)
    any_spec = pl.BlockSpec(memory_space=pl.ANY)
    out = pl.pallas_call(
        _kernel,
        out_shape=jax.ShapeDtypeStruct((S_TOT, DM), BF16),
        in_specs=[any_spec] * 10,
        out_specs=any_spec,
        scratch_shapes=[
            pltpu.VMEM((NP, 9, DM // 2, 128), U32),
            pltpu.VMEM((5, HD, 128), BF16),
            pltpu.VMEM((RING, NP * QW), F32),
            pltpu.VMEM((5, DM, 128), BF16),
            pltpu.VMEM((5, DM, 128), BF16),
            pltpu.VMEM((12, DM, 128), BF16),
            pltpu.VMEM((5, FF, 128), BF16),
            pltpu.VMEM((S_TOT + 64, DM), F32),
            pltpu.VMEM((S_TOT + 64, DM), F32),
            pltpu.VMEM((S_TOT + 64, DM), F32),
            pltpu.VMEM((S_TOT + 64, DM), BF16),
            pltpu.VMEM((3, HD, DM), BF16),
            pltpu.VMEM((S_TOT, DM), BF16),
            pltpu.VMEM((MEM, DM), BF16),
            pltpu.SemaphoreType.DMA((len(GROUPS) + 5,)),
            pltpu.SemaphoreType.DMA((1,)),
        ],
        compiler_params=pltpu.CompilerParams(vmem_limit_bytes=120 * 1024 * 1024),
    )(x2, m2, wqT, wkT, wvT, wo2, B_w1, B_w2, B_w3, B_w4)
    return out.reshape(1, S_TOT, DM)
```

```python
import contextlib
import jax
import jax.numpy as jnp
import numpy as np
import jax.experimental.pallas as pl
import jax.experimental.pallas.tpu as pltpu

F32 = jnp.float32
BF16 = jnp.bfloat16
U32 = jnp.uint32

S_TOT = 2048
DM = 640
NH = 32
DH = 192
HD = NH * DH
MEM = 8
SEG = 32
NSEG = S_TOT // SEG
L = MEM + SEG
NP = NH // 2
PW = 2 * DH
QW = 3 * PW
FF = 1536
LOG2E = 1.4426950408889634
SCOPES = False
NB2C = 4

SH = 24
R0 = 344
TS = (R0 - SH) // (SEG - SH)
RING = (R0 + 31) // 32 * 32
C0 = (R0 + MEM) // 4
XCH = [(0, 96), (96, RING), (RING, 512)] + [(r, r + 256) for r in range(512, S_TOT, 256)]
DMA_DEPTH = 3
GROUPS = [((0, 1, 0), None, ()), ((0, 1, 1), None, ()), ((0, 1, 2), None, (1,)),
          ((1, 2), None, ()), ((2, 3), None, ()), ((3, 4), None, ()), ((4, 5), None, ()),
          ((5, 6), None, (2,)), ((6, 7), None, ()), ((7, 9), None, (3, 4)), ((9, 11), None, (5, 6)),
          ((11, 13), None, (7,)), ((13, 16), None, (8,)),
          (None, (0, 4), ()), (None, (4, 8), ()), (None, (8, 12), ()), (None, (12, 16), ())]
BAR_POS = {1: 8, 2: 4, 3: 2}
O_SLOTS = {13: (13, 6), 14: (15, 0)}


def _make_sched(lag_s=1, lag_v=2, lag_o=5, order='qsov'):
    ops = []
    i = 0
    done_o = 0
    while done_o < NP:
        for o in order:
            j = i - {'q': 0, 's': lag_s, 'o': lag_o, 'v': lag_v}[o]
            if 0 <= j < NP:
                ops.append((o, j))
                done_o += o == 'o'
        i += 1
    ops.append(('fin', 0))
    return ops


def _place(ops, places):
    out = []
    pl_ = {a: l for a, l in places}
    for o in ops:
        out.append(o)
        for b in pl_.get(o, ()):
            out.append(b if isinstance(b, tuple) else (b, 0))
    return out


def _sched0():
    first = {q[0]: g for g, (q, _, _) in enumerate(GROUPS) if q}
    ops = []
    tr = [('tr', (0, j, c)) for j in range(3) for c in range(3)]
    todo_x, todo_o = [], []
    for i in range(NP + 2):
        mm = [('q0', (i, c, j)) for c in range(4) for j in range(3)] if i < NP else []
        for k in range(12):
            if mm:
                if i == 0 and k < 3:
                    ops.append(('wq', k))
                    ops += [('ln0', x) for x in GROUPS[k][2]]
                if k < 3:
                    while tr and tr[0][1][:2] <= (i, k):
                        ops.append(tr.pop(0))
                ops.append(mm[k])
            if i + 1 < NP and k == BAR_POS.get(i + 1, 0):
                if i + 1 in first:
                    g = first[i + 1]
                    ops.append(('wq', g))
                    todo_x += list(GROUPS[g][2])
                tr += [('tr', (i + 1, j, c)) for j in range(3) for c in range(3)]
            if tr and not (i == 0 and k < 3):
                ops.append(tr.pop(0))
            if k == 2 and 0 <= i - 1 < NP:
                ops.append(('s', i - 1))
            if k == 5 and 0 <= i - 2 < NP:
                ops.append(('v', i - 2))
            for g, pos_ in O_SLOTS.items():
                if pos_ == (i, k):
                    ops.append(('wq', g))
                    todo_o += list(range(*GROUPS[g][1]))
            if todo_o and k in (3, 4, 7, 8, 10, 11) and todo_o[0] <= i - 3:
                ops.append(('o', todo_o.pop(0)))
            if todo_x and k == 9:
                ops.append(('ln0', todo_x.pop(0)))
    assert not tr and not todo_x
    ops += [('o', p) for p in todo_o]
    for g, (q, wo_, _) in enumerate(GROUPS):
        if not q and g not in O_SLOTS:
            ops += [('wq', g)] + [('o', p) for p in range(*wo_)]
    ops.append(('fin', 0))
    return ops


SCHED_0 = _sched0()
SCHED_1 = _place(_make_sched(lag_o=7), [(('q', 4), [('bw', 0)]), (('s', 15), ['b1'])])
SCHED_A = _place(_make_sched(lag_s=1, lag_v=3, lag_o=5, order='qsvo'),
                 [(('q', 1), ['b1']), (('q', 4), ['b2a']), (('q', 9), ['b2b']), (('q', 12), [('b2c', 0)]),
                  (('v', 13), [('b2c', 1)]), (('o', 13), ['pre', ('b2c', 2)]), (('fin', 0), [('b2c', 3), 'b2d'])])
SCHED_B = _place(_make_sched(lag_s=1, lag_v=3, lag_o=5, order='qvso'),
                 [(('q', 3), ['b1']), (('q', 6), ['b2a']), (('q', 11), ['b2b']),
                  (('s', 15), [('b2c', 0), ('b2c', 1)]), (('v', 14), [('b2c', 2), ('b2c', 3), 'b2d'])])
SCHED_SA = _place(_make_sched(lag_s=2, lag_v=3, lag_o=7, order='sqov'),
                  [(('q', 1), ['b1']), (('q', 5), ['b2a']), (('q', 8), ['b2b']), (('q', 14), [('b2c', 0)]),
                   (('o', 10), ['pre', ('b2c', 1)]), (('o', 13), [('b2c', 2)]), (('fin', 0), [('b2c', 3), 'b2d'])])
SCHED_SB = _place(_make_sched(lag_s=1, lag_v=3, lag_o=6, order='qvso'),
                  [(('q', 1), ['b1']), (('q', 3), ['b2a']), (('q', 7), ['b2b']), (('q', 13), [('b2c', 0)]),
                   (('q', 14), [('b2c', 1)]), (('s', 15), [('b2c', 2)]), (('v', 15), [('b2c', 3), 'b2d'])])
SCHED_S2 = []
for _op in SCHED_SA:
    if _op[0] in ('b2a', 'b2b') or _op == ('b2c', 0):
        SCHED_S2.append(('bw', {'b2a': 1, 'b2b': 2, 'b2c': 3}[_op[0]]))
    SCHED_S2.append(_op)
SCHED_E = [('b2a', 0), ('b2b', 0)] + [('b2c', i) for i in range(NB2C)] + [('b2d', 0)]


def _ln(x, eps=1e-5):
    m = jnp.mean(x, axis=-1, keepdims=True)
    xc = x - m
    v = jnp.mean(xc * xc, axis=-1, keepdims=True)
    return xc * jax.lax.rsqrt(v + eps)


def _gelu(x):
    return jax.nn.gelu(x, approximate=True)


def _dot(a, b):
    return jnp.dot(a, b, preferred_element_type=F32)


def _dot_nt(a, b):
    return jax.lax.dot_general(a, b, (((1,), (1,)), ((), ())), preferred_element_type=F32)


def _scope(name):
    return jax.named_scope(name) if SCOPES else contextlib.nullcontext()


def _wload(ref, ntile, k0=0, kn=None):
    if kn is None:
        return jnp.concatenate([pltpu.bitcast(ref[c], BF16) for c in range(ntile)], axis=1)
    return jnp.concatenate([pltpu.bitcast(ref[c, pl.ds(k0 // 2, kn // 2), :], BF16) for c in range(ntile)], axis=1)


def _kernel(x_hbm, mem0_hbm, wq_hbm, wk_hbm, wv_hbm, wo_hbm, w1_hbm, w2_hbm, w3_hbm, w4_hbm,
            out_hbm,
            wqkv, wob, ring, w1b, w2b, w3b, w4b, xbuf, ybuf, hbuf, obuf, stage, xin, mem0,
            sem_in, sem_out):
    w_hbm = (wq_hbm, wk_hbm, wv_hbm, wo_hbm)
    def cp_x(i, sem):
        r0, r1 = XCH[i]
        return [pltpu.make_async_copy(x_hbm.at[pl.ds(r0, r1 - r0), :], xin.at[pl.ds(r0, r1 - r0), :], sem)]

    def cp_w(src_ref, dst_ref, ntile, sem):
        return [pltpu.make_async_copy(src_ref.at[:, pl.ds(c * 128, 128)], dst_ref.at[c], sem) for c in range(ntile)]

    def cp_rows(j, p0, p1, sem):
        rows = pl.ds(p0 * PW, (p1 - p0) * PW)
        if j < 3:
            return [pltpu.make_async_copy(w_hbm[j].at[rows, :], stage.at[j, rows, :], sem)]
        return [pltpu.make_async_copy(w_hbm[j].at[rows, pl.ds(c * 128, 128)], wob.at[c, rows, :], sem)
                for c in range(5)]

    cps = {'m': [pltpu.make_async_copy(mem0_hbm, mem0, sem_in.at[0])] + cp_x(0, sem_in.at[0])}
    for g, (qkv, wo_, xc) in enumerate(GROUPS):
        sem = sem_in.at[1 + g]
        cps['g', g] = []
        if qkv:
            cps['g', g] += [c for j in (qkv[2:] or range(3)) for c in cp_rows(j, qkv[0], qkv[1], sem)]
        if wo_:
            cps['g', g] += cp_rows(3, *wo_, sem)
        for i in xc:
            cps['g', g] += cp_x(i, sem)
    for i, (src_ref, dst_ref, nt) in enumerate(((w1_hbm, w1b, 5), (w2_hbm, w2b, 5), (w3_hbm, w3b, 12),
                                                (w4_hbm, w4b, 5))):
        cps['w', i] = cp_w(src_ref, dst_ref, nt, sem_in.at[1 + len(GROUPS) + i])
    queue = list(cps)
    pos = {'started': 0, 'done': 0}

    def top_up(limit=DMA_DEPTH):
        while pos['started'] < min(len(queue), pos['done'] + limit):
            for c in cps[queue[pos['started']]]:
                c.start()
            pos['started'] += 1

    def arrive(key):
        assert key == queue[pos['done']]
        for c in cps[key]:
            c.wait()
        pos['done'] += 1
        top_up()

    top_up(3)
    wo, w1, w2, w3, w4 = (r.bitcast(U32) for r in (wob, w1b, w2b, w3b, w4b))

    z8 = jnp.zeros((8, DM), F32)
    hbuf[pl.ds(0, 8), :] = z8
    hbuf[pl.ds(8 + S_TOT, 8), :] = z8
    arrive('m')

    def ln0(i):
        for r in range(XCH[i][0], XCH[i][1], SEG):
            xv = xin[pl.ds(r, SEG), :].astype(F32)
            xbuf[pl.ds(r, SEG), :] = xv
            ybuf[pl.ds(r, SEG), :] = _ln(xv)
    ln0(0)

    row = jax.lax.broadcasted_iota(jnp.int32, (L, 128), 0)
    lane = jax.lax.broadcasted_iota(jnp.int32, (L, 128), 1)
    NEG = np.float32(-1e30)
    MASKED = np.float32(-1e9 * LOG2E)
    realA = lane < L
    realB = (lane >= 64) & (lane < 64 + L)
    validA = realA & ((row < MEM) | (row >= lane))
    validB = realB & ((row < MEM) | (row >= lane - 64))
    valid = validA | validB
    fill = jnp.where(realA | realB, MASKED, NEG)
    isA = lane < 64
    SC = np.float32(DH ** -0.5 * LOG2E)
    lane48 = jax.lax.broadcasted_iota(jnp.int32, (48, 128), 1)
    lo48 = lane48 < 64

    def blk(t):
        tb = jnp.concatenate([t, jnp.zeros((8, PW), F32)], axis=0).astype(BF16)
        t0 = tb[:, 0:128]
        t1 = tb[:, 128:256]
        t2 = tb[:, 256:384]
        z16 = jnp.zeros((16, 128), BF16)
        z64 = jnp.zeros((64, 128), BF16)
        z80 = jnp.zeros((80, 128), BF16)
        zb = jnp.zeros((48, 128), BF16)
        c0 = jnp.concatenate([t0, z80], axis=0)
        c1 = jnp.concatenate([jnp.where(lo48, t1, zb), z16, jnp.where(lo48, zb, t1), z16], axis=0)
        c2 = jnp.concatenate([z64, t2, z16], axis=0)
        return jnp.concatenate([c0, c1, c2], axis=1)

    def run(sched, rA=None, mem=None, rB1=None, rB2=None, y=None, yPre=None, short=None, nB=SEG, final=False):
        st = {}
        if rA is not None and sched is not SCHED_0:
            yv = ybuf[pl.ds(y[0], y[1]), :] if isinstance(y, tuple) else y
            st['h'] = jnp.concatenate([mem, yv], axis=0)

        def f_pre(_):
            st['ypre'] = ybuf[pl.ds(yPre[0], yPre[1]), :]

        def f_wq(g):
            arrive(('g', g))

        def f_tr(pjc):
            p, j, c = pjc
            for m in range(5):
                blk_ = stage[j, pl.ds(p * PW + c * 128, 128), pl.ds(m * 128, 128)]
                wqkv[p, 3 * j + c, pl.ds(m * 64, 64), :] = pltpu.bitcast(blk_.T, U32)

        def f_bw(i):
            arrive(('w', i))

        def split_qkv(p, qkv):
            st['q', p] = qkv[:, 0:PW]
            st['k', p] = blk(qkv[:, PW:2 * PW])
            st['v', p] = blk(qkv[:, 2 * PW:3 * PW])

        def f_qkv0(pcj):
            p, c, j = pcj
            if c == 0:
                lhs = jnp.concatenate([mem, ybuf[pl.ds(0, C0 - MEM), :]], axis=0)
            else:
                lhs = ybuf[pl.ds(c * C0 - MEM, C0), :]
            res = _dot(lhs, _wload(wqkv.at[p, pl.ds(3 * j, 3)], 3))
            col = p * QW + j * PW
            if c == 0:
                st['qkv'[j], p] = res[0:L] if j == 0 else blk(res[0:L])
                ring[pl.ds(SEG, C0 - L), col:col + PW] = res[L:]
            else:
                ring[pl.ds(c * C0 - MEM, C0), col:col + PW] = res

        def f_qkv(p):
            res = _dot(st['h'], _wload(wqkv.at[p], 9))
            if short is not None:
                groups, rseg = short
                for g in range(SH // 8):
                    ring[pl.ds(groups[g], 8), p * QW:(p + 1) * QW] = res[MEM + 8 * g:MEM + 8 * g + 8]
                res = jnp.concatenate([res[0:MEM], ring[pl.ds(rseg, SEG), p * QW:(p + 1) * QW]], axis=0)
            split_qkv(p, res)

        def f_s(p):
            t = _dot_nt(st['q', p], st['k', p]) * SC
            s = jnp.where(valid, t, fill)
            mA = jnp.max(jnp.where(isA, s, NEG), axis=-1, keepdims=True)
            mB = jnp.max(jnp.where(isA, NEG, s), axis=-1, keepdims=True)
            e = jnp.exp2(s - jnp.where(isA, mA, mB))
            lA = jnp.sum(jnp.where(isA, e, 0.0), axis=-1, keepdims=True)
            lB = jnp.sum(jnp.where(isA, 0.0, e), axis=-1, keepdims=True)
            l = jnp.where(isA, lA, lB)
            r = pl.reciprocal(l, approx=True)
            r = r * (2.0 - l * r)
            st['p', p] = e * r

        def f_pv(p):
            st['o', p] = _dot(st['p', p], st['v', p])

        def f_o(p):
            c = _dot(st['o', p], _wload(wo, 5, p * PW, PW))
            st['acc'] = c if 'acc' not in st else st['acc'] + c

        def f_fin(_):
            acc = st['acc']
            xbuf[pl.ds(rA, SEG), :] = xbuf[pl.ds(rA, SEG), :] + acc[MEM:, :]
            st['mem'] = acc[0:MEM, :]

        def f_b1(_):
            x1 = xbuf[pl.ds(rB1, SEG), :]
            y = _ln(x1)
            ybuf[pl.ds(rB1, SEG), :] = y
            hbuf[pl.ds(rB1 + 8, SEG), :] = _gelu(_dot(_ln(y), _wload(w1, 5)))

        def f_b2a(_):
            lane_h = jax.lax.broadcasted_iota(jnp.int32, (nB, 128), 1)

            def sh(j, d):
                win = hbuf[pl.ds(rB2, nB + 16), j * 128:(j + 1) * 128]
                return win[8 + d:8 + d + nB, :]
            cols = [
                sh(0, -1),
                jnp.where(lane_h < 32, sh(1, -1), sh(1, 1)),
                jnp.where(lane_h < 64, sh(2, 1), sh(2, -2)),
                jnp.where(lane_h < 96, sh(3, -2), sh(3, 2)),
                sh(4, 2),
            ]
            hs_in = jnp.concatenate(cols, axis=1)
            st['y1'] = ybuf[pl.ds(rB2, nB), :] + _dot(hs_in, _wload(w2, 5))

        def f_b2b(_):
            st['g'] = _gelu(_dot(_ln(st['y1']), _wload(w3, 12)))

        def f_b2c(i):
            kc = FF // NB2C
            c = _dot(st['g'][:, i * kc:(i + 1) * kc], _wload(w4, 5, i * kc, kc))
            st['h2'] = c if 'h2' not in st else st['h2'] + c

        def f_b2d(_):
            xn = xbuf[pl.ds(rB2, nB), :] + (st['y1'] + st['h2'])
            if not final:
                xbuf[pl.ds(rB2, nB), :] = xn
                ybuf[pl.ds(rB2, nB), :] = _ln(xn)
            obuf[pl.ds(rB2, nB), :] = xn.astype(BF16)

        fs = {'q': f_qkv, 'q0': f_qkv0, 's': f_s, 'v': f_pv, 'o': f_o, 'fin': f_fin, 'b1': f_b1, 'b2a': f_b2a,
              'b2b': f_b2b, 'b2c': f_b2c, 'b2d': f_b2d, 'wq': f_wq, 'tr': f_tr, 'bw': f_bw, 'ln0': ln0,
              'pre': f_pre}
        for op, p in sched:
            fs[op](p)
        return st.get('mem'), st.get('ypre')

    def seg_row(t):
        return pl.multiple_of((t & (NSEG - 1)) * SEG, SEG)

    def new_rows(t):
        return R0 + SH * (t - 1)

    with _scope("step0"):
        mem, _ = run(SCHED_0, rA=0, mem=mem0[...].astype(F32))
    with _scope("step1"):
        mem, _ = run(SCHED_1, rA=SEG, mem=mem, rB1=0, y=(new_rows(1), SH),
                     short=([(new_rows(1) + 8 * g) % RING for g in range(SH // 8)], SEG))

    def short_body(u, mem, first=False):
        t0 = 2 * u + 2
        y = (pl.multiple_of(new_rows(t0), 8), SH)
        for k in range(2):
            t = t0 + k
            groups = [pl.multiple_of(jax.lax.rem(new_rows(t) + 8 * g, RING), 8) for g in range(SH // 8)]
            rseg = pl.multiple_of(jax.lax.rem(t * SEG, RING), SEG)
            mem, y = run(SCHED_SB if k else (SCHED_S2 if first else SCHED_SA), rA=seg_row(t), mem=mem, rB1=seg_row(t - 1), rB2=seg_row(t - 2),
                         y=y, yPre=None if k else (pl.multiple_of(new_rows(t + 1), 8), SH), short=(groups, rseg))
        return mem

    with _scope("short"):
        mem = short_body(jnp.int32(0), mem, first=True)
        mem = jax.lax.fori_loop(1, (TS - 2) // 2, short_body, mem)

    def body(u, mem):
        t0 = 2 * u + TS
        y = (seg_row(t0), SEG)
        mem = jnp.where(t0 == NSEG, mem0[...].astype(F32), mem)
        for k in range(2):
            t = t0 + k
            mem, y = run(SCHED_B if k else SCHED_A, rA=seg_row(t), mem=mem, rB1=seg_row(t - 1), rB2=seg_row(t - 2),
                         y=y, yPre=None if k else (seg_row(t + 1), SEG))

        @pl.when(t0 >= NSEG + 2)
        def _():
            r = pl.multiple_of((t0 - NSEG - 2) * SEG, 2 * SEG)
            pltpu.make_async_copy(obuf.at[pl.ds(r, 2 * SEG), :], out_hbm.at[pl.ds(r, 2 * SEG), :], sem_out.at[0]).start()
        return mem

    with _scope("main"):
        jax.lax.fori_loop(0, (2 * NSEG - TS) // 2, body, mem)

    with _scope("epi"):
        r63 = (NSEG - 1) * SEG
        r62 = (NSEG - 2) * SEG
        run([('b1', 0)] + SCHED_E, rB1=r63, rB2=r62, nB=2 * SEG, final=True)
        pltpu.make_async_copy(obuf.at[pl.ds(r62, 2 * SEG), :], out_hbm.at[pl.ds(r62, 2 * SEG), :], sem_out.at[0]).start()
        pltpu.make_async_copy(obuf.at[pl.ds(0, S_TOT), :], out_hbm, sem_out.at[0]).wait()


@jax.jit
def pallas_interleave_layers__memory_aug_recurrent_mem_tr__mixer_s_mlp__prompt_kernel(A_x, A_mem0, A_Wq, A_Wk, A_Wv, A_Wo, A_seg_len, B_x, B_w1, B_w2, B_w3, B_w4):
    del A_seg_len, B_x
    x2 = A_x.reshape(S_TOT, DM)
    m2 = A_mem0.reshape(MEM, DM)
    wqT = A_Wq.transpose(1, 2, 0).reshape(HD, DM)
    wkT = A_Wk.transpose(1, 2, 0).reshape(HD, DM)
    wvT = A_Wv.transpose(1, 2, 0).reshape(HD, DM)
    wo2 = A_Wo.reshape(HD, DM)
    any_spec = pl.BlockSpec(memory_space=pl.ANY)
    out = pl.pallas_call(
        _kernel,
        out_shape=jax.ShapeDtypeStruct((S_TOT, DM), BF16),
        in_specs=[any_spec] * 10,
        out_specs=any_spec,
        scratch_shapes=[
            pltpu.VMEM((NP, 9, DM // 2, 128), U32),
            pltpu.VMEM((5, HD, 128), BF16),
            pltpu.VMEM((RING, NP * QW), F32),
            pltpu.VMEM((5, DM, 128), BF16),
            pltpu.VMEM((5, DM, 128), BF16),
            pltpu.VMEM((12, DM, 128), BF16),
            pltpu.VMEM((5, FF, 128), BF16),
            pltpu.VMEM((S_TOT + 64, DM), F32),
            pltpu.VMEM((S_TOT + 64, DM), F32),
            pltpu.VMEM((S_TOT + 64, DM), F32),
            pltpu.VMEM((S_TOT + 64, DM), BF16),
            pltpu.VMEM((3, HD, DM), BF16),
            pltpu.VMEM((S_TOT, DM), BF16),
            pltpu.VMEM((MEM, DM), BF16),
            pltpu.SemaphoreType.DMA((len(GROUPS) + 5,)),
            pltpu.SemaphoreType.DMA((1,)),
        ],
        compiler_params=pltpu.CompilerParams(vmem_limit_bytes=120 * 1024 * 1024),
    )(x2, m2, wqT, wkT, wvT, wo2, B_w1, B_w2, B_w3, B_w4)
    return out.reshape(1, S_TOT, DM)
```
